```python
import jax
import jax.numpy as jnp

def _softmax(x, axis=-1):
    return jax.nn.softmax(x, axis=axis)
def _gelu(x):
    return jax.nn.gelu(x, approximate=True)
def _silu(x):
    return jax.nn.silu(x)
def _sigmoid(x):
    return jax.nn.sigmoid(x)
def _layernorm(x, axis=-1, eps=1e-5):
    m = jnp.mean(x, axis=axis, keepdims=True)
    v = jnp.var(x, axis=axis, keepdims=True)
    return (x - m) / jnp.sqrt(v + eps)
def _scatter_add(tgt, idx, src, axis=0):
    return tgt.at[idx].add(src)
def _segment_sum(src, seg, n):
    return jax.ops.segment_sum(src, seg, n)
class _Rng:
    def __init__(self, key):
        self._k = key
    def _next(self):
        self._k, sub = jax.random.split(self._k)
        return sub
    def normal(self, shape):
        return jax.random.normal(self._next(), shape, dtype=jnp.bfloat16)
    def randint(self, lo, hi, shape):
        return jax.random.randint(self._next(), shape, lo, hi, dtype=jnp.int32)
    def uniform(self, shape, lo=0.0, hi=1.0):
        return jax.random.uniform(self._next(), shape, jnp.bfloat16, lo, hi)
    def permutation(self, n):
        return jax.random.permutation(self._next(), n)


kernel_name = 'sequential_preLN__sliding_local_dilated__glu_gated_geglu__prompt'

def setup_inputs():
    _rng = _Rng(jax.random.key(int.from_bytes(__import__("os").urandom(4), "little")))
    _w = (lambda a: (lambda t: t.astype(jnp.bfloat16) if jnp.issubdtype(t.dtype, jnp.floating) else t)(jnp.asarray(a)))
    def _A_setup():
        B, S, D = 1, 2048, 1024
        return {
            "x": _w((lambda *s: _rng.normal(s) * 0.05)(B, S, D)),
            "wqkv": _w((lambda *s: _rng.normal(s) * 0.05)(D, 3 * D)),
            "wo": _w((lambda *s: _rng.normal(s) * 0.05)(D, D)),
        }
    _A_in = _A_setup()

    def _B_setup():
        B, S, Dm, Df = 1, 2048, 1024, 3584
        return {
            "x": _w((lambda *s: _rng.normal(s) * 0.05)(B, S, Dm)),
            "w_gate": _w((lambda *s: _rng.normal(s) * 0.05)(Dm, Df) * (Dm ** -0.5)),
            "w_up": _w((lambda *s: _rng.normal(s) * 0.05)(Dm, Df) * (Dm ** -0.5)),
            "w_down": _w((lambda *s: _rng.normal(s) * 0.05)(Df, Dm) * (Df ** -0.5)),
        }
    _B_in = _B_setup()

    return {
        "A_x": _A_in["x"],
        "A_wqkv": _A_in["wqkv"],
        "A_wo": _A_in["wo"],
        "B_x": _B_in["x"],
        "B_w_gate": _B_in["w_gate"],
        "B_w_up": _B_in["w_up"],
        "B_w_down": _B_in["w_down"],
    }

def reference(A_x, A_wqkv, A_wo, B_x, B_w_gate, B_w_up, B_w_down):
    def _A_ref(x, wqkv, wo):
        B, S, D = x.shape
        H = 32; Dh = D // H
        W, dil = 8, 2
        qkv = (lambda x, *d: x.transpose(*d))((x @ wqkv).reshape(B, S, 3, H, Dh), 2, 0, 3, 1, 4)
        q, k, v = qkv[0], qkv[1], qkv[2]
        scale = Dh ** -0.5
        pos = jnp.arange(S)
        off = jnp.arange(W) * dil
        idx = pos[:, None] - off[None, :]
        mask = idx >= 0
        idx_c = jnp.where(mask, idx, 0).reshape(-1)
        kg = k[:, :, idx_c, :].reshape(B, H, S, W, Dh)
        vg = v[:, :, idx_c, :].reshape(B, H, S, W, Dh)
        logits = jnp.einsum("bhsd,bhswd->bhsw", q, kg) * scale
        logits = jnp.where(mask[None, None, :, :], logits, -1e9)
        attn = _softmax(logits, axis=-1)
        o = jnp.einsum("bhsw,bhswd->bhsd", attn, vg)
        return (lambda x, *d: x.transpose(*d))(o, 0, 2, 1, 3).reshape(B, S, D) @ wo

    def _B_ref(x, w_gate, w_up, w_down):
        g = jnp.einsum("bsd,df->bsf", x, w_gate)
        u = jnp.einsum("bsd,df->bsf", x, w_up)
        h = _gelu(g) * u
        return jnp.einsum("bsf,fd->bsd", h, w_down)

    x = A_x
    h = x + _A_ref(_layernorm(x, axis=-1), A_wqkv, A_wo)
    h2 = h + _B_ref(_layernorm(h, axis=-1), B_w_gate, B_w_up, B_w_down)
    return h2
```

```python
import functools
import numpy as np
import jax
import jax.numpy as jnp
from jax import lax
import jax.experimental.pallas as pl
import jax.experimental.pallas.tpu as pltpu

CFG = dict(TA=256, TB=256, FC=512, RC=16, skipA=False, skipB=False)

S, D, DF = 2048, 1024, 3584
H, DH, W, DIL = 32, 32, 8, 2
NT = D // 128
HALO = 16
F32, BF16 = jnp.float32, jnp.bfloat16


def _ln(x):
    m = jnp.mean(x, axis=-1, keepdims=True)
    xc = x - m
    v = jnp.mean(xc * xc, axis=-1, keepdims=True)
    return xc * lax.rsqrt(v + 1e-5)


def _permute_cols(w_ref, c0, r0, nr):
    n = nr // 2
    lane = lax.broadcasted_iota(jnp.int32, (n, 128), 1)
    tiles = []
    for t in range(NT):
        u = pltpu.bitcast(w_ref[pl.ds(r0, nr), c0 + t * 128:c0 + (t + 1) * 128], jnp.int32)
        j, g, hh = lane >> 5, (lane >> 2) & 7, lane & 3
        src = hh * 32 + ((g - t) & 7) * 4 + j
        tiles.append(jnp.take_along_axis(u, src, axis=1))
    g = (lane >> 2) & 7
    cur = [tiles[(-t) % NT] for t in range(NT)]
    for b in (1, 2, 4):
        m = (g & b) != 0
        cur = [jnp.where(m, cur[(t - b) % NT], cur[t]) for t in range(NT)]
    for tp in range(NT):
        j, t, hh = lane >> 5, (lane >> 2) & 7, lane & 3
        src = j * 32 + ((t + tp) & 7) * 4 + hh
        u = jnp.take_along_axis(cur[tp], src, axis=1) if tp else cur[tp]
        w_ref[pl.ds(r0, nr), c0 + tp * 128:c0 + (tp + 1) * 128] = pltpu.bitcast(u, BF16)


def _kernel(x_hbm, wqkv_hbm, wo_hbm, wg_hbm, wu_hbm, wd_hbm, out_hbm,
            x_v, wqkv_v, wo_v, wo_f, wg_v, wu_v, wd_v, xn_v, q_v, k_v, v_v, o_v, h_v, hn_v, a_v, out_v,
            sem_in, sem_out):
    TA, TB, FC, RC = CFG['TA'], CFG['TB'], CFG['FC'], CFG['RC']
    nA, nB = S // TA, S // TB
    cps = {}
    def mk(name, src, dst):
        cps[name] = pltpu.make_async_copy(src, dst, sem_in.at[len(cps)])
        cps[name].start()
    mk('x0', x_hbm.at[pl.ds(0, 2 * TA)], x_v.at[pl.ds(0, 2 * TA)])
    for s in range(3):
        mk(f'w{s}', wqkv_hbm.at[:, pl.ds(s * D, D)], wqkv_v.at[:, pl.ds(s * D, D)])
    mk('x1', x_hbm.at[pl.ds(2 * TA, S - 2 * TA)], x_v.at[pl.ds(2 * TA, S - 2 * TA)])
    mk('wo', wo_hbm, wo_v)
    mk('wg', wg_hbm, wg_v)
    mk('wu', wu_hbm, wu_v)
    mk('wd', wd_hbm, wd_v)

    def ln1(i):
        r = pl.ds(i * TA, TA)
        xn_v[r, :] = _ln(x_v[r, :].astype(F32)).astype(BF16)

    def qkv(i, s):
        r = pl.ds(i * TA, TA)
        y = jnp.dot(xn_v[r, :], wqkv_v[:, s * D:(s + 1) * D], preferred_element_type=F32)
        dst, off = ((q_v, 0), (k_v, HALO), (v_v, HALO))[s]
        for t in range(NT):
            dst[t, pl.ds(off + i * TA, TA), :] = y[:, t * 128:(t + 1) * 128]

    def attn_rows(r0):
        logits = []
        for w in range(W):
            acc = None
            for t in range(NT):
                p = q_v[t, pl.ds(r0, RC), :] * k_v[t, pl.ds(HALO + r0 - DIL * w, RC), :]
                acc = p if acc is None else acc + p
            acc = acc + pltpu.roll(acc, 64, 1)
            acc = acc + pltpu.roll(acc, 32, 1)
            acc = acc * (DH ** -0.5)
            if r0 < DIL * w:
                row = lax.broadcasted_iota(jnp.int32, (RC, 128), 0) + r0
                acc = jnp.where(row >= DIL * w, acc, -1e9)
            logits.append(acc)
        m = functools.reduce(jnp.maximum, logits)
        e = [jnp.exp(l - m) for l in logits]
        inv = 1.0 / functools.reduce(jnp.add, e)
        p = [a * inv for a in e]
        for t in range(NT):
            acc = None
            for w in range(W):
                c = p[w] * v_v[t, pl.ds(HALO + r0 - DIL * w, RC), :]
                acc = c if acc is None else acc + c
            o_v[pl.ds(r0, RC), t * 128:(t + 1) * 128] = acc.astype(BF16)

    def attn(i):
        for c in range(TA // RC):
            attn_rows(i * TA + c * RC)

    def wo(i):
        r = pl.ds(i * TA, TA)
        h_v[r, :] = x_v[r, :].astype(F32) + jnp.dot(o_v[r, :], wo_v[...], preferred_element_type=F32)

    def ln2(i):
        r = pl.ds(i * TA, TA)
        hn_v[r, :] = _ln(h_v[r, :]).astype(BF16)

    def permute_wo():
        for t in range(NT):
            wo_f[t] = wo_v[:, t * 128:(t + 1) * 128].astype(F32)
        for t in range(NT):
            for d in range(DH):
                wo_v[d * H:(d + 1) * H, t * 128:(t + 1) * 128] = wo_f[t, pl.ds(d, H, stride=DH), :].astype(BF16)

    cps['x0'].wait()
    if not CFG['skipA']:
        ln1(0)
        ln1(1)
        for s in range(3):
            cps[f'w{s}'].wait()
            for r0 in range(0, D, 64):
                _permute_cols(wqkv_v, s * D, r0, 64)
            qkv(0, s)
        for t in range(NT):
            k_v[t, 0:HALO, :] = jnp.broadcast_to(k_v[t, HALO:HALO + 1, :], (HALO, 128))
            v_v[t, 0:HALO, :] = jnp.broadcast_to(v_v[t, HALO:HALO + 1, :], (HALO, 128))
        cps['x1'].wait()
        cps['wo'].wait()
        permute_wo()
        for i in range(nA + 2):
            if i + 2 < nA: ln1(i + 2)
            if i < nA: attn(i)
            if i + 1 < nA:
                for s in range(3): qkv(i + 1, s)
            if 0 <= i - 1 < nA: wo(i - 1)
            if 0 <= i - 2 < nA: ln2(i - 2)
    else:
        for n in ('w0', 'w1', 'w2', 'x1', 'wo'): cps[n].wait()
        h_v[...] = x_v[...].astype(F32)
        hn_v[...] = x_v[...]
    cps['wg'].wait()
    cps['wu'].wait()
    cps['wd'].wait()

    def out_copy(i):
        r = pl.ds(pl.multiple_of(i * TB, TB), TB)
        return pltpu.make_async_copy(out_v.at[r], out_hbm.at[r], sem_out.at[i])

    def ffn(i, _):
        r = pl.ds(pl.multiple_of(i * TB, TB), TB)
        if not CFG['skipB']:
            hn = hn_v[r, :]
            for c in range(DF // FC):
                cs = slice(c * FC, (c + 1) * FC)
                g = jnp.dot(hn, wg_v[:, cs], preferred_element_type=F32)
                u = jnp.dot(hn, wu_v[:, cs], preferred_element_type=F32)
                a_v[:, cs] = (jax.nn.gelu(g, approximate=True) * u).astype(BF16)
            y = jnp.dot(a_v[...], wd_v[...], preferred_element_type=F32)
            out_v[r, :] = (h_v[r, :] + y).astype(BF16)
        else:
            out_v[r, :] = (h_v[r, :]).astype(BF16) + hn_v[r, :]
        out_copy(i).start()
    lax.fori_loop(0, nB, ffn, None)
    for i in range(nB):
        out_copy(i).wait()


@jax.jit
def pallas_sequential_preLN__sliding_local_dilated__glu_gated_geglu__prompt_kernel(
        A_x, A_wqkv, A_wo, B_x, B_w_gate, B_w_up, B_w_down):
    del B_x
    TB = CFG['TB']
    any_spec = pl.BlockSpec(memory_space=pl.ANY)
    V = pltpu.VMEM
    out = pl.pallas_call(
        _kernel,
        in_specs=[any_spec] * 6,
        out_specs=any_spec,
        out_shape=jax.ShapeDtypeStruct((S, D), BF16),
        scratch_shapes=[
            V((S, D), BF16), V((D, 3 * D), BF16), V((D, D), BF16), V((NT, D, 128), F32),
            V((D, DF), BF16), V((D, DF), BF16), V((DF, D), BF16),
            V((S, D), BF16), V((NT, S, 128), F32), V((NT, HALO + S, 128), F32), V((NT, HALO + S, 128), F32),
            V((S, D), BF16), V((S, D), F32), V((S, D), BF16), V((TB, DF), BF16), V((S, D), BF16),
            pltpu.SemaphoreType.DMA((16,)), pltpu.SemaphoreType.DMA((S // TB,)),
        ],
        compiler_params=pltpu.CompilerParams(vmem_limit_bytes=120 * 1024 * 1024),
    )(A_x.reshape(S, D), A_wqkv, A_wo, B_w_gate, B_w_up, B_w_down)
    return out.reshape(A_x.shape)
```

```python
import functools
import numpy as np
import jax
import jax.numpy as jnp
from jax import lax
import jax.experimental.pallas as pl
import jax.experimental.pallas.tpu as pltpu

CFG = dict(TA=256, TB=128, FC=512, NC=256, PR=128, skipB=False, skipP=False, scopes=False, flags={}, RP=64, WS=4, TS=2, KSPLIT=2, RA=8, LAG=32, PAD=2, dz=False)

S, D, DF = 2048, 1024, 3584
H, DH, W, DIL = 32, 32, 8, 2
NT = D // 128
HALO = 16
F32, BF16 = jnp.float32, jnp.bfloat16


def _ln(x):
    m = jnp.mean(x, axis=-1, keepdims=True)
    xc = x - m
    v = jnp.mean(xc * xc, axis=-1, keepdims=True)
    return xc * lax.rsqrt(v + 1e-5)


def _head_minor(tiles):
    lane = lax.broadcasted_iota(jnp.int32, tiles[0].shape, 1)
    g = (lane >> 2) & 7
    cur = list(tiles)
    for b in (1, 2, 4):
        cur = [jnp.where((g & b) != 0, cur[(m + b) % NT], cur[m]) for m in range(NT)]
    cur = [jnp.take_along_axis(cur[m], (lane & 3) * 32 + ((g - m) & 7) * 4 + (lane >> 5), axis=1)
           for m in range(NT)]
    cur = [cur[(-t) % NT] for t in range(NT)]
    for b in (1, 2, 4):
        cur = [jnp.where((g & b) != 0, cur[(t - b) % NT], cur[t]) for t in range(NT)]
    return cur


def _scope(name, fn):
    if CFG['scopes']:
        with jax.named_scope('s_' + name):
            fn()
    else:
        fn()


KS = HALO + S
K, O, Q, V = 0, 1, 2, 3
A0 = 4 * NT * KS


def _kernel(x_hbm, wqkv_hbm, wo_hbm, wg_hbm, wu_hbm, wd_hbm, out_hbm,
            x_v, raw_v, w_v, wo_f, wg_v, wu_v, wd_v, lhs_v, o_v, p_v, f_v, h_v, hn_v, a_v, out_v,
            sem_in, sem_out):
    TA, TB, FC, PR = CFG['TA'], CFG['TB'], CFG['FC'], CFG['PR']
    nA, nB = S // TA, S // TB
    P = functools.partial
    cps = {}

    def mk(name, src, dst):
        cps[name] = pltpu.make_async_copy(src, dst, sem_in.at[len(cps)])

    def start(*names):
        for n in names:
            cps[n].start()

    def wait(*names):
        for n in names:
            _scope('w' + n, cps[n].wait)

    KC = 256
    mk('x0', x_hbm.at[pl.ds(0, TA)], x_v.at[pl.ds(0, TA)])
    mk('x1', x_hbm.at[pl.ds(TA, 2 * TA)], x_v.at[pl.ds(TA, 2 * TA)])
    mk('x2', x_hbm.at[pl.ds(3 * TA, S - 3 * TA)], x_v.at[pl.ds(3 * TA, S - 3 * TA)])
    for c in range(D // KC):
        mk(f'wk{c}', wqkv_hbm.at[:, pl.ds(D + c * KC, KC)], raw_v.at[K, :, pl.ds(c * KC, KC)])
    mk('wq', wqkv_hbm.at[:, pl.ds(0, D)], raw_v.at[Q])
    mk('wv', wqkv_hbm.at[:, pl.ds(2 * D, D)], raw_v.at[V])
    mk('wo', wo_hbm, raw_v.at[O])
    mk('wg', wg_hbm, wg_v)
    mk('wu', wu_hbm, wu_v)
    mk('wd', wd_hbm, wd_v)

    def al(r, n):
        return pl.ds(r if isinstance(r, int) else pl.multiple_of(r, min(n, 16)), n)

    def tile(s, t):
        return (s * NT + t) * KS + HALO

    def ln1(r0, n):
        lhs_v[al(r0 // 2, n // 2), :] = pltpu.bitcast(_ln(x_v[al(r0, n), :].astype(F32)).astype(BF16), jnp.int32)

    def ln2(r0, n):
        y = jnp.concatenate([f_v[al(tile(O, t) + r0, n), :] for t in range(NT)], axis=1)
        h = x_v[al(r0, n), :].astype(F32) + y
        h_v[al(r0, n), :] = h
        hn_v[al(r0, n), :] = _ln(h).astype(BF16)

    def permute_w(s, r0):
        tiles = [pltpu.bitcast(raw_v[s, r0:r0 + PR, t * 128:(t + 1) * 128], jnp.int32) for t in range(NT)]
        for t, u in enumerate(_head_minor(tiles)):
            w_v[s, r0 // 2:(r0 + PR) // 2, t * 128:(t + 1) * 128] = u

    def permute_k(r0):
        rs = [pl.ds(tile(K, t) + r0, PR // 2) for t in range(NT)]
        for r, u in zip(rs, _head_minor([f_v[r, :] for r in rs])):
            f_v[r, :] = u

    def permute_wo(t):
        cs = slice(t * 128, (t + 1) * 128)
        wo_f[t] = raw_v[O, :, cs].astype(F32)
        for d in range(DH):
            u = wo_f[t, pl.ds(d, H, stride=DH), :].astype(BF16)
            w_v[O, d * H // 2:(d + 1) * H // 2, cs] = pltpu.bitcast(u, jnp.int32)

    def fill_halo(s):
        for t in range(NT):
            f_v[pl.ds(tile(s, t) - HALO, HALO), :] = jnp.broadcast_to(f_v[pl.ds(tile(s, t), 1), :], (HALO, 128))

    def unit(s, j, raw=False, tiles=range(NT)):
        RP, ks = CFG['RP'], CFG['KSPLIT']
        kw = D // ks
        src = (jnp.where(s == O, nA, 0) if not isinstance(s, int) else (s == O) * nA) + j
        for t in tiles:
            cs = slice(t * 128, (t + 1) * 128)
            for k in range(ks):
                lhs = pltpu.bitcast(lhs_v[al(src * (TA // 2), TA // 2), k * kw:(k + 1) * kw], BF16)
                if raw:
                    w = raw_v[s, k * kw:(k + 1) * kw, cs]
                else:
                    w = pltpu.bitcast(w_v[s, k * kw // 2:(k + 1) * kw // 2, cs], BF16)
                y = jnp.dot(lhs, w, preferred_element_type=F32)
                for r0 in range(0, TA, RP):
                    yr = y[r0:r0 + RP]
                    if k > 0:
                        yr = yr + f_v[pl.ds(A0 + r0, RP), :]
                    if k < ks - 1:
                        f_v[pl.ds(A0 + r0, RP), :] = yr
                    else:
                        f_v[al(tile(s, t) + j * TA + r0, RP), :] = yr
                    yield

    def run(units, shadow, n_tiles=NT):
        total = len(units) * n_tiles * CFG['KSPLIT'] * (TA // CFG['RP'])
        n = done = 0
        for u in units:
            for _ in u:
                n += 1
                upto = min(len(shadow), (len(shadow) * n + total - 2) // (total - 1))
                for task in shadow[done:upto]:
                    task()
                done = upto
        assert n == total and done == len(shadow)

    def logits(acc, i, r0, n, ws):
        for t in range(NT):
            q = f_v[al(tile(Q, t) + i * TA + r0, n), :]
            for w in ws:
                p = q * f_v[pl.ds(tile(K, t) + i * TA + r0 - DIL * w, n), :]
                acc[w] = p if t == 0 else acc[w] + p
        if len(acc) == W:
            softmax(acc, i, r0, n)

    def softmax(parts, i, r0, n):
        scale = DH ** -0.5
        dz = (i // nA) * 8 if CFG['dz'] else 0
        lg = []
        for w in range(W):
            acc = parts[w]
            acc = acc + pltpu.roll(acc, 64, 1)
            acc = acc + pltpu.roll(acc, 32, 1)
            if r0 < DIL * w:
                row = lax.broadcasted_iota(jnp.int32, (n, 128), 0) + (i * TA + r0)
                acc = jnp.where(row >= DIL * w, acc, -1e9 / scale)
            lg.append(acc)
        m = functools.reduce(jnp.maximum, lg)
        e = [jnp.exp2((l - m) * (scale * np.log2(np.e))) for l in lg]
        inv = 1.0 / functools.reduce(jnp.add, e)
        for w in range(W):
            p_v[w, pl.ds(r0 + dz, n), :] = e[w] * inv

    def mix(i, r0, ts):
        p = [p_v[w, pl.ds(r0, 16), :] for w in range(W)]
        for t in ts:
            acc = functools.reduce(jnp.add, [
                p[w] * f_v[pl.ds(tile(V, t) + i * TA + r0 - DIL * w, 16), :] for w in range(W)])
            o_v[pl.ds(r0 // 2, 8), t * 128:(t + 1) * 128] = pltpu.bitcast(acc.astype(BF16), jnp.int32)

    def flush(j, r0, n):
        lhs_v[al((nA + j) * (TA // 2) + r0, n), :] = o_v[pl.ds(r0, n), :]

    ln1_t = lambda j, n=1: [P(ln1, r, 32) for r in range(j * TA, (j + n) * TA, 32)]
    perm_t = lambda s: [P(permute_w, s, r0) for r0 in range(0, D, PR)]
    permk_t = lambda j: [P(permute_k, r) for r in range(j * TA, (j + 1) * TA, PR // 2)]

    if not CFG['skipP']:
        start('x0', 'wk0')
        wait('x0')
        start('wk1')
        ln1(0, TA)
        o_v[...] = jnp.zeros_like(o_v)
        nxt = [f'wk{c}' for c in range(D // KC)][2:] + ['x1', 'wq']
        for c in range(D // KC):
            wait(f'wk{c}')
            start(nxt[c])
            _scope('k0', lambda: run([unit(K, 0, True, range(2 * c, 2 * c + 2))], [], 2))
        wait('x1')
        start('wv')
        ln1(TA, TA)
        _scope('k1', lambda: run([unit(K, 1, True)], perm_t(K) + ln1_t(2)))
        wait('wq')
        start('x2')
        _scope('k2', lambda: run([unit(K, 2)], perm_t(Q) + permk_t(0) + [P(fill_halo, K)]))
        wait('wv', 'x2')
        start('wo')
        _scope('q0', lambda: run([unit(Q, 0)], perm_t(V) + ln1_t(3)))
        wait('wo')
        start('wg', 'wu', 'wd')
        _scope('v0', lambda: run([unit(V, 0), unit(K, 3), unit(K, 4)],
                                 ln1_t(4, 4) + permk_t(1) + [P(permute_wo, t) for t in range(NT)] + [P(fill_halo, V)]))

    def step(i):
        WS, TS, RA = CFG['WS'], CFG['TS'], CFG['RA']
        last = i == nA - 1
        units = [unit(jnp.where(last, O, Q), jnp.where(last, nA - 4, i + 1)),
                 unit(jnp.where(last, O, V), jnp.where(last, nA - 3, i + 1)),
                 unit(jnp.where(i < nA - 5, K, O), jnp.where(i < nA - 5, i + 5, jnp.where(last, nA - 2, i + 5 - nA)))]
        shadow = []
        LAG = CFG['LAG']
        for r0 in range(0, TA + LAG, 16):
            a = []
            for r in range(r0, r0 + 16, RA):
                parts = {}
                a += [P(logits, parts, i, r, RA, range(w, w + WS)) for w in range(0, W, WS)]
            c = [P(mix, i, r0 - LAG, range(t, t + TS)) for t in range(0, NT, TS)]
            if r0 >= TA: a = []
            nf = TA // 2 * 16 // LAG
            if r0 < LAG: c = [P(flush, jnp.maximum(i - 1, 0), r0 // 16 * nf + r, nf // 2) for r in (0, nf // 2)]
            shadow += a[:len(a) // 2] + c[:len(c) // 2] + a[len(a) // 2:] + c[len(c) // 2:]
        shadow += [lambda: None] * CFG['PAD']
        run(units, shadow)
    lax.fori_loop(0, nA, lambda i, _: _scope('step', lambda: step(i)), None)

    if not CFG['skipP']:
        flush(nA - 1, 0, TA // 2)
        _scope('wo', lambda: run([unit(O, nA - 1)], [P(ln2, r, 32) for r in range(0, TB, 32)]))
        wait('wg', 'wu', 'wd')

    def out_copy(i):
        r = pl.ds(pl.multiple_of(i * TB, TB), TB)
        return pltpu.make_async_copy(out_v.at[r], out_hbm.at[r], sem_out.at[i])

    def ffn(i):
        r = pl.ds(pl.multiple_of(i * TB, TB), TB)
        if not CFG['skipB']:
            hn = hn_v[r, :]
            for c in range(DF // FC):
                cs = slice(c * FC, (c + 1) * FC)
                g = jnp.dot(hn, wg_v[:, cs], preferred_element_type=F32)
                u = jnp.dot(hn, wu_v[:, cs], preferred_element_type=F32)
                a_v[:, cs] = (jax.nn.gelu(g, approximate=True) * u).astype(BF16)
            ln2(pl.multiple_of(jnp.minimum(i + 1, nB - 1) * TB, TB), TB)
            y = jnp.dot(a_v[...], wd_v[...], preferred_element_type=F32)
            out_v[r, :] = (h_v[r, :] + y).astype(BF16)
        else:
            out_v[r, :] = x_v[r, :]
        out_copy(i).start()
    lax.fori_loop(0, nB, lambda i, _: _scope('ffn', lambda: ffn(i)), None)
    for i in range(nB):
        out_copy(i).wait()


@jax.jit
def pallas_sequential_preLN__sliding_local_dilated__glu_gated_geglu__prompt_kernel(
        A_x, A_wqkv, A_wo, B_x, B_w_gate, B_w_up, B_w_down):
    del B_x
    TA, TB = CFG['TA'], CFG['TB']
    any_spec = pl.BlockSpec(memory_space=pl.ANY)
    M = pltpu.VMEM
    out = pl.pallas_call(
        _kernel,
        in_specs=[any_spec] * 6,
        out_specs=any_spec,
        out_shape=jax.ShapeDtypeStruct((S, D), BF16),
        scratch_shapes=[
            M((S, D), BF16), M((4, D, D), BF16), M((4, D // 2, D), jnp.int32), M((NT, D, 128), F32),
            M((D, DF), BF16), M((D, DF), BF16), M((DF, D), BF16),
            M((S, D), jnp.int32), M((TA // 2, D), jnp.int32), M((W, TA, 128), F32), M((A0 + TA, 128), F32),
            M((S, D), F32), M((S, D), BF16), M((TB, DF), BF16), M((S, D), BF16),
            pltpu.SemaphoreType.DMA((24,)), pltpu.SemaphoreType.DMA((S // TB,)),
        ],
        compiler_params=pltpu.CompilerParams(vmem_limit_bytes=120 * 1024 * 1024, flags=CFG['flags'] or None),
    )(A_x.reshape(S, D), A_wqkv, A_wo, B_w_gate, B_w_up, B_w_down)
    return out.reshape(A_x.shape)
```

```python
import functools

import jax
import jax.experimental.pallas as pl
import jax.experimental.pallas.tpu as pltpu
import jax.numpy as jnp
import numpy as np
from jax import lax

CFG = dict(FC=512, PR=32, RP=32, WS=2, TS=2, LAG=32, PAD=2, LR=16, OC=256, nest=0, fnest=0, nobc=False,
           skipP=0, skipB=False, scopes=False, flags={})

S, D, DF = 2048, 1024, 3584
H, DH, W, DIL = 32, 32, 8, 2
NT = D // 128
TA, TB = 256, 128
NA, NB = S // TA, S // TB
HALO = 16
KS = HALO + S
K, Q, V, O = 0, 1, 2, 3
KC = 256
F32, BF16, I32 = jnp.float32, jnp.bfloat16, jnp.int32
P = functools.partial


def _layernorm(x):
    xc = x - jnp.mean(x, axis=-1, keepdims=True)
    return xc * lax.rsqrt(jnp.mean(xc * xc, axis=-1, keepdims=True) + 1e-5)


def _pack(x):
    return pltpu.bitcast(x.astype(BF16), I32)


def _gather_tiles(tiles, sign):
    g = (lax.broadcasted_iota(I32, tiles[0].shape, 1) >> 2) & 7
    cur = [tiles[(sign * m) % NT] for m in range(NT)]
    for b in (1, 2, 4):
        cur = [jnp.where((g & b) != 0, cur[(m + sign * b) % NT], cur[m]) for m in range(NT)]
    return cur


def _shuffle_lanes(u, m):
    lane = lax.broadcasted_iota(I32, u.shape, 1)
    return jnp.take_along_axis(u, (lane & 3) * 32 + (((lane >> 2) - m) & 7) * 4 + (lane >> 5), axis=1)


def _merge(*lists):
    keyed = [((n + 0.5) / len(l), k, t) for k, l in enumerate(lists) for n, t in enumerate(l)]
    return [t for _, _, t in sorted(keyed, key=lambda e: e[:2])]


def _pad(tasks, n, front=0):
    return [lambda: None] * front + tasks + [lambda: None] * n


def _rows(r, n):
    return pl.ds(r if isinstance(r, int) else pl.multiple_of(r, min(n, 16)), n)


def _cols(t):
    return slice(t * 128, (t + 1) * 128)


def _tile(s, t):
    return (s * NT + t) * KS + HALO


def _scope(name, fn):
    if CFG['scopes']:
        with jax.named_scope('s_' + name):
            fn()
    else:
        fn()


def _kernel(x_hbm, wqkv_hbm, wo_hbm, wg_hbm, wu_hbm, wd_hbm, out_hbm,
            x_v,
            wk_v, wg_v, wu_v, wd_v,
            t1_v, t2_v, t3_v,
            m_v,
            f_v,
            p_v, o_v,
            a_v,
            out_v, sems):
    FC, PR, RP, LR = CFG['FC'], CFG['PR'], CFG['RP'], CFG['LR']
    raw = {Q: S, V: S + D, O: S + 2 * D}

    blocks = lambda lo, hi: (x_hbm.at[pl.ds(lo * TA, (hi - lo) * TA)], x_v.at[pl.ds(lo * TA, (hi - lo) * TA)])
    wk = lambda c: (wqkv_hbm.at[:, pl.ds(D + c * KC, KC)], wk_v.at[:, pl.ds(c * KC, KC)])
    copies = {
        'x0': blocks(0, 1), 'wk0': wk(0), 'x1': blocks(1, 2), 'wk1': wk(1), 'wk2': wk(2), 'wk3': wk(3),
        'x2': blocks(2, 3), 'x3': blocks(3, 5),
        'wq': (wqkv_hbm.at[:, pl.ds(0, D)], x_v.at[pl.ds(raw[Q], D)]),
        'wv': (wqkv_hbm.at[:, pl.ds(2 * D, D)], x_v.at[pl.ds(raw[V], D)]),
        'x5': blocks(5, NA), 'wo': (wo_hbm, x_v.at[pl.ds(raw[O], D)]),
        'wg': (wg_hbm, wg_v), 'wu': (wu_hbm, wu_v), 'wd': (wd_hbm, wd_v)}
    copies = {name: pltpu.make_async_copy(*c, sems.at[n % 3]) for n, (name, c) in enumerate(copies.items())}

    def start(*names):
        for n in names:
            copies[n].start()

    def wait(*names):
        for n in names:
            _scope('w' + n, copies[n].wait)

    start('x0', 'wk0')
    zero = lax.while_loop(lambda c: c > 0, lambda c: c - 16, 16)

    def pace(y):
        x_v[_rows(zero + S + 3 * D, 16), 0:128] = y[:16, :128].astype(BF16)

    def run(name, *lists):
        def go():
            for task in _merge(*lists):
                task()
        if CFG['skipP'] and name != CFG['skipP']:
            return
        if CFG['nest'] == 1 or (CFG['nest'] == 2 and name == 'step'):
            pl.when(zero == 0)(lambda: _scope(name, go))
        else:
            _scope(name, go)

    def project(s, j, tiles=range(NT), as_given=False):
        held = {}
        lhs_row = ((s == O) * NA + j) * (TA // 2)
        w_row, y_row = S + s * (D // 2), _tile(s, 0) + j * TA

        def task(t, r0):
            if r0 == 0:
                lhs = pltpu.bitcast(m_v[_rows(lhs_row, TA // 2), :], BF16)
                if as_given:
                    w = wk_v[:, _cols(t)]
                else:
                    w = pltpu.bitcast(m_v[_rows(w_row, D // 2), _cols(t)], BF16)
                held['y'] = jnp.dot(lhs, w, preferred_element_type=F32)
            y = held['y'][r0:r0 + RP]
            r = y_row + (t * KS + r0)
            if isinstance(s, int):
                r = r + zero
                pace(y)
                if as_given:
                    t1_v[0, _rows(zero + D // 2, 8), :] = pltpu.bitcast(y[:8], I32)
            f_v[_rows(r, RP), :] = y
        return [P(task, t, r0) for t in tiles for r0 in range(0, TA, RP)]

    def norm1(lo, hi):
        def task(r0):
            m_v[pl.ds(r0 // 2, LR // 2), :] = _pack(_layernorm(x_v[pl.ds(r0, LR), :].astype(F32)))
        return _pad([P(task, r) for r in range(lo * TA, hi * TA, LR)], 2)

    def hidden(r0, n, cs=range(NT)):
        y = jnp.concatenate([f_v[_rows(_tile(O, t) + r0, n), :] for t in cs], axis=1)
        return x_v[_rows(r0, n), cs[0] * 128:(cs[-1] + 1) * 128].astype(F32) + y

    def norm2(i, slot):
        def task(r0):
            a_v[slot, pl.ds(r0 // 2, LR // 2), 0:D] = _pack(_layernorm(hidden(i * TB + r0, LR)))
        return [P(task, r) for r in range(0, TB, LR)]

    def reorder_cols(s):
        def stage1(r0):
            src = (lambda t: wk_v[pl.ds(2 * r0, 16), _cols(t)]) if s == K else (
                lambda t: x_v[pl.ds(raw[s] + 2 * r0, 16), _cols(t)])
            for m, u in enumerate(_gather_tiles([pltpu.bitcast(src(t), I32) for t in range(NT)], 1)):
                t1_v[m, _rows(zero + r0, 8), :] = u

        def stage2(r0, m):
            t2_v[m, _rows(zero + r0, PR), :] = _shuffle_lanes(t1_v[m, pl.ds(r0, PR), :], m)

        def stage3(r0):
            for t, u in enumerate(_gather_tiles([t2_v[m, pl.ds(r0, 8), :] for m in range(NT)], -1)):
                m_v[pl.ds(S + s * (D // 2) + r0, 8), _cols(t)] = u
        tasks = []
        for r0 in range(0, D // 2 + 2 * PR, PR):
            tasks += _merge([P(stage1, r) for r in range(r0, r0 + PR, 8) if r < D // 2],
                            [P(stage2, r0 - PR, m) for m in range(NT) if 0 <= r0 - PR < D // 2],
                            [P(stage3, r - 2 * PR) for r in range(r0, r0 + PR, 8) if r >= 2 * PR])
        return _pad(tasks, 4 * 64 // PR)

    def reorder_keys(j):
        held = []

        def task(r0):
            if held:
                lo, tiles = held.pop()
                for t, u in enumerate(tiles):
                    f_v[pl.ds(_tile(K, t) + lo, 8), :] = u
            if r0 < (j + 1) * TA:
                tiles = _gather_tiles([f_v[pl.ds(_tile(K, t) + r0, 8), :] for t in range(NT)], 1)
                held.append((r0, _gather_tiles([_shuffle_lanes(u, m) for m, u in enumerate(tiles)], -1)))
        return [P(task, r) for r in range(j * TA, (j + 1) * TA + 8, 8)]

    def reorder_rows():
        def stage1(t, h0):
            for h in range(h0, h0 + 4):
                t3_v[t, pl.ds(zero + h * (DH + 1), DH), :] = x_v[pl.ds(raw[O] + h * DH, DH), _cols(t)].astype(F32)

        def stage2(t, d0):
            for d in range(d0, d0 + 4):
                m_v[pl.ds(S + (O * D + d * H) // 2, H // 2), _cols(t)] = _pack(t3_v[t, pl.ds(d, H, stride=DH + 1), :])
        tasks = []
        for t in range(NT + 1):
            tasks += _merge([P(stage1, t, h) for h in range(0, H, 4) if t < NT],
                            [P(stage2, t - 1, d) for d in range(0, DH, 4) if t > 0])
        return _pad(tasks, 4)

    def fill_halo(s, t):
        f_v[pl.ds(_tile(s, t) - HALO, HALO), :] = jnp.broadcast_to(f_v[pl.ds(_tile(s, t), 1), :], (HALO, 128))

    def flush(j, r0, n):
        m_v[_rows((NA + j) * (TA // 2) + r0, n), :] = o_v[pl.ds(r0, n), :]

    def attention(i):
        WS, TS, LAG = CFG['WS'], CFG['TS'], CFG['LAG']
        first = isinstance(i, int)
        scale = DH ** -0.5

        def scores(parts, r0, ws):
            for t in range(NT):
                q = f_v[_rows(_tile(Q, t) + i * TA + r0, 16), :]
                for w in ws:
                    qk = q * f_v[pl.ds(_tile(K, t) + i * TA + r0 - DIL * w, 16), :]
                    parts[w] = qk if t == 0 else parts[w] + qk
            if len(parts) < W:
                return
            logits = []
            for w in range(W):
                l = parts[w] + pltpu.roll(parts[w], 64, 1)
                l = l + pltpu.roll(l, 32, 1)
                if first and r0 < DIL * w:
                    l = jnp.where(lax.broadcasted_iota(I32, l.shape, 0) + r0 >= DIL * w, l, -1e9 / scale)
                logits.append(l)
            top = functools.reduce(jnp.maximum, logits)
            e = [jnp.exp2((l - top) * (scale * np.log2(np.e))) for l in logits]
            inv = 1.0 / functools.reduce(jnp.add, e)
            for w in range(W):
                p_v[w, pl.ds(r0, 16), :] = e[w] * inv

        def mix(r0, ts):
            p = [p_v[w, pl.ds(r0, 16), :] for w in range(W)]
            for t in ts:
                o_v[pl.ds(r0 // 2, 8), _cols(t)] = _pack(functools.reduce(jnp.add, [
                    p[w] * f_v[pl.ds(_tile(V, t) + i * TA + r0 - DIL * w, 16), :] for w in range(W)]))
        tasks = []
        for r0 in range(0, TA + LAG, 16):
            a, b = [], []
            if r0 < TA:
                parts = {}
                a = [P(scores, parts, r0, range(w, w + WS)) for w in range(0, W, WS)]
            if r0 >= LAG:
                b = [P(mix, r0 - LAG, range(t, t + TS)) for t in range(0, NT, TS)]
            elif not first:
                n = TA // 4 * 16 // LAG
                b = [P(flush, i - 1, r0 // 8 * n + r, n) for r in (0, n)]
            tasks += _merge(a, b)
        return _pad(tasks, CFG['PAD'])

    def keys01(lo, hi):
        return sum((project(K, j, [t], True) for t in range(lo, hi) for j in (0, 1)), [])

    wait('x0')
    start('x1')
    run('n0', norm1(0, 1))
    wait('wk0')
    start('wk1')
    run('k0', project(K, 0, range(2), True))
    wait('x1')
    start('wk2')
    run('k0', norm1(1, 2) + project(K, 1, range(2), True))
    wait('wk1')
    start('wk3', 'x2')
    run('k0', keys01(2, 4))
    wait('wk2', 'wk3', 'x2')
    start('x3')
    run('k1', keys01(4, NT), reorder_cols(K), norm1(2, 3), _pad([P(start, 'wq')], 2, 1))
    wait('x3')
    run('k2', project(K, 2), reorder_keys(0), norm1(3, 5), [P(start, 'wv')])
    wait('wq')
    run('k3', project(K, 3), reorder_cols(Q), [P(fill_halo, K, t) for t in range(NT)], [P(start, 'x5')])
    wait('wv')
    start('wo')
    run('k4', project(K, 4), reorder_cols(V))
    wait('x5')
    run('v0', project(V, 0) + project(Q, 0), reorder_keys(1), norm1(5, NA),
        _pad([P(fill_halo, V, t) for t in range(NT)], 0, NT))
    wait('wo')
    run('step0', project(Q, 1) + project(V, 1) + project(K, 5), attention(0), reorder_rows())
    start('wg', 'wu', 'wd')

    def step(i, _):
        last, late = i == NA - 1, i >= NA - 5
        run('step',
            project(jnp.where(last, O, Q), jnp.where(last, NA - 4, i + 1))
            + project(jnp.where(last, O, V), jnp.where(last, NA - 3, i + 1))
            + project(jnp.where(late, O, K), jnp.where(late, jnp.where(last, NA - 2, i + 5 - NA), i + 5)),
            attention(i))
    lax.fori_loop(1, NA, step, None)
    run('wo', [P(flush, NA - 1, 0, TA // 2)] + project(O, NA - 1), _pad(norm2(0, 0), 4))
    wait('wg', 'wu', 'wd')

    def ffn(i, slot, nxt):
        OC = CFG['OC']
        r = _rows(i * TB, TB)
        hn = pltpu.bitcast(a_v[slot, :, 0:D], BF16)
        for c in range(0, DF, FC):
            g = jnp.dot(hn, wg_v[:, c:c + FC], preferred_element_type=F32)
            u = jnp.dot(hn, wu_v[:, c:c + FC], preferred_element_type=F32)
            a_v[2, :, c:c + FC] = _pack(jax.nn.gelu(g, approximate=True) * u)
        pace(u)
        norm = norm2(nxt, 1 - slot)
        for t in range(NT):
            act = pltpu.bitcast(a_v[2], BF16)
            for task in norm[len(norm) * t // (NT - 1):len(norm) * (t + 1) // (NT - 1)]:
                task()
            y = jnp.dot(act, wd_v[:, _cols(t)], preferred_element_type=F32)
            out_v[r, _cols(t)] = (hidden(i * TB, TB, [t]) + y).astype(BF16)
            pace(y)
            if (t + 1) * 128 % OC == 0:
                c = pl.ds((t + 1) * 128 - OC, OC)
                pltpu.make_async_copy(out_v.at[r, c], out_hbm.at[r, c], sems.at[0]).start()

    def ffn_step(i, _):
        body = P(ffn, i, i & 1, jnp.minimum(i + 1, NB - 1))
        if CFG['fnest']:
            pl.when(zero == 0)(lambda: _scope('ffn', body))
        else:
            _scope('ffn', body)
    if not CFG['skipB']:
        lax.fori_loop(0, NB, ffn_step, None)
        pltpu.make_async_copy(out_v, out_v, sems.at[0]).wait()


@jax.jit
def pallas_sequential_preLN__sliding_local_dilated__glu_gated_geglu__prompt_kernel(
        A_x, A_wqkv, A_wo, B_x, B_w_gate, B_w_up, B_w_down):
    del B_x
    in_hbm = pl.BlockSpec(memory_space=pl.ANY)
    vmem = pltpu.VMEM
    out = pl.pallas_call(
        _kernel,
        in_specs=[in_hbm] * 6,
        out_specs=in_hbm,
        out_shape=jax.ShapeDtypeStruct((S, D), BF16),
        scratch_shapes=[
            vmem((S + 3 * D + 16, D), BF16),
            vmem((D, D), BF16), vmem((D, DF), BF16), vmem((D, DF), BF16), vmem((DF, D), BF16),
            vmem((NT, D // 2 + 8, 128), I32), vmem((NT, D // 2, 128), I32), vmem((NT, H * (DH + 1), 128), F32),
            vmem((S + 2 * D, D), I32),
            vmem((4 * NT * KS, 128), F32),
            vmem((W, TA, 128), F32), vmem((TA // 2, D), I32),
            vmem((3, TB // 2, DF), I32),
            vmem((S, D), BF16), pltpu.SemaphoreType.DMA((3,)),
        ],
        compiler_params=pltpu.CompilerParams(vmem_limit_bytes=120 * 1024 * 1024, flags=CFG['flags'] or None,
                                             disable_bounds_checks=CFG['nobc']),
    )(A_x.reshape(S, D), A_wqkv, A_wo, B_w_gate, B_w_up, B_w_down)
    return out.reshape(A_x.shape)
```

```python
import functools

import jax
import jax.experimental.pallas as pl
import jax.experimental.pallas.tpu as pltpu
import jax.numpy as jnp
import numpy as np
from jax import lax

CFG = dict(DN=256, PR=32, RP=32, WS=2, TS=2, LAG=32, PAD=2, LR=16, nest=0, fnest=0, nobc=True,
           skipP=0, skipB=False, scopes=False, flags={})

S, D, DF = 2048, 1024, 3584
H, DH, W, DIL = 32, 32, 8, 2
NT = D // 128
TA = 256
NA = S // TA
FC = DF // (NA - 1)
FH = DF // 2
HALO = 16
KS = HALO + S
K, Q, V, O = 0, 1, 2, 3
KC = 256
F32, BF16, I32 = jnp.float32, jnp.bfloat16, jnp.int32
P = functools.partial


def _layernorm(x):
    xc = x - jnp.mean(x, axis=-1, keepdims=True)
    return xc * lax.rsqrt(jnp.mean(xc * xc, axis=-1, keepdims=True) + 1e-5)


def _pack(x):
    return pltpu.bitcast(x.astype(BF16), I32)


def _gather_tiles(tiles, sign):
    g = (lax.broadcasted_iota(I32, tiles[0].shape, 1) >> 2) & 7
    cur = [tiles[(sign * m) % NT] for m in range(NT)]
    for b in (1, 2, 4):
        cur = [jnp.where((g & b) != 0, cur[(m + sign * b) % NT], cur[m]) for m in range(NT)]
    return cur


def _shuffle_lanes(u, m):
    lane = lax.broadcasted_iota(I32, u.shape, 1)
    return jnp.take_along_axis(u, (lane & 3) * 32 + (((lane >> 2) - m) & 7) * 4 + (lane >> 5), axis=1)


def _lhs_terms(a11, a12, a21, a22):
    return [a11 + a22, a21 + a22, a11, a22, a11 + a12, a21 - a11, a12 - a22]


def _rhs_terms(b11, b12, b21, b22):
    return [b11 + b22, b11, b12 - b22, b21 - b11, b22, b11 + b12, b21 + b22]


def _quadrants(product):
    m0, m1 = product(0), product(1)
    c22 = m0 - m1
    m3 = product(3)
    c21, c11 = m1 + m3, m0 + m3
    m2 = product(2)
    c22 = c22 + m2
    m4 = product(4)
    c12, c11 = m2 + m4, c11 - m4
    c22 = c22 + product(5)
    return c11 + product(6), c12, c21, c22


def _merge(*lists):
    keyed = [((n + 0.5) / len(l), k, t) for k, l in enumerate(lists) for n, t in enumerate(l)]
    return [t for _, _, t in sorted(keyed, key=lambda e: e[:2])]


def _pad(tasks, n, front=0):
    return [lambda: None] * front + tasks + [lambda: None] * n


def _rows(r, n):
    return pl.ds(r if isinstance(r, int) else pl.multiple_of(r, min(n, 16)), n)


def _cols(t):
    return slice(t * 128, (t + 1) * 128)


def _tile(s, t):
    return (s * NT + t) * KS + HALO


def _scope(name, fn):
    if CFG['scopes']:
        with jax.named_scope('s_' + name):
            fn()
    else:
        fn()


def _kernel(x_hbm, wqkv_hbm, wo_hbm, wg_hbm, wu_hbm, wd_hbm, out_hbm,
            x_v,
            wk_v,
            wgu_v, wd_v,
            t1_v, t2_v, t3_v,
            m_v,
            f_v,
            p_v, o_v,
            hn_v, a_v,
            out_v, sems):
    PR, RP, LR = CFG['PR'], CFG['RP'], CFG['LR']
    raw = {Q: S, V: S + D, O: S + 2 * D}

    blocks = lambda lo, hi: (x_hbm.at[pl.ds(lo * TA, (hi - lo) * TA)], x_v.at[pl.ds(lo * TA, (hi - lo) * TA)])
    wk = lambda c: (wqkv_hbm.at[:, pl.ds(D + c * KC, KC)], wk_v.at[:, pl.ds(c * KC, KC)])
    copies = {
        'x0': blocks(0, 1), 'wk0': wk(0), 'x1': blocks(1, 2), 'wk1': wk(1), 'wk2': wk(2), 'wk3': wk(3),
        'x2': blocks(2, 3), 'x3': blocks(3, 5),
        'wq': (wqkv_hbm.at[:, pl.ds(0, D)], x_v.at[pl.ds(raw[Q], D)]),
        'wv': (wqkv_hbm.at[:, pl.ds(2 * D, D)], x_v.at[pl.ds(raw[V], D)]),
        'x5': blocks(5, NA), 'wo': (wo_hbm, x_v.at[pl.ds(raw[O], D)])}
    copies = {name: pltpu.make_async_copy(*c, sems.at[n % 3]) for n, (name, c) in enumerate(copies.items())}

    def start(*names):
        for n in names:
            copies[n].start()

    def wait(*names):
        for n in names:
            _scope('w' + n, copies[n].wait)

    start('x0', 'wk0')
    zero = lax.while_loop(lambda c: c > 0, lambda c: c - 16, 16)

    def pace(y):
        x_v[_rows(zero + S + 3 * D, 16), 0:128] = y[:16, :128].astype(BF16)

    def run(name, *lists):
        def go():
            for task in _merge(*lists):
                task()
        if CFG['skipP'] and name != CFG['skipP']:
            return
        if CFG['nest'] == 1 or (CFG['nest'] == 2 and name == 'step'):
            pl.when(zero == 0)(lambda: _scope(name, go))
        else:
            _scope(name, go)

    def project(s, j, tiles=range(NT), as_given=False):
        held = {}
        lhs_row = ((s == O) * NA + j) * (TA // 2)
        w_row, y_row = S + s * (D // 2), _tile(s, 0) + j * TA

        def task(t, r0):
            if r0 == 0:
                lhs = pltpu.bitcast(m_v[_rows(lhs_row, TA // 2), :], BF16)
                if as_given:
                    w = wk_v[:, _cols(t)]
                else:
                    w = pltpu.bitcast(m_v[_rows(w_row, D // 2), _cols(t)], BF16)
                held['y'] = jnp.dot(lhs, w, preferred_element_type=F32)
            y = held['y'][r0:r0 + RP]
            r = y_row + (t * KS + r0)
            pace(y)
            if isinstance(s, int):
                r = r + zero
                if as_given:
                    t1_v[0, _rows(zero + D // 2, 8), :] = pltpu.bitcast(y[:8], I32)
            f_v[_rows(r, RP), :] = y
        return [P(task, t, r0) for t in tiles for r0 in range(0, TA, RP)]

    def norm1(lo, hi):
        def task(r0):
            m_v[pl.ds(r0 // 2, LR // 2), :] = _pack(_layernorm(x_v[pl.ds(r0, LR), :].astype(F32)))
        return _pad([P(task, r) for r in range(lo * TA, hi * TA, LR)], 2)

    def hidden(r0, n, cs=range(NT)):
        y = jnp.concatenate([f_v[_rows(_tile(O, t) + r0, n), :] for t in cs], axis=1)
        return x_v[_rows(r0, n), cs[0] * 128:(cs[-1] + 1) * 128].astype(F32) + y

    def norm2(j, slot, lo, n):
        def task(r0):
            top, bot = (_layernorm(hidden(j * TA + half + r0, 16)) for half in (0, TA // 2))
            for k, u in enumerate(_lhs_terms(top[:, :D // 2], top[:, D // 2:], bot[:, :D // 2], bot[:, D // 2:])):
                hn_v[slot, k, _rows(r0 // 2, 8), :] = _pack(u)
        return [P(task, lo + r) for r in range(0, n, 16)]

    def ffn_copies(c):
        r, f = S + (c & 1) * (D + FC), pl.ds(pl.multiple_of(c * FC, FC), FC)
        return [pltpu.make_async_copy(wg_hbm.at[:, f], x_v.at[_rows(r, D), pl.ds(0, FC)], sems.at[0]),
                pltpu.make_async_copy(wu_hbm.at[:, f], x_v.at[_rows(r, D), pl.ds(FC, FC)], sems.at[1]),
                pltpu.make_async_copy(wd_hbm.at[f], x_v.at[_rows(r + D, FC)], sems.at[2])]

    def ffn_weights(c):
        base = S + (c & 1) * (D + FC)
        get = lambda r, t: x_v[_rows(base + r, 16), _cols(t)].astype(F32)

        def gate_up(r0, pair):
            for m in range(2):
                t = m * (FC // 128) + 2 * pair
                terms = _rhs_terms(get(r0, t), get(r0, t + 1), get(D // 2 + r0, t), get(D // 2 + r0, t + 1))
                for k, u in enumerate(terms):
                    wgu_v[c * (FC // 256) + pair, k, pl.ds(r0 // 2, 8), _cols(m)] = _pack(u)

        def down(pair, r0, t0):
            r = D + pair * 256 + r0
            for t in (t0, t0 + 1):
                terms = _rhs_terms(get(r, t), get(r, t + NT // 2), get(r + 128, t), get(r + 128, t + NT // 2))
                for k, u in enumerate(terms):
                    wd_v[k, _rows((c * (FC // 256) + pair) * 64 + r0 // 2, 8), _cols(t)] = _pack(u)
        return _pad([P(gate_up, r, p) for p in range(FC // 256) for r in range(0, D // 2, 16)]
                    + [P(down, p, r, t) for p in range(FC // 256) for r in range(0, 128, 16) for t in (0, 2)], 2)

    def reorder_cols(s):
        def stage1(r0):
            src = (lambda t: wk_v[pl.ds(2 * r0, 16), _cols(t)]) if s == K else (
                lambda t: x_v[pl.ds(raw[s] + 2 * r0, 16), _cols(t)])
            for m, u in enumerate(_gather_tiles([pltpu.bitcast(src(t), I32) for t in range(NT)], 1)):
                t1_v[m, _rows(zero + r0, 8), :] = u

        def stage2(r0, m):
            t2_v[m, _rows(zero + r0, PR), :] = _shuffle_lanes(t1_v[m, pl.ds(r0, PR), :], m)

        def stage3(r0):
            for t, u in enumerate(_gather_tiles([t2_v[m, pl.ds(r0, 8), :] for m in range(NT)], -1)):
                m_v[pl.ds(S + s * (D // 2) + r0, 8), _cols(t)] = u
        tasks = []
        for r0 in range(0, D // 2 + 2 * PR, PR):
            tasks += _merge([P(stage1, r) for r in range(r0, r0 + PR, 8) if r < D // 2],
                            [P(stage2, r0 - PR, m) for m in range(NT) if 0 <= r0 - PR < D // 2],
                            [P(stage3, r - 2 * PR) for r in range(r0, r0 + PR, 8) if r >= 2 * PR])
        return _pad(tasks, 4 * 64 // PR)

    def reorder_keys(j):
        held = []

        def task(r0):
            if held:
                lo, tiles = held.pop()
                for t, u in enumerate(tiles):
                    f_v[pl.ds(_tile(K, t) + lo, 8), :] = u
            if r0 < (j + 1) * TA:
                tiles = _gather_tiles([f_v[pl.ds(_tile(K, t) + r0, 8), :] for t in range(NT)], 1)
                held.append((r0, _gather_tiles([_shuffle_lanes(u, m) for m, u in enumerate(tiles)], -1)))
        return [P(task, r) for r in range(j * TA, (j + 1) * TA + 8, 8)]

    def reorder_rows():
        def stage1(t, h0):
            for h in range(h0, h0 + 4):
                t3_v[t % 2, pl.ds(zero + h * (DH + 1), DH), :] = x_v[pl.ds(raw[O] + h * DH, DH), _cols(t)].astype(F32)

        def stage2(t, d0):
            for d in range(d0, d0 + 4):
                m_v[pl.ds(S + (O * D + d * H) // 2, H // 2), _cols(t)] = _pack(t3_v[t % 2, pl.ds(d, H, stride=DH + 1), :])
        tasks = []
        for t in range(NT + 1):
            tasks += _merge([P(stage1, t, h) for h in range(0, H, 4) if t < NT],
                            [P(stage2, t - 1, d) for d in range(0, DH, 4) if t > 0])
        return _pad(tasks, 4)

    def fill_halo(s, t):
        f_v[pl.ds(_tile(s, t) - HALO, HALO), :] = jnp.broadcast_to(f_v[pl.ds(_tile(s, t), 1), :], (HALO, 128))

    def flush(j, r0, n):
        m_v[_rows((NA + j) * (TA // 2) + r0, n), :] = o_v[pl.ds(r0, n), :]

    def attention(i):
        WS, TS, LAG = CFG['WS'], CFG['TS'], CFG['LAG']
        first = isinstance(i, int)
        scale = DH ** -0.5

        def scores(parts, r0, ws):
            for t in range(NT):
                q = f_v[_rows(_tile(Q, t) + i * TA + r0, 16), :]
                for w in ws:
                    qk = q * f_v[pl.ds(_tile(K, t) + i * TA + r0 - DIL * w, 16), :]
                    parts[w] = qk if t == 0 else parts[w] + qk
            if len(parts) < W:
                return
            logits = []
            for w in range(W):
                l = parts[w] + pltpu.roll(parts[w], 64, 1)
                l = l + pltpu.roll(l, 32, 1)
                if first and r0 < DIL * w:
                    l = jnp.where(lax.broadcasted_iota(I32, l.shape, 0) + r0 >= DIL * w, l, -1e9 / scale)
                logits.append(l)
            top = functools.reduce(jnp.maximum, logits)
            e = [jnp.exp2((l - top) * (scale * np.log2(np.e))) for l in logits]
            inv = 1.0 / functools.reduce(jnp.add, e)
            for w in range(W):
                p_v[w, pl.ds(r0, 16), :] = e[w] * inv

        def mix(r0, ts):
            p = [p_v[w, pl.ds(r0, 16), :] for w in range(W)]
            for t in ts:
                o_v[pl.ds(r0 // 2, 8), _cols(t)] = _pack(functools.reduce(jnp.add, [
                    p[w] * f_v[pl.ds(_tile(V, t) + i * TA + r0 - DIL * w, 16), :] for w in range(W)]))
        tasks = []
        for r0 in range(0, TA + LAG, 16):
            a, b = [], []
            if r0 < TA:
                parts = {}
                a = [P(scores, parts, r0, range(w, w + WS)) for w in range(0, W, WS)]
            if r0 >= LAG:
                b = [P(mix, r0 - LAG, range(t, t + TS)) for t in range(0, NT, TS)]
            elif not first:
                n = TA // 4 * 16 // LAG
                b = [P(flush, i - 1, r0 // 8 * n + r, n) for r in (0, n)]
            tasks += _merge(a, b)
        return _pad(tasks, CFG['PAD'])

    def keys01(lo, hi):
        return sum((project(K, j, [t], True) for t in range(lo, hi) for j in (0, 1)), [])

    wait('x0')
    start('x1')
    run('n0', norm1(0, 1))
    wait('wk0')
    start('wk1')
    run('k0', project(K, 0, range(2), True))
    wait('x1')
    start('wk2')
    run('k0', norm1(1, 2) + project(K, 1, range(2), True))
    wait('wk1')
    start('wk3', 'x2')
    run('k0', keys01(2, 4))
    wait('wk2', 'wk3', 'x2')
    start('x3')
    run('k1', keys01(4, NT), reorder_cols(K), norm1(2, 3), _pad([P(start, 'wq')], 2, 1))
    wait('x3')
    run('k2', project(K, 2), reorder_keys(0), norm1(3, 5), [P(start, 'wv')])
    wait('wq')
    run('k3', project(K, 3), reorder_cols(Q), [P(fill_halo, K, t) for t in range(NT)], [P(start, 'x5')])
    wait('wv')
    start('wo')
    run('k4', project(K, 4), reorder_cols(V))
    wait('x5')
    run('v0', project(V, 0) + project(Q, 0), reorder_keys(1), norm1(5, NA),
        _pad([P(fill_halo, V, t) for t in range(NT)], 0, NT))
    wait('wo')
    for copy in ffn_copies(0):
        copy.start()
    run('step0', project(Q, 1) + project(V, 1) + project(K, 5), attention(0), reorder_rows())

    def step(i, _):
        for copy in ffn_copies(i - 1):
            copy.wait()

        @pl.when(i < NA - 1)
        def _():
            for copy in ffn_copies(i):
                copy.start()
        last, late = i == NA - 1, i >= NA - 5
        run('step',
            project(jnp.where(last, O, Q), jnp.where(last, NA - 4, i + 1))
            + project(jnp.where(last, O, V), jnp.where(last, NA - 3, i + 1))
            + project(jnp.where(late, O, K), jnp.where(late, jnp.where(last, NA - 2, i + 5 - NA), i + 5)),
            attention(i), ffn_weights(i - 1))
    lax.fori_loop(1, NA, step, None)
    run('wo', [P(flush, NA - 1, 0, TA // 2)] + project(O, NA - 1), _pad(norm2(0, 0, 0, TA // 2), 2))

    def ffn(i):
        j, half = i >> 1, i & 1
        slot, pairs, DN = j & 1, FH // 256, CFG['DN']
        norm = norm2(jnp.minimum(j + 1, NA - 1), 1 - slot, half * (TA // 4), TA // 4)
        for p in range(pairs):
            def product(k):
                hn = pltpu.bitcast(hn_v[slot, k], BF16)
                if k == 6:
                    for task in norm[len(norm) * p // pairs:len(norm) * (p + 1) // pairs]:
                        task()
                y = jnp.dot(hn, pltpu.bitcast(wgu_v[half * pairs + p, k], BF16), preferred_element_type=F32)
                if k == 0:
                    pace(y)
                return y
            gu = _quadrants(product)
            act = [jax.nn.gelu(c[:, :128], approximate=True) * c[:, 128:] for c in gu]
            for k, u in enumerate(_lhs_terms(*act)):
                a_v[k, :, _cols(p)] = _pack(u)
        for c in range(0, D // 2, DN):
            y = _quadrants(lambda k: jnp.dot(
                pltpu.bitcast(a_v[k], BF16), pltpu.bitcast(wd_v[k, _rows(half * (FH // 4), FH // 4), c:c + DN], BF16),
                preferred_element_type=F32))
            for n in (2, 1, 3, 0):
                r = j * TA + n // 2 * (TA // 2)
                for t in range(DN // 128):
                    tt = (n % 2 * (D // 2) + c) // 128 + t
                    acc = f_v[_rows(_tile(O, tt) + r, TA // 2), :] + y[n][:, _cols(t)]
                    f_v[_rows(_tile(O, tt) + r, TA // 2), :] = acc
                    out_v[_rows(r, TA // 2), _cols(tt)] = (x_v[_rows(r, TA // 2), _cols(tt)].astype(F32) + acc).astype(BF16)

        @pl.when(half == 1)
        def _():
            pltpu.make_async_copy(out_v.at[_rows(j * TA, TA)], out_hbm.at[_rows(j * TA, TA)], sems.at[0]).start()

    if not CFG['skipB']:
        lax.fori_loop(0, 2 * NA, lambda i, _: _scope('ffn', P(ffn, i)), None)
        pltpu.make_async_copy(out_v, out_v, sems.at[0]).wait()


@jax.jit
def pallas_sequential_preLN__sliding_local_dilated__glu_gated_geglu__prompt_kernel(
        A_x, A_wqkv, A_wo, B_x, B_w_gate, B_w_up, B_w_down):
    del B_x
    in_hbm = pl.BlockSpec(memory_space=pl.ANY)
    vmem = pltpu.VMEM
    out = pl.pallas_call(
        _kernel,
        in_specs=[in_hbm] * 6,
        out_specs=in_hbm,
        out_shape=jax.ShapeDtypeStruct((S, D), BF16),
        scratch_shapes=[
            vmem((S + 3 * D + 16, D), BF16),
            vmem((D, D), BF16), vmem((DF // 256, 7, D // 4, 256), I32), vmem((7, DF // 4, D // 2), I32),
            vmem((NT, D // 2 + 8, 128), I32), vmem((NT, D // 2, 128), I32), vmem((2, H * (DH + 1), 128), F32),
            vmem((S + 2 * D, D), I32),
            vmem((4 * NT * KS, 128), F32),
            vmem((W, TA, 128), F32), vmem((TA // 2, D), I32),
            vmem((2, 7, TA // 4, D // 2), I32), vmem((7, TA // 4, FH // 2), I32),
            vmem((S, D), BF16), pltpu.SemaphoreType.DMA((3,)),
        ],
        compiler_params=pltpu.CompilerParams(vmem_limit_bytes=126 * 1024 * 1024, flags=CFG['flags'] or None,
                                             disable_bounds_checks=CFG['nobc']),
    )(A_x.reshape(S, D), A_wqkv, A_wo, B_w_gate, B_w_up, B_w_down)
    return out.reshape(A_x.shape)
```

```python
import functools

import jax
import jax.experimental.pallas as pl
import jax.experimental.pallas.tpu as pltpu
import jax.numpy as jnp
import numpy as np
from jax import lax

CFG = dict(FP=2, halves=2, PR=32, RP=32, WS=2, TS=2, LAG=32, PAD=2, LR=16, nest=0, fnest=0, nobc=True,
           skipP=0, skipB=False, scopes=False, flags={})

S, D, DF = 2048, 1024, 3584
H, DH, W, DIL = 32, 32, 8, 2
NT = D // 128
TA = 256
NA = S // TA
FC = 256
NC = DF // (2 * FC)
HALO = 16
KS = HALO + S
K, Q, V, O = 0, 1, 2, 3
H0 = 4 * NT * KS
KC = 256
F32, BF16, I32 = jnp.float32, jnp.bfloat16, jnp.int32
P = functools.partial


def _layernorm(x):
    xc = x - jnp.mean(x, axis=-1, keepdims=True)
    return xc * lax.rsqrt(jnp.mean(xc * xc, axis=-1, keepdims=True) + 1e-5)


def _pack(x):
    return pltpu.bitcast(x.astype(BF16), I32)


def _gather_tiles(tiles, sign):
    g = (lax.broadcasted_iota(I32, tiles[0].shape, 1) >> 2) & 7
    cur = [tiles[(sign * m) % NT] for m in range(NT)]
    for b in (1, 2, 4):
        cur = [jnp.where((g & b) != 0, cur[(m + sign * b) % NT], cur[m]) for m in range(NT)]
    return cur


def _shuffle_lanes(u, m):
    lane = lax.broadcasted_iota(I32, u.shape, 1)
    return jnp.take_along_axis(u, (lane & 3) * 32 + (((lane >> 2) - m) & 7) * 4 + (lane >> 5), axis=1)


def _lhs_terms(a11, a12, a21, a22):
    return [a11 + a22, a21 + a22, a11, a22, a11 + a12, a21 - a11, a12 - a22]


def _rhs_terms(b11, b12, b21, b22):
    c11, c12, c21, c22 = (b.astype(F32) for b in (b11, b12, b21, b22))
    return [c11 + c22, b11, c12 - c22, c21 - c11, b22, c11 + c12, c21 + c22]


def _quadrants(product):
    m0, m1 = product(0), product(1)
    c22 = m0 - m1
    m3 = product(3)
    c21, c11 = m1 + m3, m0 + m3
    m2 = product(2)
    c22 = c22 + m2
    m4 = product(4)
    c12, c11 = m2 + m4, c11 - m4
    c22 = c22 + product(5)
    return c11 + product(6), c12, c21, c22


def _merge(*lists):
    keyed = [((n + 0.5) / len(l), k, t) for k, l in enumerate(lists) for n, t in enumerate(l)]
    return [t for _, _, t in sorted(keyed, key=lambda e: e[:2])]


def _pad(tasks, n, front=0):
    return [lambda: None] * front + tasks + [lambda: None] * n


def _rows(r, n):
    return pl.ds(r if isinstance(r, int) else pl.multiple_of(r, min(n, 16)), n)


def _cols(t):
    return slice(t * 128, (t + 1) * 128)


def _tile(s, t):
    return (s * NT + t) * KS + HALO


def _scope(name, fn):
    if CFG['scopes']:
        with jax.named_scope('s_' + name):
            fn()
    else:
        fn()


def _kernel(x_hbm, wqkv_hbm, wo_hbm, wg_hbm, wu_hbm, wd_hbm, out_hbm,
            x_v,
            wk_v,
            wgu_v, wd_v,
            t1_v, t2_v, t3_v,
            m_v,
            f_v,
            p_v, o_v,
            hn_v, a_v,
            out_v, sems):
    PR, RP, LR = CFG['PR'], CFG['RP'], CFG['LR']
    raw = {Q: S, V: S + D, O: S + 2 * D}

    blocks = lambda lo, hi: (x_hbm.at[pl.ds(lo * TA, (hi - lo) * TA)], x_v.at[pl.ds(lo * TA, (hi - lo) * TA)])
    wk = lambda c: (wqkv_hbm.at[:, pl.ds(D + c * KC, KC)], wk_v.at[:, pl.ds(c * KC, KC)])
    copies = {
        'x0': blocks(0, 1), 'wk0': wk(0), 'x1': blocks(1, 2), 'wk1': wk(1), 'wk2': wk(2), 'wk3': wk(3),
        'x2': blocks(2, 3), 'x3': blocks(3, 5),
        'wq': (wqkv_hbm.at[:, pl.ds(0, D)], x_v.at[pl.ds(raw[Q], D)]),
        'wv': (wqkv_hbm.at[:, pl.ds(2 * D, D)], x_v.at[pl.ds(raw[V], D)]),
        'x5': blocks(5, NA), 'wo': (wo_hbm, x_v.at[pl.ds(raw[O], D)])}
    copies = {name: pltpu.make_async_copy(*c, sems.at[n % 3]) for n, (name, c) in enumerate(copies.items())}

    def start(*names):
        for n in names:
            copies[n].start()

    def wait(*names):
        for n in names:
            _scope('w' + n, copies[n].wait)

    start('x0', 'wk0')
    zero = lax.while_loop(lambda c: c > 0, lambda c: c - 16, 16)

    def pace(y):
        x_v[_rows(zero + S + 3 * D, 16), 0:128] = y[:16, :128].astype(BF16)

    def run(name, *lists):
        def go():
            for task in _merge(*lists):
                task()
        if CFG['skipP'] and name != CFG['skipP']:
            return
        if CFG['nest'] == 1 or (CFG['nest'] == 2 and name == 'step'):
            pl.when(zero == 0)(lambda: _scope(name, go))
        else:
            _scope(name, go)

    def project(s, j, tiles=range(NT), as_given=False):
        held = {}
        lhs_row = ((s == O) * NA + j) * (TA // 2)
        w_row, y_row = S + s * (D // 2), _tile(s, 0) + j * TA

        def task(t, r0):
            if r0 == 0:
                lhs = pltpu.bitcast(m_v[_rows(lhs_row, TA // 2), :], BF16)
                if as_given:
                    w = wk_v[:, _cols(t)]
                else:
                    w = pltpu.bitcast(m_v[_rows(w_row, D // 2), _cols(t)], BF16)
                held['y'] = jnp.dot(lhs, w, preferred_element_type=F32)
            y = held['y'][r0:r0 + RP]
            r = y_row + (t * KS + r0)
            pace(y)
            if isinstance(s, int):
                r = r + zero
                if as_given:
                    t1_v[0, _rows(zero + D // 2, 8), :] = pltpu.bitcast(y[:8], I32)
            f_v[_rows(r, RP), :] = y
        return [P(task, t, r0) for t in tiles for r0 in range(0, TA, RP)]

    def norm1(lo, hi):
        def task(r0):
            m_v[pl.ds(r0 // 2, LR // 2), :] = _pack(_layernorm(x_v[pl.ds(r0, LR), :].astype(F32)))
        return _pad([P(task, r) for r in range(lo * TA, hi * TA, LR)], 2)

    def hidden(r0, n, cs=range(NT)):
        y = jnp.concatenate([f_v[_rows(_tile(O, t) + r0, n), :] for t in cs], axis=1)
        return x_v[_rows(r0, n), cs[0] * 128:(cs[-1] + 1) * 128].astype(F32) + y

    def norm_terms(source, store, n):
        stats = {}

        def center(r):
            h = source(r)
            for t in range(NT):
                f_v[pl.ds(H0 + t * TA + r, 16), :] = h[:, _cols(t)]
            stats[r] = jnp.mean(h, axis=-1, keepdims=True)

        def spread(r):
            hc = jnp.concatenate([f_v[pl.ds(H0 + t * TA + r, 16), :] for t in range(NT)], axis=1) - stats[r]
            stats[r] = (stats[r], lax.rsqrt(jnp.mean(hc * hc, axis=-1, keepdims=True) + 1e-5))

        def terms(r0, t):
            get = lambda r, t: (f_v[pl.ds(H0 + t * TA + r, 16), :] - stats[r][0]) * stats[r][1]
            for k, u in enumerate(_lhs_terms(*[get(r, c) for r in (r0, r0 + TA // 2) for c in (t, t + NT // 2)])):
                store(k, r0, t, _pack(u))
        return ([P(f, r0 + r) for f in (center, spread) for r0 in range(0, n, 16) for r in (0, TA // 2)]
                + [P(terms, r0, t) for r0 in range(0, n, 16) for t in range(NT // 2)])

    def norm2(j):
        def store(k, r0, t, u):
            hn_v[j, k, pl.ds(r0 // 2, 8), _cols(t)] = u
        return norm_terms(lambda r: hidden(j * TA + r, 16), store, TA // 2)

    def ffn_copies(c):
        r, f = S + (c & 1) * (D + FC), pl.ds(pl.multiple_of(c * FC, FC), FC)
        return [pltpu.make_async_copy(wg_hbm.at[:, f], x_v.at[_rows(r, D), pl.ds(0, FC)], sems.at[0]),
                pltpu.make_async_copy(wu_hbm.at[:, f], x_v.at[_rows(r, D), pl.ds(FC, FC)], sems.at[1]),
                pltpu.make_async_copy(wd_hbm.at[f], x_v.at[_rows(r + D, FC)], sems.at[2])]

    def ffn_weights(half, c):
        base = S + ((half * NC + c) & 1) * (D + FC)
        get = lambda r, col: x_v[_rows(base + r, 16), col:col + 256]

        def gate_up(r0, m):
            top, bot = get(r0, m * FC), get(D // 2 + r0, m * FC)
            for k, u in enumerate(_rhs_terms(top[:, :128], top[:, 128:], bot[:, :128], bot[:, 128:])):
                wgu_v[half][c, k, pl.ds(r0 // 2, 8), _cols(m)] = _pack(u)

        def down(r0, t):
            top, bot = get(D + r0, t * 256), get(D + FC // 2 + r0, t * 256)
            for k, u in enumerate(_rhs_terms(top[:, :128], top[:, 128:], bot[:, :128], bot[:, 128:])):
                wd_v[half][k, _rows(c * (FC // 4) + r0 // 2, 8), _cols(t)] = _pack(u)
        return _pad([P(gate_up, r, m) for r in range(0, D // 2, 16) for m in range(2)]
                    + [P(down, r, t) for r in range(0, FC // 2, 16) for t in range(NT // 2)], 2)

    def reorder_cols(s):
        def stage1(r0):
            src = (lambda t: wk_v[pl.ds(2 * r0, 16), _cols(t)]) if s == K else (
                lambda t: x_v[pl.ds(raw[s] + 2 * r0, 16), _cols(t)])
            for m, u in enumerate(_gather_tiles([pltpu.bitcast(src(t), I32) for t in range(NT)], 1)):
                t1_v[m, _rows(zero + r0, 8), :] = u

        def stage2(r0, m):
            t2_v[m, _rows(zero + r0, PR), :] = _shuffle_lanes(t1_v[m, pl.ds(r0, PR), :], m)

        def stage3(r0):
            for t, u in enumerate(_gather_tiles([t2_v[m, pl.ds(r0, 8), :] for m in range(NT)], -1)):
                m_v[pl.ds(S + s * (D // 2) + r0, 8), _cols(t)] = u
        tasks = []
        for r0 in range(0, D // 2 + 2 * PR, PR):
            tasks += _merge([P(stage1, r) for r in range(r0, r0 + PR, 8) if r < D // 2],
                            [P(stage2, r0 - PR, m) for m in range(NT) if 0 <= r0 - PR < D // 2],
                            [P(stage3, r - 2 * PR) for r in range(r0, r0 + PR, 8) if r >= 2 * PR])
        return _pad(tasks, 4 * 64 // PR)

    def reorder_keys(j):
        held = []

        def task(r0):
            if held:
                lo, tiles = held.pop()
                for t, u in enumerate(tiles):
                    f_v[pl.ds(_tile(K, t) + lo, 8), :] = u
            if r0 < (j + 1) * TA:
                tiles = _gather_tiles([f_v[pl.ds(_tile(K, t) + r0, 8), :] for t in range(NT)], 1)
                held.append((r0, _gather_tiles([_shuffle_lanes(u, m) for m, u in enumerate(tiles)], -1)))
        return [P(task, r) for r in range(j * TA, (j + 1) * TA + 8, 8)]

    def reorder_rows():
        def stage1(t, h0):
            for h in range(h0, h0 + 4):
                t3_v[t % 2, pl.ds(zero + h * (DH + 1), DH), :] = x_v[pl.ds(raw[O] + h * DH, DH), _cols(t)].astype(F32)

        def stage2(t, d0):
            for d in range(d0, d0 + 4):
                m_v[pl.ds(S + (O * D + d * H) // 2, H // 2), _cols(t)] = _pack(t3_v[t % 2, pl.ds(d, H, stride=DH + 1), :])
        tasks = []
        for t in range(NT + 1):
            tasks += _merge([P(stage1, t, h) for h in range(0, H, 4) if t < NT],
                            [P(stage2, t - 1, d) for d in range(0, DH, 4) if t > 0])
        return _pad(tasks, 4)

    def fill_halo(s, t):
        f_v[pl.ds(_tile(s, t) - HALO, HALO), :] = jnp.broadcast_to(f_v[pl.ds(_tile(s, t), 1), :], (HALO, 128))

    def flush(j, r0, n):
        m_v[_rows((NA + j) * (TA // 2) + r0, n), :] = o_v[pl.ds(r0, n), :]

    def attention(i):
        WS, TS, LAG = CFG['WS'], CFG['TS'], CFG['LAG']
        first = isinstance(i, int)
        scale = DH ** -0.5

        def scores(parts, r0, ws):
            for t in range(NT):
                q = f_v[_rows(_tile(Q, t) + i * TA + r0, 16), :]
                for w in ws:
                    qk = q * f_v[pl.ds(_tile(K, t) + i * TA + r0 - DIL * w, 16), :]
                    parts[w] = qk if t == 0 else parts[w] + qk
            if len(parts) < W:
                return
            logits = []
            for w in range(W):
                l = parts[w] + pltpu.roll(parts[w], 64, 1)
                l = l + pltpu.roll(l, 32, 1)
                if first and r0 < DIL * w:
                    l = jnp.where(lax.broadcasted_iota(I32, l.shape, 0) + r0 >= DIL * w, l, -1e9 / scale)
                logits.append(l)
            top = functools.reduce(jnp.maximum, logits)
            e = [jnp.exp2((l - top) * (scale * np.log2(np.e))) for l in logits]
            inv = 1.0 / functools.reduce(jnp.add, e)
            for w in range(W):
                p_v[w, pl.ds(r0, 16), :] = e[w] * inv

        def mix(r0, ts):
            p = [p_v[w, pl.ds(r0, 16), :] for w in range(W)]
            for t in ts:
                o_v[pl.ds(r0 // 2, 8), _cols(t)] = _pack(functools.reduce(jnp.add, [
                    p[w] * f_v[pl.ds(_tile(V, t) + i * TA + r0 - DIL * w, 16), :] for w in range(W)]))
        tasks = []
        for r0 in range(0, TA + LAG, 16):
            a, b = [], []
            if r0 < TA:
                parts = {}
                a = [P(scores, parts, r0, range(w, w + WS)) for w in range(0, W, WS)]
            if r0 >= LAG:
                b = [P(mix, r0 - LAG, range(t, t + TS)) for t in range(0, NT, TS)]
            elif not first:
                n = TA // 4 * 16 // LAG
                b = [P(flush, i - 1, r0 // 8 * n + r, n) for r in (0, n)]
            tasks += _merge(a, b)
        return _pad(tasks, CFG['PAD'])

    def keys01(lo, hi):
        return sum((project(K, j, [t], True) for t in range(lo, hi) for j in (0, 1)), [])

    wait('x0')
    start('x1')
    run('n0', norm1(0, 1))
    wait('wk0')
    start('wk1')
    run('k0', project(K, 0, range(2), True))
    wait('x1')
    start('wk2')
    run('k0', norm1(1, 2) + project(K, 1, range(2), True))
    wait('wk1')
    start('wk3', 'x2')
    run('k0', keys01(2, 4))
    wait('wk2', 'wk3', 'x2')
    start('x3')
    run('k1', keys01(4, NT), reorder_cols(K), norm1(2, 3), _pad([P(start, 'wq')], 2, 1))
    wait('x3')
    run('k2', project(K, 2), reorder_keys(0), norm1(3, 5), [P(start, 'wv')])
    wait('wq')
    run('k3', project(K, 3), reorder_cols(Q), [P(fill_halo, K, t) for t in range(NT)], [P(start, 'x5')])
    wait('wv')
    start('wo')
    run('k4', project(K, 4), reorder_cols(V))
    wait('x5')
    run('v0', project(V, 0) + project(Q, 0), reorder_keys(1), norm1(5, NA),
        _pad([P(fill_halo, V, t) for t in range(NT)], 0, NT))
    wait('wo')
    for copy in ffn_copies(0):
        copy.start()
    run('step0', project(Q, 1) + project(V, 1) + project(K, 5), attention(0), reorder_rows())

    def step(i, _):
        for copy in ffn_copies(i - 1):
            copy.wait()
        for copy in ffn_copies(i):
            copy.start()
        last, late = i == NA - 1, i >= NA - 5
        run('step',
            project(jnp.where(last, O, Q), jnp.where(last, NA - 4, i + 1))
            + project(jnp.where(last, O, V), jnp.where(last, NA - 3, i + 1))
            + project(jnp.where(late, O, K), jnp.where(late, jnp.where(last, NA - 2, i + 5 - NA), i + 5)),
            attention(i), ffn_weights(0, i - 1))
    lax.fori_loop(1, NA, step, None)
    run('wo', [P(flush, NA - 1, 0, TA // 2)] + project(O, NA - 1), _pad(norm2(0), 2))

    def ffn(half, j):
        slots = [[] for _ in range(7 * (2 * NC + NT // 2) * CFG['FP'])]
        if half == 0:
            @pl.when(j < NC)
            def _():
                for copy in ffn_copies(NC + j):
                    copy.wait()

            @pl.when(j < NC - 1)
            def _():
                for copy in ffn_copies(NC + j + 1):
                    copy.start()
            norm, split = norm2(jnp.minimum(j + 1, NA - 1)), 7 * 2 * NC * CFG['FP']
            early = _merge(norm[:len(norm) // 2], ffn_weights(1, jnp.minimum(j, NC - 1)))
            for tasks, lo, hi in ((early, 0, split), (norm[len(norm) // 2:], split, len(slots) - 2)):
                for n, task in enumerate(tasks):
                    slots[lo + n * (hi - lo) // len(tasks)].append(task)

        def product(lhs, rhs):
            y = jnp.dot(pltpu.bitcast(lhs, BF16), pltpu.bitcast(rhs, BF16), preferred_element_type=F32)
            for t in range(y.shape[1] // 128):
                for r0 in range(0, TA // 2, TA // 2 // CFG['FP']):
                    tasks = slots.pop(0)
                    if tasks:
                        f_v[_rows(zero + H0 + NT * TA, 8), :] = y[r0:r0 + 8, _cols(t)]
                        pace(y[r0:r0 + 16, _cols(t)])
                    for task in tasks:
                        task()
            return y
        for c in range(NC):
            gu = _quadrants(lambda k: product(hn_v[j, k], wgu_v[half][c, k]))
            act = [jax.nn.gelu(y[:, :128], approximate=True) * y[:, 128:] for y in gu]
            for k, u in enumerate(_lhs_terms(*act)):
                a_v[k, :, _cols(c)] = _pack(u)
        for t in range(NT // 2):
            y = _quadrants(lambda k: product(a_v[k], wd_v[half][k, :, _cols(t)]))
            for n in (2, 1, 3, 0):
                r, tt = j * TA + n // 2 * (TA // 2), 2 * t + n % 2
                if half == 0:
                    f_v[_rows(_tile(Q, tt) + r, TA // 2), :] = y[n]
                else:
                    out_v[_rows(r, TA // 2), _cols(tt)] = (
                        hidden(r, TA // 2, [tt]) + (f_v[_rows(_tile(Q, tt) + r, TA // 2), :] + y[n])).astype(BF16)
            if half == 1:
                block = (_rows(j * TA, TA), pl.ds(t * 256, 256))
                pltpu.make_async_copy(out_v.at[block], out_hbm.at[block], sems.at[0]).start()
        assert not slots

    if not CFG['skipB']:
        for half in range(CFG['halves']):
            lax.fori_loop(0, NA, lambda j, _: _scope('ffn', P(ffn, half, j)), None)
        pltpu.make_async_copy(out_v, out_v, sems.at[0]).wait()


@jax.jit
def pallas_sequential_preLN__sliding_local_dilated__glu_gated_geglu__prompt_kernel(
        A_x, A_wqkv, A_wo, B_x, B_w_gate, B_w_up, B_w_down):
    del B_x
    in_hbm = pl.BlockSpec(memory_space=pl.ANY)
    vmem = pltpu.VMEM
    out = pl.pallas_call(
        _kernel,
        in_specs=[in_hbm] * 6,
        out_specs=in_hbm,
        out_shape=jax.ShapeDtypeStruct((S, D), BF16),
        scratch_shapes=[
            vmem((S + 3 * D + 16, D), BF16),
            vmem((D, D), BF16), [vmem((NC, 7, D // 4, FC), I32)] * 2, [vmem((7, DF // 8, D // 2), I32)] * 2,
            vmem((NT, D // 2 + 8, 128), I32), vmem((NT, D // 2, 128), I32), vmem((2, H * (DH + 1), 128), F32),
            vmem((S + 2 * D, D), I32),
            vmem((H0 + NT * TA + 8, 128), F32),
            vmem((W, TA, 128), F32), vmem((TA // 2, D), I32),
            vmem((NA, 7, TA // 4, D // 2), I32), vmem((7, TA // 4, DF // 4), I32),
            vmem((S, D), BF16), pltpu.SemaphoreType.DMA((3,)),
        ],
        compiler_params=pltpu.CompilerParams(vmem_limit_bytes=126 * 1024 * 1024, flags=CFG['flags'] or None,
                                             disable_bounds_checks=CFG['nobc']),
    )(A_x.reshape(S, D), A_wqkv, A_wo, B_w_gate, B_w_up, B_w_down)
    return out.reshape(A_x.shape)
```

```python
import functools

import jax
import jax.experimental.pallas as pl
import jax.experimental.pallas.tpu as pltpu
import jax.numpy as jnp
import numpy as np
from jax import lax

CFG = dict(passes=(0, 1, 2, 3), WE=196, PR=32, RP=32, WS=2, TS=2, LAG=32, PAD=2, LR=16, nest=0, fnest=0, nobc=True,
           skipP=0, skipB=False, scopes=False, flags={})

S, D, DF = 2048, 1024, 3584
H, DH, W, DIL = 32, 32, 8, 2
NT = D // 128
TA = 256
NA = S // TA
TF, NF = 512, S // 512
FC = 512
HALO = 16
KS = HALO + S
K, Q, V, O = 0, 1, 2, 3
H0 = 4 * NT * KS
KC = 256
F32, BF16, I32 = jnp.float32, jnp.bfloat16, jnp.int32
P = functools.partial


def _layernorm(x):
    xc = x - jnp.mean(x, axis=-1, keepdims=True)
    return xc * lax.rsqrt(jnp.mean(xc * xc, axis=-1, keepdims=True) + 1e-5)


def _pack(x):
    return pltpu.bitcast(x.astype(BF16), I32)


def _gather_tiles(tiles, sign):
    g = (lax.broadcasted_iota(I32, tiles[0].shape, 1) >> 2) & 7
    cur = [tiles[(sign * m) % NT] for m in range(NT)]
    for b in (1, 2, 4):
        cur = [jnp.where((g & b) != 0, cur[(m + sign * b) % NT], cur[m]) for m in range(NT)]
    return cur


def _shuffle_lanes(u, m):
    lane = lax.broadcasted_iota(I32, u.shape, 1)
    return jnp.take_along_axis(u, (lane & 3) * 32 + (((lane >> 2) - m) & 7) * 4 + (lane >> 5), axis=1)


LHS = ((0, 1, 3), (2, 1, 3), (0, 0, 0), (3, 0, 3), (0, 1, 1), (2, -1, 0), (1, -1, 3))
RHS = ((0, 1, 3), (0, 0, 0), (1, -1, 3), (2, -1, 0), (3, 0, 3), (0, 1, 1), (2, 1, 3))


def _term(rule, quadrant):
    a, sign, b = rule
    if sign == 0:
        return quadrant(a)
    x, y = quadrant(a).astype(F32), quadrant(b).astype(F32)
    return x + y if sign > 0 else x - y


def _terms(rules, *quadrants):
    return [_term(rule, quadrants.__getitem__) for rule in rules]


USES = (((0, 1), (3, 1)), ((2, 1), (3, -1)), ((1, 1), (3, 1)), ((0, 1), (2, 1)), ((1, 1), (0, -1)), ((3, 1),), ((0, 1),))
UP_ORDER = (0, 1, 3, 2, 4, 5, 6)
DOWN_ORDER = (3, 6, 1, 0, 2, 4, 5)


def _quadrants(product, order):
    acc = {}
    for n in order:
        m = product(n)
        for q, sign in USES[n]:
            if q not in acc:
                acc[q] = (sign, m)
            else:
                s, c = acc.pop(q)
                acc[q] = (1, c + m if s == sign else c - m if s > 0 else m - c)
    return {q: c for q, (_, c) in acc.items()}


def _inner_terms(rules, k, block):
    outer = [_term(rules[k], lambda q: block(q // 2 * 2 + i, q % 2 * 2 + j)) for i in (0, 1) for j in (0, 1)]
    return enumerate(_terms(rules, *outer), 7 * k)


class _Blocks(dict):
    __add__ = lambda a, b: _Blocks({q: a[q] + b[q] for q in a})
    __sub__ = lambda a, b: _Blocks({q: a[q] - b[q] for q in a})


def _sixteenths(product, order):
    c = _quadrants(lambda k: _Blocks(_quadrants(lambda n: product(7 * k + n), order)), order)
    return {(o // 2 * 2 + i // 2, o % 2 * 2 + i % 2): c[o][i] for o in c for i in c[o]}


def _merge(*lists):
    keyed = [((n + 0.5) / len(l), k, t) for k, l in enumerate(lists) for n, t in enumerate(l)]
    return [t for _, _, t in sorted(keyed, key=lambda e: e[:2])]


def _pad(tasks, n, front=0):
    return [lambda: None] * front + tasks + [lambda: None] * n


def _rows(r, n):
    return pl.ds(r if isinstance(r, int) else pl.multiple_of(r, min(n, 16)), n)


def _cols(t):
    return slice(t * 128, (t + 1) * 128)


def _tile(s, t):
    return (s * NT + t) * KS + HALO


def _scope(name, fn):
    if CFG['scopes']:
        with jax.named_scope('s_' + name):
            fn()
    else:
        fn()


def _kernel(x_hbm, wqkv_hbm, wo_hbm, wg_hbm, wu_hbm, wd_hbm, out_hbm,
            x_v,
            wk_v,
            wgu2_v, wd2_v,
            t1_v, t2_v, t3_v,
            m_v,
            f_v,
            p_v, o_v,
            a_v,
            sems):
    PR, RP, LR = CFG['PR'], CFG['RP'], CFG['LR']
    raw = {Q: S, V: S + D, O: S + 2 * D}

    blocks = lambda lo, hi: (x_hbm.at[pl.ds(lo * TA, (hi - lo) * TA)], x_v.at[pl.ds(lo * TA, (hi - lo) * TA)])
    wk = lambda c: (wqkv_hbm.at[:, pl.ds(D + c * KC, KC)], wk_v.at[:, pl.ds(c * KC, KC)])
    copies = {
        'x0': blocks(0, 1), 'wk0': wk(0), 'x1': blocks(1, 2), 'wk1': wk(1), 'wk2': wk(2), 'wk3': wk(3),
        'x2': blocks(2, 3), 'x3': blocks(3, 5),
        'wq': (wqkv_hbm.at[:, pl.ds(0, D)], x_v.at[pl.ds(raw[Q], D)]),
        'wv': (wqkv_hbm.at[:, pl.ds(2 * D, D)], x_v.at[pl.ds(raw[V], D)]),
        'x5': blocks(5, NA), 'wo': (wo_hbm, x_v.at[pl.ds(raw[O], D)])}
    copies = {name: pltpu.make_async_copy(*c, sems.at[n % 3]) for n, (name, c) in enumerate(copies.items())}

    def start(*names):
        for n in names:
            copies[n].start()

    def wait(*names):
        for n in names:
            _scope('w' + n, copies[n].wait)

    start('x0', 'wk0')
    zero = lax.while_loop(lambda c: c > 0, lambda c: c - 16, 16)

    def pace(y):
        x_v[_rows(zero + S + 3 * D, 16), 0:128] = y[:16, :128].astype(BF16)

    def run(name, *lists):
        def go():
            for task in _merge(*lists):
                task()
        if CFG['skipP'] and name != CFG['skipP']:
            return
        if CFG['nest'] == 1 or (CFG['nest'] == 2 and name == 'step'):
            pl.when(zero == 0)(lambda: _scope(name, go))
        else:
            _scope(name, go)

    def project(s, j, tiles=range(NT), as_given=False):
        held = {}
        lhs_row = ((s == O) * NA + j) * (TA // 2)
        w_row, y_row = S + s * (D // 2), _tile(s, 0) + j * TA

        def task(t, r0):
            if r0 == 0:
                lhs = pltpu.bitcast(m_v[_rows(lhs_row, TA // 2), :], BF16)
                if as_given:
                    w = wk_v[:, _cols(t)]
                else:
                    w = pltpu.bitcast(m_v[_rows(w_row, D // 2), _cols(t)], BF16)
                held['y'] = jnp.dot(lhs, w, preferred_element_type=F32)
            y = held['y'][r0:r0 + RP]
            r = y_row + (t * KS + r0)
            pace(y)
            if isinstance(s, int):
                r = r + zero
                if as_given:
                    t1_v[0, _rows(zero + D // 2, 8), :] = pltpu.bitcast(y[:8], I32)
            f_v[_rows(r, RP), :] = y
        return [P(task, t, r0) for t in tiles for r0 in range(0, TA, RP)]

    def norm1(lo, hi):
        def task(r0):
            m_v[pl.ds(r0 // 2, LR // 2), :] = _pack(_layernorm(x_v[pl.ds(r0, LR), :].astype(F32)))
        return _pad([P(task, r) for r in range(lo * TA, hi * TA, LR)], 2)

    def hidden(r0, n, cs=range(NT)):
        y = jnp.concatenate([f_v[_rows(_tile(O, t) + r0, n), :] for t in cs], axis=1)
        return x_v[_rows(r0, n), cs[0] * 128:(cs[-1] + 1) * 128].astype(F32) + y

    def norm_stats(stats, r0, n):
        def center(r):
            h = hidden(r0 + r, 16)
            for t in range(NT):
                f_v[pl.ds(H0 + t * TF + r, 16), :] = h[:, _cols(t)]
            stats[r] = jnp.mean(h, axis=-1, keepdims=True)

        def spread(r):
            hc = jnp.concatenate([f_v[pl.ds(H0 + t * TF + r, 16), :] for t in range(NT)], axis=1) - stats[r]
            stats[r] = (stats[r], lax.rsqrt(jnp.mean(hc * hc, axis=-1, keepdims=True) + 1e-5))
        return [P(f, r) for f in (center, spread) for r in range(0, n, 16)]

    def normed(stats, r, t):
        return (f_v[pl.ds(H0 + t * TF + r, 16), :] - stats[r][0]) * stats[r][1]

    def hn2(j, n):
        return j * (13 * TF // 8) + n // 4 * (TF // 8), n % 4 * 256

    def norm_rows(stats):
        def task(r):
            for t in range(NT):
                f_v[pl.ds(H0 + t * TF + r, 16), :] = normed(stats, r, t)
        return [P(task, r) for r in range(0, TF, 16)]

    def hn2_terms(j):
        def task(r0, t, k):
            for n, u in _inner_terms(LHS, k, lambda r, c: f_v[pl.ds(H0 + (2 * c + t) * TF + r * (TF // 4) + r0, 16), :]):
                row, col = hn2(j, n)
                m_v[_rows(row + r0 // 2, 8), pl.ds(col + t * 128, 128)] = _pack(u)
        return [P(task, r0, t, k) for r0 in range(0, TF // 4, 16) for t in range(2) for k in range(7)]

    def staged(c):
        return S + (c & 1) * (D + FC)

    def ffn_copies(c):
        r, f = staged(c), pl.ds(pl.multiple_of(c * FC, FC), FC)
        return [pltpu.make_async_copy(wg_hbm.at[:, f], x_v.at[_rows(r, D), pl.ds(0, FC)], sems.at[0]),
                pltpu.make_async_copy(wu_hbm.at[:, f], x_v.at[_rows(r, D), pl.ds(FC, FC)], sems.at[1]),
                pltpu.make_async_copy(wd_hbm.at[f], x_v.at[_rows(r + D, FC)], sems.at[2])]

    def weights2(p, c, part, parts):
        base = staged(c)

        def quad(r0, pitch, col, k):
            return _inner_terms(RHS, k, lambda r, c: x_v[
                _rows(base + r0 + r * pitch, 16), pl.ds(col + c // 2 * 256, 256)][:, _cols(c % 2)])

        def gate_up(r0, m, k):
            for n, u in quad(r0, D // 4, m * FC, k):
                wgu2_v[p % 2][c, n, _rows(r0 // 2, 8), _cols(m)] = _pack(u)

        def down(r0, t, k):
            for n, u in quad(D + r0, FC // 4, t * 512, k):
                wd2_v[p % 2][n, _rows(c * 64 + r0 // 2, 8), _cols(t)] = _pack(u)
        def down1(r0, i, t):
            top, bot = (x_v[_rows(base + D + (2 * h + i) * 128 + r0, 16), t * 128:t * 128 + 640] for h in (0, 1))
            for k, u in enumerate(_terms(RHS, top[:, :128], top[:, 512:], bot[:, :128], bot[:, 512:])):
                wd2_v[p % 2][2 * k + t // 2, _rows(i * 64 + r0 // 2, 8), _cols(t % 2)] = _pack(u)
        n = D // 4 // parts
        if p == 3:
            return ([P(gate_up, part * n + r, m, k) for r in range(0, n, 16) for m in (0, 1) for k in range(7)]
                    + [P(down1, part * (n // 2) + r, i, t) for r in range(0, n // 2, 16) for i in (0, 1) for t in range(4)])
        return ([P(gate_up, part * n + r, m, k) for r in range(0, n, 16) for m in (0, 1) for k in range(7)]
                + [P(down, part * (n // 2) + r, t, k) for r in range(0, n // 2, 16) for t in (0, 1) for k in range(7)])

    def reorder_cols(s):
        def stage1(r0):
            src = (lambda t: wk_v[pl.ds(2 * r0, 16), _cols(t)]) if s == K else (
                lambda t: x_v[pl.ds(raw[s] + 2 * r0, 16), _cols(t)])
            for m, u in enumerate(_gather_tiles([pltpu.bitcast(src(t), I32) for t in range(NT)], 1)):
                t1_v[m, _rows(zero + r0, 8), :] = u

        def stage2(r0, m):
            t2_v[m, _rows(zero + r0, PR), :] = _shuffle_lanes(t1_v[m, pl.ds(r0, PR), :], m)

        def stage3(r0):
            for t, u in enumerate(_gather_tiles([t2_v[m, pl.ds(r0, 8), :] for m in range(NT)], -1)):
                m_v[pl.ds(S + s * (D // 2) + r0, 8), _cols(t)] = u
        tasks = []
        for r0 in range(0, D // 2 + 2 * PR, PR):
            tasks += _merge([P(stage1, r) for r in range(r0, r0 + PR, 8) if r < D // 2],
                            [P(stage2, r0 - PR, m) for m in range(NT) if 0 <= r0 - PR < D // 2],
                            [P(stage3, r - 2 * PR) for r in range(r0, r0 + PR, 8) if r >= 2 * PR])
        return _pad(tasks, 4 * 64 // PR)

    def reorder_keys(j):
        held = []

        def task(r0):
            if held:
                lo, tiles = held.pop()
                for t, u in enumerate(tiles):
                    f_v[pl.ds(_tile(K, t) + lo, 8), :] = u
            if r0 < (j + 1) * TA:
                tiles = _gather_tiles([f_v[pl.ds(_tile(K, t) + r0, 8), :] for t in range(NT)], 1)
                held.append((r0, _gather_tiles([_shuffle_lanes(u, m) for m, u in enumerate(tiles)], -1)))
        return [P(task, r) for r in range(j * TA, (j + 1) * TA + 8, 8)]

    def reorder_rows():
        def stage1(t, h0):
            for h in range(h0, h0 + 4):
                t3_v[t % 2, pl.ds(zero + h * (DH + 1), DH), :] = x_v[pl.ds(raw[O] + h * DH, DH), _cols(t)].astype(F32)

        def stage2(t, d0):
            for d in range(d0, d0 + 4):
                m_v[pl.ds(S + (O * D + d * H) // 2, H // 2), _cols(t)] = _pack(t3_v[t % 2, pl.ds(d, H, stride=DH + 1), :])
        tasks = []
        for t in range(NT + 1):
            tasks += _merge([P(stage1, t, h) for h in range(0, H, 4) if t < NT],
                            [P(stage2, t - 1, d) for d in range(0, DH, 4) if t > 0])
        return _pad(tasks, 4)

    def fill_halo(s, t):
        f_v[pl.ds(_tile(s, t) - HALO, HALO), :] = jnp.broadcast_to(f_v[pl.ds(_tile(s, t), 1), :], (HALO, 128))

    def flush(j, r0, n):
        m_v[_rows((NA + j) * (TA // 2) + r0, n), :] = o_v[pl.ds(r0, n), :]

    def attention(i):
        WS, TS, LAG = CFG['WS'], CFG['TS'], CFG['LAG']
        first = isinstance(i, int)
        scale = DH ** -0.5

        def scores(parts, r0, ws):
            for t in range(NT):
                q = f_v[_rows(_tile(Q, t) + i * TA + r0, 16), :]
                for w in ws:
                    qk = q * f_v[pl.ds(_tile(K, t) + i * TA + r0 - DIL * w, 16), :]
                    parts[w] = qk if t == 0 else parts[w] + qk
            if len(parts) < W:
                return
            logits = []
            for w in range(W):
                l = parts[w] + pltpu.roll(parts[w], 64, 1)
                l = l + pltpu.roll(l, 32, 1)
                if first and r0 < DIL * w:
                    l = jnp.where(lax.broadcasted_iota(I32, l.shape, 0) + r0 >= DIL * w, l, -1e9 / scale)
                logits.append(l)
            top = functools.reduce(jnp.maximum, logits)
            e = [jnp.exp2((l - top) * (scale * np.log2(np.e))) for l in logits]
            inv = 1.0 / functools.reduce(jnp.add, e)
            for w in range(W):
                p_v[w, pl.ds(r0, 16), :] = e[w] * inv

        def mix(r0, ts):
            p = [p_v[w, pl.ds(r0, 16), :] for w in range(W)]
            for t in ts:
                o_v[pl.ds(r0 // 2, 8), _cols(t)] = _pack(functools.reduce(jnp.add, [
                    p[w] * f_v[pl.ds(_tile(V, t) + i * TA + r0 - DIL * w, 16), :] for w in range(W)]))
        tasks = []
        for r0 in range(0, TA + LAG, 16):
            a, b = [], []
            if r0 < TA:
                parts = {}
                a = [P(scores, parts, r0, range(w, w + WS)) for w in range(0, W, WS)]
            if r0 >= LAG:
                b = [P(mix, r0 - LAG, range(t, t + TS)) for t in range(0, NT, TS)]
            elif not first:
                n = TA // 4 * 16 // LAG
                b = [P(flush, i - 1, r0 // 8 * n + r, n) for r in (0, n)]
            tasks += _merge(a, b)
        return _pad(tasks, CFG['PAD'])

    def keys01(lo, hi):
        return sum((project(K, j, [t], True) for t in range(lo, hi) for j in (0, 1)), [])

    wait('x0')
    start('x1')
    run('n0', norm1(0, 1))
    wait('wk0')
    start('wk1')
    run('k0', project(K, 0, range(2), True))
    wait('x1')
    start('wk2')
    run('k0', norm1(1, 2) + project(K, 1, range(2), True))
    wait('wk1')
    start('wk3', 'x2')
    run('k0', keys01(2, 4))
    wait('wk2', 'wk3', 'x2')
    start('x3')
    run('k1', keys01(4, NT), reorder_cols(K), norm1(2, 3), _pad([P(start, 'wq')], 2, 1))
    wait('x3')
    run('k2', project(K, 2), reorder_keys(0), norm1(3, 5), [P(start, 'wv')])
    wait('wq')
    run('k3', project(K, 3), reorder_cols(Q), [P(fill_halo, K, t) for t in range(NT)], [P(start, 'x5')])
    wait('wv')
    start('wo')
    run('k4', project(K, 4), reorder_cols(V))
    wait('x5')
    run('v0', project(V, 0) + project(Q, 0), reorder_keys(1), norm1(5, NA),
        _pad([P(fill_halo, V, t) for t in range(NT)], 0, NT))
    wait('wo')
    for copy in ffn_copies(0):
        copy.start()
    run('step0', project(Q, 1) + project(V, 1) + project(K, 5), attention(0), reorder_rows())


    def next_chunk(c, when):
        @pl.when(when)
        def _():
            for copy in ffn_copies(c):
                copy.wait()

            @pl.when(c < DF // FC - 1)
            def _():
                for copy in ffn_copies(c + 1):
                    copy.start()

    def step(i, _):
        last, late, n = i == NA - 1, i >= NA - 5, i - 1
        next_chunk(n >> 2, (n & 3) == 0)
        run('step',
            project(jnp.where(last, O, Q), jnp.where(last, NA - 4, i + 1))
            + project(jnp.where(last, O, V), jnp.where(last, NA - 3, i + 1))
            + project(jnp.where(late, O, K), jnp.where(late, jnp.where(last, NA - 2, i + 5 - NA), i + 5)),
            attention(i), _pad(weights2(0, n >> 2, n & 3, 4), 2))
    lax.fori_loop(1, NA, step, None)
    stats = {}
    run('wo', [P(flush, NA - 1, 0, TA // 2)] + project(O, NA - 1), _pad(weights2(0, 1, 3, 4), 2),
        norm_stats(stats, 0, TF) + norm_rows(stats) + hn2_terms(0))

    def paced(n_tiles, *spans):
        slots = [[] for _ in range(n_tiles)]
        for tasks, lo, hi in spans:
            for n, task in enumerate(tasks):
                slots[lo + n * (hi - lo) // len(tasks)].append(task)

        def product(lhs, rhs):
            y = jnp.dot(pltpu.bitcast(lhs, BF16), pltpu.bitcast(rhs, BF16), preferred_element_type=F32)
            for t in range(y.shape[1] // 128):
                tasks = slots.pop(0)
                if tasks:
                    f_v[_rows(zero + H0 + NT * TF, 8), :] = y[:8, _cols(t)]
                    pace(y[:16, _cols(t)])
                for task in tasks:
                    task()
            return y
        return product

    def ffn(p, j):
        spans = []
        if p < 2:
            next_chunk(2 * p + 2 + (j >> 1), (j & 1) == 0)
            spans.append((weights2(p + 1, j >> 1, j & 1, 2), 0, CFG['WE']))
        if p == 2:
            next_chunk(2 * p + 2 + zero, j == 0)
            spans.append((weights2(p + 1, 0, j, NF), 0, CFG['WE']))
        if p == 0:
            stats, nxt = {}, jnp.minimum(j + 1, NF - 1)
            spans += [(norm_stats(stats, nxt * TF, TF) + norm_rows(stats), 0, 196), (hn2_terms(nxt), 196, 290)]
        product = paced(294, *spans)

        def lhs(n):
            row, col = hn2(j, n)
            return m_v[_rows(row, TF // 8), pl.ds(col, 256)]

        def activations(c):
            y = _sixteenths(lambda n: product(lhs(n), wgu2_v[p % 2][c, n]), UP_ORDER)
            return {rc: jax.nn.gelu(gu[:, :128], approximate=True) * gu[:, 128:] for rc, gu in y.items()}
        if p < 3:
            for c in range(2):
                act = activations(c)
                for k in DOWN_ORDER:
                    for n, u in _inner_terms(LHS, k, lambda r, c: act[r, c]):
                        a_v[n, :, _cols(c)] = _pack(u)
            for (r, c), y in _sixteenths(lambda n: product(a_v[n], wd2_v[p % 2][n]), DOWN_ORDER).items():
                for i in range(2):
                    rows = _rows(_tile(Q, 4 * i + c) + j * TF + r * (TF // 4), TF // 4)
                    f_v[rows, :] = f_v[rows, :] + y[:, _cols(i)] if p else y[:, _cols(i)]
            return
        act = activations(0)
        for k in DOWN_ORDER:
            for i in range(2):
                for c in range(2):
                    a_v[2 * k + i, :, _cols(c)] = _pack(_term(LHS[k], lambda q: act[q // 2 * 2 + i, q % 2 * 2 + c]))
        for i in range(2):
            for c in range(2):
                y = _quadrants(lambda k: product(a_v[2 * k + i], wd2_v[p % 2][2 * k + c]), DOWN_ORDER)
                for q in y:
                    r, t = j * TF + (q // 2 * 2 + i) * (TF // 4), q % 2 * 4 + c * 2
                    acc = jnp.concatenate([f_v[_rows(_tile(Q, t + n) + r, TF // 4), :] for n in (0, 1)], axis=1)
                    block = (_rows(r, TF // 4), pl.ds(t * 128, 256))
                    x_v[block] = (hidden(r, TF // 4, [t, t + 1]) + (acc + y[q])).astype(BF16)
                    pltpu.make_async_copy(x_v.at[block], out_hbm.at[block], sems.at[0]).start()

    for p in CFG['passes']:
        lax.fori_loop(0, NF, lambda j, _: _scope('ffn', P(ffn, p, j)), None)
    pltpu.make_async_copy(x_v.at[pl.ds(0, S)], x_v.at[pl.ds(0, S)], sems.at[0]).wait()


@jax.jit
def pallas_sequential_preLN__sliding_local_dilated__glu_gated_geglu__prompt_kernel(
        A_x, A_wqkv, A_wo, B_x, B_w_gate, B_w_up, B_w_down):
    del B_x
    in_hbm = pl.BlockSpec(memory_space=pl.ANY)
    vmem = pltpu.VMEM
    out = pl.pallas_call(
        _kernel,
        in_specs=[in_hbm] * 6,
        out_specs=in_hbm,
        out_shape=jax.ShapeDtypeStruct((S, D), BF16),
        scratch_shapes=[
            vmem((S + 3 * D + 16, D), BF16),
            vmem((D, D), BF16), [vmem((2, 49, D // 8, 256), I32)] * 2, [vmem((49, FC // 4, 256), I32)] * 2,
            vmem((NT, D // 2 + 8, 128), I32), vmem((NT, D // 2, 128), I32), vmem((2, H * (DH + 1), 128), F32),
            vmem((S + 2 * D, D), I32),
            vmem((H0 + NT * TF + 8, 128), F32),
            vmem((W, TA, 128), F32), vmem((TA // 2, D), I32),
            vmem((49, TF // 8, 256), I32),
            pltpu.SemaphoreType.DMA((3,)),
        ],
        compiler_params=pltpu.CompilerParams(vmem_limit_bytes=126 * 1024 * 1024, flags=CFG['flags'] or None,
                                             disable_bounds_checks=CFG['nobc']),
    )(A_x.reshape(S, D), A_wqkv, A_wo, B_w_gate, B_w_up, B_w_down)
    return out.reshape(A_x.shape)
```

```python
import functools

import jax
import jax.experimental.pallas as pl
import jax.experimental.pallas.tpu as pltpu
import jax.numpy as jnp
import numpy as np
from jax import lax

CFG = dict(passes=(0, 1, 2, 3), NS=3, UP=((0, 98),), DN=(196, 284), WD=2, WD0=2, PP=16, PR=32, RP=32, WS=2, TS=2, LAG=32, PAD=2, LR=16, nest=0, fnest=0, nobc=True,
           skipP=0, skipB=False, scopes=False, flags={})

S, D, DF = 2048, 1024, 3584
H, DH, W, DIL = 32, 32, 8, 2
NT = D // 128
TA = 256
NA = S // TA
TF, NF = 512, S // 512
FC = 512
HALO = 16
KS = HALO + S
K, Q, V, O = 0, 1, 2, 3
H0 = 4 * NT * KS
KC = 256
F32, BF16, I32 = jnp.float32, jnp.bfloat16, jnp.int32
P = functools.partial


def _layernorm(x):
    xc = x - jnp.mean(x, axis=-1, keepdims=True)
    return xc * lax.rsqrt(jnp.mean(xc * xc, axis=-1, keepdims=True) + 1e-5)


def _pack(x):
    return pltpu.bitcast(x.astype(BF16), I32)


def _gather_tiles(tiles, sign):
    g = (lax.broadcasted_iota(I32, tiles[0].shape, 1) >> 2) & 7
    cur = [tiles[(sign * m) % NT] for m in range(NT)]
    for b in (1, 2, 4):
        cur = [jnp.where((g & b) != 0, cur[(m + sign * b) % NT], cur[m]) for m in range(NT)]
    return cur


def _shuffle_lanes(u, m):
    lane = lax.broadcasted_iota(I32, u.shape, 1)
    return jnp.take_along_axis(u, (lane & 3) * 32 + (((lane >> 2) - m) & 7) * 4 + (lane >> 5), axis=1)


LHS = ((0, 1, 3), (2, 1, 3), (0, 0, 0), (3, 0, 3), (0, 1, 1), (2, -1, 0), (1, -1, 3))
RHS = ((0, 1, 3), (0, 0, 0), (1, -1, 3), (2, -1, 0), (3, 0, 3), (0, 1, 1), (2, 1, 3))


def _term(rule, quadrant):
    a, sign, b = rule
    if sign == 0:
        return quadrant(a)
    x, y = quadrant(a).astype(F32), quadrant(b).astype(F32)
    return x + y if sign > 0 else x - y


def _terms(rules, *quadrants):
    return [_term(rule, quadrants.__getitem__) for rule in rules]


USES = (((0, 1), (3, 1)), ((2, 1), (3, -1)), ((1, 1), (3, 1)), ((0, 1), (2, 1)), ((1, 1), (0, -1)), ((3, 1),), ((0, 1),))
UP_ORDER = (0, 1, 3, 2, 4, 5, 6)
DOWN_ORDER = (3, 6, 1, 0, 2, 4, 5)


def _quadrants(product, order):
    acc = {}
    for n in order:
        m = product(n)
        for q, sign in USES[n]:
            if q not in acc:
                acc[q] = (sign, m)
            else:
                s, c = acc.pop(q)
                acc[q] = (1, c + m if s == sign else c - m if s > 0 else m - c)
    return {q: c for q, (_, c) in acc.items()}


def _inner_terms(rules, k, block):
    outer = [_term(rules[k], lambda q: block(q // 2 * 2 + i, q % 2 * 2 + j)) for i in (0, 1) for j in (0, 1)]
    return enumerate(_terms(rules, *outer), 7 * k)


class _Blocks(dict):
    __add__ = lambda a, b: _Blocks({q: a[q] + b[q] for q in a})
    __sub__ = lambda a, b: _Blocks({q: a[q] - b[q] for q in a})


def _sixteenths(product, order):
    c = _quadrants(lambda k: _Blocks(_quadrants(lambda n: product(7 * k + n), order)), order)
    return {(o // 2 * 2 + i // 2, o % 2 * 2 + i % 2): c[o][i] for o in c for i in c[o]}


def _merge(*lists):
    keyed = [((n + 0.5) / len(l), k, t) for k, l in enumerate(lists) for n, t in enumerate(l)]
    return [t for _, _, t in sorted(keyed, key=lambda e: e[:2])]


def _pad(tasks, n, front=0):
    return [lambda: None] * front + tasks + [lambda: None] * n


def _rows(r, n):
    return pl.ds(r if isinstance(r, int) else pl.multiple_of(r, min(n, 16)), n)


def _cols(t):
    return slice(t * 128, (t + 1) * 128)


def _tile(s, t):
    return (s * NT + t) * KS + HALO


def _scope(name, fn):
    if CFG['scopes']:
        with jax.named_scope('s_' + name):
            fn()
    else:
        fn()


def _kernel(x_hbm, wqkv_hbm, wo_hbm, wg_hbm, wu_hbm, wd_hbm, out_hbm,
            x_v,
            wk_v,
            wgu2_v, wd2_v,
            t1_v, t2_v, t3_v,
            m_v,
            f_v,
            p_v, o_v,
            a_v,
            sems):
    PR, RP, LR = CFG['PR'], CFG['RP'], CFG['LR']
    raw = {Q: S, V: S + D, O: S + 2 * D}

    blocks = lambda lo, hi: (x_hbm.at[pl.ds(lo * TA, (hi - lo) * TA)], x_v.at[pl.ds(lo * TA, (hi - lo) * TA)])
    wk = lambda c: (wqkv_hbm.at[:, pl.ds(D + c * KC, KC)], wk_v.at[:, pl.ds(c * KC, KC)])
    copies = {
        'x0': blocks(0, 1), 'wk0': wk(0), 'x1': blocks(1, 2), 'wk1': wk(1), 'wk2': wk(2), 'wk3': wk(3),
        'x2': blocks(2, 3), 'x3': blocks(3, 5),
        'wq': (wqkv_hbm.at[:, pl.ds(0, D)], x_v.at[pl.ds(raw[Q], D)]),
        'wv': (wqkv_hbm.at[:, pl.ds(2 * D, D)], x_v.at[pl.ds(raw[V], D)]),
        'x5': blocks(5, NA), 'wo': (wo_hbm, x_v.at[pl.ds(raw[O], D)])}
    copies = {name: pltpu.make_async_copy(*c, sems.at[n % 3]) for n, (name, c) in enumerate(copies.items())}

    def start(*names):
        for n in names:
            copies[n].start()

    def wait(*names):
        for n in names:
            _scope('w' + n, copies[n].wait)

    start('x0', 'wk0')
    zero = lax.while_loop(lambda c: c > 0, lambda c: c - 16, 16)

    def pace(y):
        x_v[_rows(zero + S + 3 * D, 16), 0:128] = y[:16, :128].astype(BF16)

    def run(name, *lists):
        def go():
            for task in _merge(*lists):
                task()
        if CFG['skipP'] and name != CFG['skipP']:
            return
        if CFG['nest'] == 1 or (CFG['nest'] == 2 and name == 'step'):
            pl.when(zero == 0)(lambda: _scope(name, go))
        else:
            _scope(name, go)

    def project(s, j, tiles=range(NT), as_given=False):
        held = {}
        lhs_row = ((s == O) * NA + j) * (TA // 2)
        w_row, y_row = S + s * (D // 2), _tile(s, 0) + j * TA

        def task(t, r0):
            if r0 == 0:
                lhs = pltpu.bitcast(m_v[_rows(lhs_row, TA // 2), :], BF16)
                if as_given:
                    w = wk_v[:, _cols(t)]
                else:
                    w = pltpu.bitcast(m_v[_rows(w_row, D // 2), _cols(t)], BF16)
                held['y'] = jnp.dot(lhs, w, preferred_element_type=F32)
            y = held['y'][r0:r0 + RP]
            r = y_row + (t * KS + r0)
            pace(y)
            if isinstance(s, int):
                r = r + zero
                if as_given:
                    t1_v[0, _rows(zero + D // 2, 8), :] = pltpu.bitcast(y[:8], I32)
            f_v[_rows(r, RP), :] = y
        return [P(task, t, r0) for t in tiles for r0 in range(0, TA, RP)]

    def norm1(lo, hi):
        def task(r0):
            m_v[pl.ds(r0 // 2, LR // 2), :] = _pack(_layernorm(x_v[pl.ds(r0, LR), :].astype(F32)))
        return _pad([P(task, r) for r in range(lo * TA, hi * TA, LR)], 2)

    def hidden(r0, n, cs=range(NT)):
        y = jnp.concatenate([f_v[_rows(_tile(O, t) + r0, n), :] for t in cs], axis=1)
        return x_v[_rows(r0, n), cs[0] * 128:(cs[-1] + 1) * 128].astype(F32) + y

    def norm_stats(stats, r0, n):
        def center(r):
            h = hidden(r0 + r, 16)
            for t in range(NT):
                f_v[pl.ds(H0 + t * TF + r, 16), :] = h[:, _cols(t)]
            stats[r] = jnp.mean(h, axis=-1, keepdims=True)

        def spread(r):
            hc = jnp.concatenate([f_v[pl.ds(H0 + t * TF + r, 16), :] for t in range(NT)], axis=1) - stats[r]
            stats[r] = (stats[r], lax.rsqrt(jnp.mean(hc * hc, axis=-1, keepdims=True) + 1e-5))
        return [P(f, r) for f in (center, spread) for r in range(0, n, 16)]

    def normed(stats, r, t):
        return (f_v[pl.ds(H0 + t * TF + r, 16), :] - stats[r][0]) * stats[r][1]

    def hn2(j, n):
        return j * (13 * TF // 8) + n // 4 * (TF // 8), n % 4 * 256

    def norm_rows(stats):
        def task(r):
            for t in range(NT):
                f_v[pl.ds(H0 + t * TF + r, 16), :] = normed(stats, r, t)
        return [P(task, r) for r in range(0, TF, 16)]

    def hn2_terms(j):
        def task(r0, t, k):
            for n, u in _inner_terms(LHS, k, lambda r, c: f_v[pl.ds(H0 + (2 * c + t) * TF + r * (TF // 4) + r0, 16), :]):
                row, col = hn2(j, n)
                m_v[_rows(row + r0 // 2, 8), pl.ds(col + t * 128, 128)] = _pack(u)
        return [P(task, r0, t, k) for r0 in range(0, TF // 4, 16) for t in range(2) for k in range(7)]

    def staged(c):
        return S + (c & 1) * (D + FC)

    def ffn_copies(c):
        r, f = staged(c), pl.ds(pl.multiple_of(c * FC, FC), FC)
        return [pltpu.make_async_copy(wg_hbm.at[:, f], x_v.at[_rows(r, D), pl.ds(0, FC)], sems.at[0]),
                pltpu.make_async_copy(wu_hbm.at[:, f], x_v.at[_rows(r, D), pl.ds(FC, FC)], sems.at[1]),
                pltpu.make_async_copy(wd_hbm.at[f], x_v.at[_rows(r + D, FC)], sems.at[2])]

    def weights2(p, c, part, parts):
        base = staged(c)

        def quad(r0, pitch, col, k):
            return _inner_terms(RHS, k, lambda r, c: x_v[
                _rows(base + r0 + r * pitch, 16), pl.ds(col + c // 2 * 256, 256)][:, _cols(c % 2)])

        def gate_up(r0, m, k):
            for n, u in quad(r0, D // 4, m * FC, k):
                wgu2_v[p % 2][c, n, _rows(r0 // 2, 8), _cols(m)] = _pack(u)

        def down(r0, t, k):
            for n, u in quad(D + r0, FC // 4, t * 512, k):
                wd2_v[p % 2][n, _rows(c * 64 + r0 // 2, 8), _cols(t)] = _pack(u)
        def down1(r0, i, t):
            top, bot = (x_v[_rows(base + D + (2 * h + i) * 128 + r0, 16), t * 128:t * 128 + 640] for h in (0, 1))
            for k, u in enumerate(_terms(RHS, top[:, :128], top[:, 512:], bot[:, :128], bot[:, 512:])):
                wd2_v[p % 2][2 * k + t // 2, _rows(i * 64 + r0 // 2, 8), _cols(t % 2)] = _pack(u)
        n = D // 4 // parts
        if p == 3:
            return ([P(gate_up, part * n + r, m, k) for r in range(0, n, 16) for m in (0, 1) for k in range(7)]
                    + [P(down1, part * (n // 2) + r, i, t) for r in range(0, n // 2, 16) for i in (0, 1) for t in range(4)])
        return ([P(gate_up, part * n + r, m, k) for r in range(0, n, 16) for m in (0, 1) for k in range(7)]
                + [P(down, part * (n // 2) + r, t, k) for r in range(0, n // 2, 16) for t in (0, 1) for k in range(7)])

    def reorder_cols(s):
        def stage1(r0):
            src = (lambda t: wk_v[pl.ds(2 * r0, 16), _cols(t)]) if s == K else (
                lambda t: x_v[pl.ds(raw[s] + 2 * r0, 16), _cols(t)])
            for m, u in enumerate(_gather_tiles([pltpu.bitcast(src(t), I32) for t in range(NT)], 1)):
                t1_v[m, _rows(zero + r0, 8), :] = u

        def stage2(r0, m):
            t2_v[m, _rows(zero + r0, PR), :] = _shuffle_lanes(t1_v[m, pl.ds(r0, PR), :], m)

        def stage3(r0):
            for t, u in enumerate(_gather_tiles([t2_v[m, pl.ds(r0, 8), :] for m in range(NT)], -1)):
                m_v[pl.ds(S + s * (D // 2) + r0, 8), _cols(t)] = u
        tasks = []
        for r0 in range(0, D // 2 + 2 * PR, PR):
            tasks += _merge([P(stage1, r) for r in range(r0, r0 + PR, 8) if r < D // 2],
                            [P(stage2, r0 - PR, m) for m in range(NT) if 0 <= r0 - PR < D // 2],
                            [P(stage3, r - 2 * PR) for r in range(r0, r0 + PR, 8) if r >= 2 * PR])
        return _pad(tasks, CFG['PP'])

    def reorder_keys(j):
        held = []

        def task(r0):
            if held:
                lo, tiles = held.pop()
                for t, u in enumerate(tiles):
                    f_v[pl.ds(_tile(K, t) + lo, 8), :] = u
            if r0 < (j + 1) * TA:
                tiles = _gather_tiles([f_v[pl.ds(_tile(K, t) + r0, 8), :] for t in range(NT)], 1)
                held.append((r0, _gather_tiles([_shuffle_lanes(u, m) for m, u in enumerate(tiles)], -1)))
        return [P(task, r) for r in range(j * TA, (j + 1) * TA + 8, 8)]

    def reorder_rows():
        def stage1(t, h0):
            for h in range(h0, h0 + 4):
                t3_v[t % 2, pl.ds(zero + h * (DH + 1), DH), :] = x_v[pl.ds(raw[O] + h * DH, DH), _cols(t)].astype(F32)

        def stage2(t, d0):
            for d in range(d0, d0 + 4):
                m_v[pl.ds(S + (O * D + d * H) // 2, H // 2), _cols(t)] = _pack(t3_v[t % 2, pl.ds(d, H, stride=DH + 1), :])
        tasks = []
        for t in range(NT + 1):
            tasks += _merge([P(stage1, t, h) for h in range(0, H, 4) if t < NT],
                            [P(stage2, t - 1, d) for d in range(0, DH, 4) if t > 0])
        return _pad(tasks, 4)

    def fill_halo(s, t):
        f_v[pl.ds(_tile(s, t) - HALO, HALO), :] = jnp.broadcast_to(f_v[pl.ds(_tile(s, t), 1), :], (HALO, 128))

    def flush(j, r0, n):
        m_v[_rows((NA + j) * (TA // 2) + r0, n), :] = o_v[pl.ds(r0, n), :]

    def attention(i):
        WS, TS, LAG = CFG['WS'], CFG['TS'], CFG['LAG']
        first = isinstance(i, int)
        scale = DH ** -0.5

        def scores(parts, r0, ws):
            for t in range(NT):
                q = f_v[_rows(_tile(Q, t) + i * TA + r0, 16), :]
                for w in ws:
                    qk = q * f_v[pl.ds(_tile(K, t) + i * TA + r0 - DIL * w, 16), :]
                    parts[w] = qk if t == 0 else parts[w] + qk
            if len(parts) < W:
                return
            logits = []
            for w in range(W):
                l = parts[w] + pltpu.roll(parts[w], 64, 1)
                l = l + pltpu.roll(l, 32, 1)
                if first and r0 < DIL * w:
                    l = jnp.where(lax.broadcasted_iota(I32, l.shape, 0) + r0 >= DIL * w, l, -1e9 / scale)
                logits.append(l)
            top = functools.reduce(jnp.maximum, logits)
            e = [jnp.exp2((l - top) * (scale * np.log2(np.e))) for l in logits]
            inv = 1.0 / functools.reduce(jnp.add, e)
            for w in range(W):
                p_v[w, pl.ds(r0, 16), :] = e[w] * inv

        def mix(r0, ts):
            p = [p_v[w, pl.ds(r0, 16), :] for w in range(W)]
            for t in ts:
                o_v[pl.ds(r0 // 2, 8), _cols(t)] = _pack(functools.reduce(jnp.add, [
                    p[w] * f_v[pl.ds(_tile(V, t) + i * TA + r0 - DIL * w, 16), :] for w in range(W)]))
        tasks = []
        for r0 in range(0, TA + LAG, 16):
            a, b = [], []
            if r0 < TA:
                parts = {}
                a = [P(scores, parts, r0, range(w, w + WS)) for w in range(0, W, WS)]
            if r0 >= LAG:
                b = [P(mix, r0 - LAG, range(t, t + TS)) for t in range(0, NT, TS)]
            elif not first:
                n = TA // 4 * 16 // LAG
                b = [P(flush, i - 1, r0 // 8 * n + r, n) for r in (0, n)]
            tasks += _merge(a, b)
        return _pad(tasks, CFG['PAD'])

    def keys01(lo, hi):
        return sum((project(K, j, [t], True) for t in range(lo, hi) for j in (0, 1)), [])

    wait('x0')
    start('x1')
    run('n0', norm1(0, 1))
    wait('wk0')
    start('wk1')
    run('k0', project(K, 0, range(2), True))
    wait('x1')
    start('wk2')
    run('k0', norm1(1, 2) + project(K, 1, range(2), True))
    wait('wk1')
    start('wk3', 'x2')
    run('k0', keys01(2, 4))
    wait('wk2', 'wk3')
    start('x3')
    run('k1', keys01(4, NT), reorder_cols(K), _pad([P(start, 'wq')], 1, 1))
    wait('x2', 'x3')
    run('k2', norm1(2, 3) + project(K, 2), _pad(reorder_keys(0), 2, 12), _pad(norm1(3, 5), 0, 12), [P(start, 'wv')])
    wait('wq')
    run('k3', project(K, 3), reorder_cols(Q), [P(fill_halo, K, t) for t in range(NT)], [P(start, 'x5')])
    wait('wv')
    start('wo')
    run('k4', project(K, 4), reorder_cols(V))
    wait('x5')
    run('v0', project(V, 0) + project(Q, 0), reorder_keys(1), norm1(5, NA),
        _pad([P(fill_halo, V, t) for t in range(NT)], 0, NT))
    wait('wo')
    for copy in ffn_copies(0):
        copy.start()
    run('step0', project(Q, 1) + project(V, 1) + project(K, 5), attention(0), reorder_rows())


    def next_chunk(c, when):
        @pl.when(when)
        def _():
            for copy in ffn_copies(c):
                copy.wait()

            @pl.when(c < DF // FC - 1)
            def _():
                for copy in ffn_copies(c + 1):
                    copy.start()

    def step(i, _):
        last, late, n = i == NA - 1, i >= NA - 5, i - 1
        next_chunk(n >> 2, (n & 3) == 0)
        run('step',
            project(jnp.where(last, O, Q), jnp.where(last, NA - 4, i + 1))
            + project(jnp.where(last, O, V), jnp.where(last, NA - 3, i + 1))
            + project(jnp.where(late, O, K), jnp.where(late, jnp.where(last, NA - 2, i + 5 - NA), i + 5)),
            attention(i), _pad(weights2(0, n >> 2, n & 3, 4), 2))
    lax.fori_loop(1, NA, step, None)
    stats = {}
    run('wo', [P(flush, NA - 1, 0, TA // 2)] + project(O, NA - 1), _pad(weights2(0, 1, 3, 4), 2),
        norm_stats(stats, 0, TF) + norm_rows(stats) + hn2_terms(0))

    def paced(n_tiles, *spans):
        slots = [[] for _ in range(n_tiles)]
        for tasks, where, reads in spans:
            for n, task in enumerate(tasks):
                slots[where[n * len(where) // len(tasks)]].append((task, reads))

        def product(lhs, rhs):
            y = jnp.dot(pltpu.bitcast(lhs, BF16), pltpu.bitcast(rhs, BF16), preferred_element_type=F32)
            for t in range(y.shape[1] // 128):
                tasks = slots.pop(0)
                if any(reads is f_v for _, reads in tasks):
                    f_v[_rows(zero + H0 + NT * TF, 8), :] = y[:8, _cols(t)]
                if any(reads is x_v for _, reads in tasks):
                    pace(y[:16, _cols(t)])
                for task, _ in tasks:
                    task()
            return y
        return product

    def ffn(p, j):
        spans = []
        up = [98 * c + n for c in (0, 1) for lo, hi in CFG['UP'] for n in range(lo, hi)]
        down = list(range(*CFG['DN']))
        if p < 2:
            next_chunk(2 * p + 2 + (j >> 1), (j & 1) == 0)
            spans.append((weights2(p + 1, j >> 1, j & 1, 2), up + down[::CFG['WD'] if p else CFG['WD0']], x_v))
        if p == 2:
            next_chunk(2 * p + 2 + zero, j == 0)
            spans.append((weights2(p + 1, 0, j, NF), up + down[::CFG['WD']], x_v))
        if p == 0:
            stats, nxt = {}, jnp.minimum(j + 1, NF - 1)
            spans += [(norm_stats(stats, nxt * TF, TF) + norm_rows(stats), up, f_v), (hn2_terms(nxt), down, f_v)]
        product = paced(294, *spans)

        def lhs(n):
            row, col = hn2(j, n)
            return m_v[_rows(row, TF // 8), pl.ds(col, 256)]

        def activations(c):
            if CFG['NS'] & 1:
                g, u = (_sixteenths(lambda n: product(lhs(n), wgu2_v[p % 2][c, n, :, _cols(m)]), UP_ORDER) for m in (0, 1))
                return {rc: jax.nn.gelu(g[rc], approximate=True) * u[rc] for rc in g}
            y = _sixteenths(lambda n: product(lhs(n), wgu2_v[p % 2][c, n]), UP_ORDER)
            return {rc: jax.nn.gelu(gu[:, :128], approximate=True) * gu[:, 128:] for rc, gu in y.items()}
        if p < 3:
            for c in range(2):
                act = activations(c)
                for k in DOWN_ORDER:
                    for n, u in _inner_terms(LHS, k, lambda r, c: act[r, c]):
                        a_v[n, :, _cols(c)] = _pack(u)
            if CFG['NS'] & 2:
                for i in range(2):
                    for (r, c), y in _sixteenths(lambda n: product(a_v[n], wd2_v[p % 2][n, :, _cols(i)]), DOWN_ORDER).items():
                        rows = _rows(_tile(Q, 4 * i + c) + j * TF + r * (TF // 4), TF // 4)
                        f_v[rows, :] = f_v[rows, :] + y if p else y
                return
            for (r, c), y in _sixteenths(lambda n: product(a_v[n], wd2_v[p % 2][n]), DOWN_ORDER).items():
                for i in range(2):
                    rows = _rows(_tile(Q, 4 * i + c) + j * TF + r * (TF // 4), TF // 4)
                    f_v[rows, :] = f_v[rows, :] + y[:, _cols(i)] if p else y[:, _cols(i)]
            return
        act = activations(0)
        for k in DOWN_ORDER:
            for i in range(2):
                for c in range(2):
                    a_v[2 * k + i, :, _cols(c)] = _pack(_term(LHS[k], lambda q: act[q // 2 * 2 + i, q % 2 * 2 + c]))
        for i in range(2):
            for c in range(2):
                y = _quadrants(lambda k: product(a_v[2 * k + i], wd2_v[p % 2][2 * k + c]), DOWN_ORDER)
                for q in y:
                    r, t = j * TF + (q // 2 * 2 + i) * (TF // 4), q % 2 * 4 + c * 2
                    acc = jnp.concatenate([f_v[_rows(_tile(Q, t + n) + r, TF // 4), :] for n in (0, 1)], axis=1)
                    block = (_rows(r, TF // 4), pl.ds(t * 128, 256))
                    x_v[block] = (hidden(r, TF // 4, [t, t + 1]) + (acc + y[q])).astype(BF16)
                    pltpu.make_async_copy(x_v.at[block], out_hbm.at[block], sems.at[0]).start()

    for p in CFG['passes']:
        lax.fori_loop(0, NF, lambda j, _: _scope('ffn', P(ffn, p, j)), None)
    pltpu.make_async_copy(x_v.at[pl.ds(0, S)], x_v.at[pl.ds(0, S)], sems.at[0]).wait()


@jax.jit
def pallas_sequential_preLN__sliding_local_dilated__glu_gated_geglu__prompt_kernel(
        A_x, A_wqkv, A_wo, B_x, B_w_gate, B_w_up, B_w_down):
    del B_x
    in_hbm = pl.BlockSpec(memory_space=pl.ANY)
    vmem = pltpu.VMEM
    out = pl.pallas_call(
        _kernel,
        in_specs=[in_hbm] * 6,
        out_specs=in_hbm,
        out_shape=jax.ShapeDtypeStruct((S, D), BF16),
        scratch_shapes=[
            vmem((S + 3 * D + 16, D), BF16),
            vmem((D, D), BF16), [vmem((2, 49, D // 8, 256), I32)] * 2, [vmem((49, FC // 4, 256), I32)] * 2,
            vmem((NT, D // 2 + 8, 128), I32), vmem((NT, D // 2, 128), I32), vmem((2, H * (DH + 1), 128), F32),
            vmem((S + 2 * D, D), I32),
            vmem((H0 + NT * TF + 8, 128), F32),
            vmem((W, TA, 128), F32), vmem((TA // 2, D), I32),
            vmem((49, TF // 8, 256), I32),
            pltpu.SemaphoreType.DMA((3,)),
        ],
        compiler_params=pltpu.CompilerParams(vmem_limit_bytes=126 * 1024 * 1024, flags=CFG['flags'] or None,
                                             disable_bounds_checks=CFG['nobc']),
    )(A_x.reshape(S, D), A_wqkv, A_wo, B_w_gate, B_w_up, B_w_down)
    return out.reshape(A_x.shape)
```

```python
import functools

import jax
import jax.experimental.pallas as pl
import jax.experimental.pallas.tpu as pltpu
import jax.numpy as jnp
import numpy as np
from jax import lax

CFG = dict(passes=(0, 1, 2, 3), TR=16, QR=2, QD=2, QP=1, UP=((0, 98),), DN=(196, 284), WD=2, WD0=2, PP=16, PR=32, RP=32, WS=2, TS=2, LAG=32, PAD=2, LR=16, nest=0, fnest=0, nobc=True,
           skipP=0, skipB=False, scopes=False, flags={})

S, D, DF = 2048, 1024, 3584
H, DH, W, DIL = 32, 32, 8, 2
NT = D // 128
TA = 256
NA = S // TA
TF, NF = 512, S // 512
FC = 512
HALO = 16
KS = HALO + S
K, Q, V, O = 0, 1, 2, 3
H0 = 4 * NT * KS
KC = 256
F32, BF16, I32 = jnp.float32, jnp.bfloat16, jnp.int32
P = functools.partial


def _layernorm(x):
    xc = x - jnp.mean(x, axis=-1, keepdims=True)
    return xc * lax.rsqrt(jnp.mean(xc * xc, axis=-1, keepdims=True) + 1e-5)


def _gelu(x):
    c = np.sqrt(2 / np.pi)
    half = 0.5 * x
    return half + half * jnp.tanh(x * (c + (c * 0.044715) * (x * x)))


def _operand(tiles):
    return pltpu.bitcast(jnp.concatenate(tiles, axis=1), BF16)


def _gather_tiles(tiles, sign):
    g = (lax.broadcasted_iota(I32, tiles[0].shape, 1) >> 2) & 7
    cur = [tiles[(sign * m) % NT] for m in range(NT)]
    for b in (1, 2, 4):
        cur = [jnp.where((g & b) != 0, cur[(m + sign * b) % NT], cur[m]) for m in range(NT)]
    return cur


def _shuffle_lanes(u, m):
    lane = lax.broadcasted_iota(I32, u.shape, 1)
    return jnp.take_along_axis(u, (lane & 3) * 32 + (((lane >> 2) - m) & 7) * 4 + (lane >> 5), axis=1)


LHS = ((0, 1, 3), (2, 1, 3), (0, 0, 0), (3, 0, 3), (0, 1, 1), (2, -1, 0), (1, -1, 3))
RHS = ((0, 1, 3), (0, 0, 0), (1, -1, 3), (2, -1, 0), (3, 0, 3), (0, 1, 1), (2, 1, 3))


def _term(rule, quadrant):
    a, sign, b = rule
    if sign == 0:
        return quadrant(a)
    x, y = quadrant(a).astype(F32), quadrant(b).astype(F32)
    return x + y if sign > 0 else x - y


def _terms(rules, *quadrants):
    return [_term(rule, quadrants.__getitem__) for rule in rules]


USES = (((0, 1), (3, 1)), ((2, 1), (3, -1)), ((1, 1), (3, 1)), ((0, 1), (2, 1)), ((1, 1), (0, -1)), ((3, 1),), ((0, 1),))
UP_ORDER = (0, 1, 3, 2, 4, 5, 6)
DOWN_ORDER = (3, 6, 1, 0, 2, 4, 5)


def _quadrants(product, order):
    acc, left = {}, [4, 2, 2, 4]
    for n in order:
        m = product(n)
        for q, sign in USES[n]:
            if q not in acc:
                acc[q] = (sign, m)
            else:
                s, c = acc[q]
                acc[q] = (1, c + m if s == sign else c - m if s > 0 else m - c)
            left[q] -= 1
            if not left[q]:
                yield q, acc[q][1]


def _inner_terms(rules, k, block):
    outer = [_term(rules[k], lambda q: block(q // 2 * 2 + i, q % 2 * 2 + j)) for i in (0, 1) for j in (0, 1)]
    return enumerate(_terms(rules, *outer), 7 * k)


class _Blocks(dict):
    __add__ = lambda a, b: _Blocks({q: a[q] + b[q] for q in a})
    __sub__ = lambda a, b: _Blocks({q: a[q] - b[q] for q in a})


def _sixteenths(product, order):
    for o, blocks in _quadrants(lambda k: _Blocks(_quadrants(lambda n: product(7 * k + n), order)), order):
        yield o, {(o // 2 * 2 + i // 2, o % 2 * 2 + i % 2): block for i, block in blocks.items()}


def _merge(*lists):
    keyed = [((n + 0.5) / len(l), k, t) for k, l in enumerate(lists) for n, t in enumerate(l)]
    return [t for _, _, t in sorted(keyed, key=lambda e: e[:2])]


def _pad(tasks, n, front=0):
    return [lambda: None] * front + tasks + [lambda: None] * n


def _rows(r, n):
    return pl.ds(r if isinstance(r, int) else pl.multiple_of(r, min(n, 16)), n)


def _cols(t):
    return slice(t * 128, (t + 1) * 128)


def _tile(s, t):
    return (s * NT + t) * KS + HALO


def _scope(name, fn):
    if CFG['scopes']:
        with jax.named_scope('s_' + name):
            fn()
    else:
        fn()


def _kernel(x_hbm, wqkv_hbm, wo_hbm, wg_hbm, wu_hbm, wd_hbm, out_hbm,
            x_v,
            wk_v,
            wgu2_v, wd2_v,
            t1_v, t2_v, t3_v,
            m_v,
            f_v,
            p_v, o_v,
            g_v, act_v, a_v,
            sems):
    PR, RP, LR = CFG['PR'], CFG['RP'], CFG['LR']
    m_w = m_v.bitcast(I32)
    raw = {Q: S, V: S + D, O: S + 2 * D}

    blocks = lambda lo, hi: (x_hbm.at[pl.ds(lo * TA, (hi - lo) * TA)], x_v.at[pl.ds(lo * TA, (hi - lo) * TA)])
    wk = lambda c: (wqkv_hbm.at[:, pl.ds(D + c * KC, KC)], wk_v.at[:, pl.ds(c * KC, KC)])
    copies = {
        'x0': blocks(0, 1), 'wk0': wk(0), 'x1': blocks(1, 2), 'wk1': wk(1), 'wk2': wk(2), 'wk3': wk(3),
        'x2': blocks(2, 3), 'x3': blocks(3, 5),
        'wq': (wqkv_hbm.at[:, pl.ds(0, D)], x_v.at[pl.ds(raw[Q], D)]),
        'wv': (wqkv_hbm.at[:, pl.ds(2 * D, D)], x_v.at[pl.ds(raw[V], D)]),
        'x5': blocks(5, NA), 'wo': (wo_hbm, x_v.at[pl.ds(raw[O], D)])}
    copies = {name: pltpu.make_async_copy(*c, sems.at[n % 3]) for n, (name, c) in enumerate(copies.items())}

    def start(*names):
        for n in names:
            copies[n].start()

    def wait(*names):
        for n in names:
            _scope('w' + n, copies[n].wait)

    start('x0', 'wk0')
    zero = lax.while_loop(lambda c: c > 0, lambda c: c - 16, 16)

    def pace(y):
        x_v[_rows(zero + S + 3 * D, 16), 0:128] = y[:16, :128].astype(BF16)

    def run(name, *lists):
        def go():
            for task in _merge(*lists):
                task()
        if CFG['skipP'] and name != CFG['skipP']:
            return
        if CFG['nest'] == 1 or (CFG['nest'] == 2 and name == 'step'):
            pl.when(zero == 0)(lambda: _scope(name, go))
        else:
            _scope(name, go)

    def project(s, j, tiles=range(NT), as_given=False):
        held = {}
        lhs_row = ((s == O) * NA + j) * (TA // 2)
        w_row, y_row = S + s * (D // 2), _tile(s, 0) + j * TA

        def task(t, r0):
            if r0 == 0:
                lhs = _operand([m_w[k, _rows(lhs_row, TA // 2), :] for k in range(NT)])
                if as_given:
                    w = wk_v[:, _cols(t)]
                else:
                    w = _operand([m_w[t, _rows(w_row, D // 2), :]])
                held['y'] = jnp.dot(lhs, w, preferred_element_type=F32)
            y = held['y'][r0:r0 + RP]
            r = y_row + (t * KS + r0)
            pace(y)
            if isinstance(j, int):
                r = r + zero
                if as_given:
                    t1_v[0, _rows(zero + D // 2, 8), :] = pltpu.bitcast(y[:8], I32)
            f_v[_rows(r, RP), :] = y
        return [P(task, t, r0) for t in tiles for r0 in range(0, TA, RP)]

    def norm1(lo, hi):
        def task(r0):
            y = _layernorm(x_v[pl.ds(r0, LR), :].astype(F32))
            for t in range(NT):
                m_v[t, pl.ds(r0, LR), :] = y[:, _cols(t)].astype(BF16)
        return _pad([P(task, r) for r in range(lo * TA, hi * TA, LR)], 2)

    def hidden(r0, n, cs=range(NT)):
        y = jnp.concatenate([f_v[_rows(_tile(O, t) + r0, n), :] for t in cs], axis=1)
        return x_v[_rows(r0, n), cs[0] * 128:(cs[-1] + 1) * 128].astype(F32) + y

    def norm_stats(stats, j):
        rows = lambda s, t, r: _rows(_tile(s, t) + j * TF + r, 16)

        def center(r):
            y = jnp.concatenate([f_v[rows(O, t, r), :] for t in range(NT)], axis=1)
            h = x_v[_rows(j * TF + r, 16), :].astype(F32) + y
            for t in range(NT):
                f_v[pl.ds(H0 + t * TF + r, 16), :] = h[:, _cols(t)]
            stats[r] = jnp.mean(h, axis=-1, keepdims=True)

        def spread(r):
            hc = jnp.concatenate([f_v[pl.ds(H0 + t * TF + r, 16), :] for t in range(NT)], axis=1) - stats[r]
            stats[r] = (stats[r], lax.rsqrt(jnp.mean(hc * hc, axis=-1, keepdims=True) + 1e-5))

        def scale(r):
            for t in range(NT):
                f_v[pl.ds(H0 + t * TF + r, 16), :] = (f_v[pl.ds(H0 + t * TF + r, 16), :] - stats[r][0]) * stats[r][1]
        return [P(f, r) for f in (center, spread, scale) for r in range(0, TF, 16)]

    def hn2(j, n):
        return j * (13 * TF // 8) + n // 4 * (TF // 8), n % 4 * 2

    def hn2_terms(j):
        def task(r0, t, k):
            for n, u in _inner_terms(LHS, k, lambda r, c: f_v[pl.ds(H0 + (2 * c + t) * TF + r * (TF // 4) + r0, 16), :]):
                row, col = hn2(j, n)
                m_v[col + t, _rows(2 * row + r0, 16), :] = u.astype(BF16)
        return [P(task, r0, t, k) for r0 in range(0, TF // 4, 16) for t in range(2) for k in range(7)]

    def staged(c):
        return S + (c & 1) * (D + FC)

    def ffn_copies(c):
        r, f = staged(c), pl.ds(pl.multiple_of(c * FC, FC), FC)
        return [pltpu.make_async_copy(wg_hbm.at[:, f], x_v.at[_rows(r, D), pl.ds(0, FC)], sems.at[0]),
                pltpu.make_async_copy(wu_hbm.at[:, f], x_v.at[_rows(r, D), pl.ds(FC, FC)], sems.at[1]),
                pltpu.make_async_copy(wd_hbm.at[f], x_v.at[_rows(r + D, FC)], sems.at[2])]

    def weights2(p, c, part, parts):
        base = staged(c)

        def quad(r0, pitch, col, k):
            return _inner_terms(RHS, k, lambda r, c: x_v[
                _rows(base + r0 + r * pitch, 16), pl.ds(col + c // 2 * 256, 256)][:, _cols(c % 2)])

        def gate_up(r0, m, k):
            for n, u in quad(r0, D // 4, m * FC, k):
                wgu2_v[p % 2][c, n, m, _rows(r0, 16), :] = u.astype(BF16)

        def down(r0, t, k):
            for n, u in quad(D + r0, FC // 4, t * 512, k):
                wd2_v[p % 2][n, t, _rows(c * 128 + r0, 16), :] = u.astype(BF16)
        n = D // 4 // parts
        return ([P(gate_up, part * n + r, m, k) for r in range(0, n, 16) for m in (0, 1) for k in range(7)]
                + [P(down, part * (n // 2) + r, t, k) for r in range(0, n // 2, 16) for t in (0, 1) for k in range(7)])

    def reorder_cols(s):
        def stage1(r0):
            src = (lambda t: wk_v[pl.ds(2 * r0, 16), _cols(t)]) if s == K else (
                lambda t: x_v[pl.ds(raw[s] + 2 * r0, 16), _cols(t)])
            for m, u in enumerate(_gather_tiles([pltpu.bitcast(src(t), I32) for t in range(NT)], 1)):
                t1_v[m, _rows(zero + r0, 8), :] = u

        def stage2(r0, m):
            t2_v[m, _rows(zero + r0, PR), :] = _shuffle_lanes(t1_v[m, pl.ds(r0, PR), :], m)

        def stage3(r0):
            for t, u in enumerate(_gather_tiles([t2_v[m, pl.ds(r0, 8), :] for m in range(NT)], -1)):
                m_w[t, pl.ds(S + s * (D // 2) + r0, 8), :] = u
        tasks = []
        for r0 in range(0, D // 2 + 2 * PR, PR):
            tasks += _merge([P(stage1, r) for r in range(r0, r0 + PR, 8) if r < D // 2],
                            [P(stage2, r0 - PR, m) for m in range(NT) if 0 <= r0 - PR < D // 2],
                            [P(stage3, r - 2 * PR) for r in range(r0, r0 + PR, 8) if r >= 2 * PR])
        return _pad(tasks, CFG['PP'])

    def reorder_keys(j):
        held = []

        def task(r0):
            if held:
                lo, tiles = held.pop()
                for t, u in enumerate(tiles):
                    f_v[pl.ds(_tile(K, t) + lo, 8), :] = u
            if r0 < (j + 1) * TA:
                tiles = _gather_tiles([f_v[pl.ds(_tile(K, t) + r0, 8), :] for t in range(NT)], 1)
                held.append((r0, _gather_tiles([_shuffle_lanes(u, m) for m, u in enumerate(tiles)], -1)))
        return [P(task, r) for r in range(j * TA, (j + 1) * TA + 8, 8)]

    def reorder_rows():
        def stage1(t, h0):
            for h in range(h0, h0 + 4):
                t3_v[t % 2, pl.ds(zero + h * (DH + 1), DH), :] = x_v[pl.ds(raw[O] + h * DH, DH), _cols(t)].astype(F32)

        def stage2(t, d0):
            for d in range(d0, d0 + 4):
                m_v[t, pl.ds(2 * S + O * D + d * H, H), :] = t3_v[t % 2, pl.ds(d, H, stride=DH + 1), :].astype(BF16)
        tasks = []
        for t in range(NT + 1):
            tasks += _merge([P(stage1, t, h) for h in range(0, H, 4) if t < NT],
                            [P(stage2, t - 1, d) for d in range(0, DH, 4) if t > 0])
        return _pad(tasks, 4)

    def fill_halo(s, t):
        f_v[pl.ds(_tile(s, t) - HALO, HALO), :] = jnp.broadcast_to(f_v[pl.ds(_tile(s, t), 1), :], (HALO, 128))

    def flush(j, r0, n):
        for t in range(NT):
            m_w[t, _rows((NA + j) * (TA // 2) + r0, n), :] = o_v.bitcast(I32)[t, pl.ds(r0, n), :]

    def attention(i):
        WS, TS, LAG = CFG['WS'], CFG['TS'], CFG['LAG']
        first = isinstance(i, int) and i == 0
        scale = DH ** -0.5

        def scores(parts, r0, ws):
            for t in range(NT):
                q = f_v[_rows(_tile(Q, t) + i * TA + r0, 16), :]
                for w in ws:
                    qk = q * f_v[pl.ds(_tile(K, t) + i * TA + r0 - DIL * w, 16), :]
                    parts[w] = qk if t == 0 else parts[w] + qk
            if len(parts) < W:
                return
            logits = []
            for w in range(W):
                l = parts[w] + pltpu.roll(parts[w], 64, 1)
                l = l + pltpu.roll(l, 32, 1)
                if first and r0 < DIL * w:
                    l = jnp.where(lax.broadcasted_iota(I32, l.shape, 0) + r0 >= DIL * w, l, -1e9 / scale)
                logits.append(l)
            top = functools.reduce(jnp.maximum, logits)
            e = [jnp.exp2((l - top) * (scale * np.log2(np.e))) for l in logits]
            inv = 1.0 / functools.reduce(jnp.add, e)
            for w in range(W):
                p_v[w, pl.ds(r0, 16), :] = e[w] * inv

        def mix(r0, ts):
            p = [p_v[w, pl.ds(r0, 16), :] for w in range(W)]
            for t in ts:
                o_v[t, pl.ds(r0, 16), :] = functools.reduce(jnp.add, [
                    p[w] * f_v[pl.ds(_tile(V, t) + i * TA + r0 - DIL * w, 16), :] for w in range(W)]).astype(BF16)
        tasks = []
        for r0 in range(0, TA + LAG, 16):
            a, b = [], []
            if r0 < TA:
                parts = {}
                a = [P(scores, parts, r0, range(w, w + WS)) for w in range(0, W, WS)]
            if r0 >= LAG:
                b = [P(mix, r0 - LAG, range(t, t + TS)) for t in range(0, NT, TS)]
            elif not first:
                n = TA // 4 * 16 // LAG
                b = [P(flush, i - 1, r0 // 8 * n + r, n) for r in (0, n)]
            tasks += _merge(a, b)
        return _pad(tasks, CFG['PAD'])

    def keys01(lo, hi):
        return sum((project(K, j, [t], True) for t in range(lo, hi) for j in (0, 1)), [])

    wait('x0')
    start('x1')
    run('n0', norm1(0, 1))
    wait('wk0')
    start('wk1')
    run('k0', project(K, 0, range(2), True))
    wait('x1')
    start('wk2')
    run('k0', norm1(1, 2) + project(K, 1, range(2), True))
    wait('wk1')
    start('wk3', 'x2')
    run('k0', keys01(2, 4))
    wait('wk2', 'wk3')
    start('x3')
    run('k1', keys01(4, NT), reorder_cols(K), _pad([P(start, 'wq')], 1, 1))
    wait('x2', 'x3')
    run('k2', norm1(2, 3) + project(K, 2), _pad(reorder_keys(0), 2, 12), _pad(norm1(3, 5), 0, 12), [P(start, 'wv')])
    wait('wq')
    run('k3', project(K, 3), reorder_cols(Q), [P(fill_halo, K, t) for t in range(NT)], [P(start, 'x5')])
    wait('wv')
    start('wo')
    run('k4', project(K, 4), reorder_cols(V))
    wait('x5')
    run('v0', project(V, 0) + project(Q, 0), reorder_keys(1), norm1(5, NA),
        _pad([P(fill_halo, V, t) for t in range(NT)], 0, NT))
    wait('wo')
    for copy in ffn_copies(0):
        copy.start()
    run('step0', project(Q, 1) + project(V, 1) + project(K, 5), attention(0), reorder_rows())


    def next_chunk(c, when):
        @pl.when(when)
        def _():
            for copy in ffn_copies(c):
                copy.wait()

            @pl.when(c < DF // FC - 1)
            def _():
                for copy in ffn_copies(c + 1):
                    copy.start()

    def step(i, _):
        last, late, n = i == NA - 1, i >= NA - 5, i - 1
        next_chunk(n >> 2, (n & 3) == 0)
        run('step',
            project(jnp.where(last, O, Q), jnp.where(last, NA - 4, i + 1))
            + project(jnp.where(last, O, V), jnp.where(last, NA - 3, i + 1))
            + project(jnp.where(late, O, K), jnp.where(late, jnp.where(last, NA - 2, i + 5 - NA), i + 5)),
            attention(i), _pad(weights2(0, n >> 2, n & 3, 4), 2))
    lax.fori_loop(1, NA, step, None)
    stats = {}
    run('wo', [P(flush, NA - 1, 0, TA // 2)] + project(O, NA - 1), _pad(weights2(0, 1, 3, 4), 2),
        norm_stats(stats, 0) + hn2_terms(0))

    def paced(n_tiles, *spans):
        slots = [[] for _ in range(n_tiles)]
        for tasks, where, reads in spans:
            for n, task in enumerate(tasks):
                slots[where[n * len(where) // len(tasks)]].append((task, reads))

        def product(lhs, rhs):
            y = jnp.dot(_operand(lhs), _operand([rhs]), preferred_element_type=F32)
            for t in range(y.shape[1] // 128):
                tasks = slots.pop(0)
                if any(reads is f_v for _, reads in tasks):
                    f_v[_rows(zero + H0 + NT * TF, 8), :] = y[:8, _cols(t)]
                if any(reads is x_v for _, reads in tasks):
                    pace(y[:16, _cols(t)])
                for task, _ in tasks:
                    task()
            return y
        return product

    def ffn(p, j):
        spans = []
        early = [98 * c + n for c in (0, 1) for lo, hi in CFG['UP'] for n in range(lo, hi)]
        down = list(range(*CFG['DN']))
        if p < 2:
            next_chunk(2 * p + 2 + (j >> 1), (j & 1) == 0)
            spans.append((weights2(p + 1, j >> 1, j & 1, 2), early + down[::CFG['WD'] if p else CFG['WD0']], x_v))
        if p == 2:
            next_chunk(2 * p + 2 + zero, j == 0)
            spans.append((weights2(p + 1, 0, j, NF), early + down[::CFG['WD']], x_v))
        if p == 0:
            stats, nxt = {}, jnp.minimum(j + 1, NF - 1)
            spans += [(norm_stats(stats, nxt), early, f_v), (hn2_terms(nxt), down, f_v)]
        product = paced(294, *spans)

        def lhs(n):
            row, col = hn2(j, n)
            return [m_w[col + t, _rows(row, TF // 8), :] for t in range(2)]

        chunks = 2 if p < 3 else 1
        wgu_w, wd_w, a_w = (ref.bitcast(I32) for ref in (wgu2_v[p % 2], wd2_v[p % 2], a_v))
        queue, TR = [], CFG['TR']

        def terms(c, k, r0):
            for n, term in _inner_terms(LHS, k, lambda r, t: act_v[c][4 * r + t, pl.ds(r0, TR), :]):
                a_v[n, c, pl.ds(r0, TR), :] = term.astype(BF16)

        def up_product(c, m, n):
            y = product(lhs(n), wgu_w[c, n, m])
            if queue and CFG['QP']:
                act_v[queue[0][0]][zero + 16, 0:8, :] = y[:8]
            for task in queue[:3 - chunks]:
                terms(*task)
            del queue[:3 - chunks]
            return y

        def down_product(i, n):
            while any(k == n // 7 for _, k, _ in queue):
                terms(*queue.pop(0))
            y = product([a_w[n, c] for c in range(chunks)], wd_w[n, i, 0:chunks * 64, :])
            if queue and CFG['QP']:
                act_v[queue[0][0]][zero + 16, 0:8, :] = y[:8]
            for task in queue[:CFG['QD']]:
                terms(*task)
            del queue[:CFG['QD']]
            return y
        for c in range(chunks):
            for _, gate in _sixteenths(P(up_product, c, 0), UP_ORDER):
                for (r, t), g in gate.items():
                    g_v[zero + 4 * r + t] = _gelu(g)
            have, todo = set(), list(DOWN_ORDER)
            for q, up in _sixteenths(P(up_product, c, 1), UP_ORDER):
                for (r, t), u in up.items():
                    act_v[c][zero + 4 * r + t] = g_v[4 * r + t] * u
                have.add(q)
                for k in [k for k in todo if {LHS[k][0], LHS[k][2]} <= have]:
                    todo.remove(k)
                    queue += [(c, k, r0) for r0 in range(0, TF // 4, TR)]
        for i in range(2):
            for (r, c), y in (block for _, blocks in _sixteenths(P(down_product, i), DOWN_ORDER)
                              for block in blocks.items()):
                r0, t = j * TF + r * (TF // 4), 4 * i + c
                rows = _rows(_tile(Q, t) + r0, TF // 4)
                acc = f_v[rows, :] + y if p else y
                if p < 3:
                    f_v[rows, :] = acc
                else:
                    block = (_rows(r0, TF // 4), pl.ds(t * 128, 128))
                    x_v[block] = (hidden(r0, TF // 4, [t]) + acc).astype(BF16)
                    pltpu.make_async_copy(x_v.at[block], out_hbm.at[block], sems.at[0]).start()

    for p in CFG['passes']:
        lax.fori_loop(0, NF, lambda j, _: _scope('ffn', P(ffn, p, j)), None)
    pltpu.make_async_copy(x_v.at[pl.ds(0, S)], x_v.at[pl.ds(0, S)], sems.at[0]).wait()


@jax.jit
def pallas_sequential_preLN__sliding_local_dilated__glu_gated_geglu__prompt_kernel(
        A_x, A_wqkv, A_wo, B_x, B_w_gate, B_w_up, B_w_down):
    del B_x
    in_hbm = pl.BlockSpec(memory_space=pl.ANY)
    vmem = pltpu.VMEM
    out = pl.pallas_call(
        _kernel,
        in_specs=[in_hbm] * 6,
        out_specs=in_hbm,
        out_shape=jax.ShapeDtypeStruct((S, D), BF16),
        scratch_shapes=[
            vmem((S + 3 * D + 16, D), BF16),
            vmem((D, D), BF16), [vmem((2, 49, 2, D // 4, 128), BF16)] * 2, [vmem((49, 2, FC // 2, 128), BF16)] * 2,
            vmem((NT, D // 2 + 8, 128), I32), vmem((NT, D // 2, 128), I32), vmem((2, H * (DH + 1), 128), F32),
            vmem((NT, 2 * S + 4 * D, 128), BF16),
            vmem((H0 + NT * TF + 8, 128), F32),
            vmem((W, TA, 128), F32), vmem((NT, TA, 128), BF16),
            vmem((16, TF // 4, 128), F32), [vmem((17, TF // 4, 128), F32)] * 2, vmem((49, 2, TF // 4, 128), BF16),
            pltpu.SemaphoreType.DMA((3,)),
        ],
        compiler_params=pltpu.CompilerParams(vmem_limit_bytes=126 * 1024 * 1024, flags=CFG['flags'] or None,
                                             disable_bounds_checks=CFG['nobc']),
    )(A_x.reshape(S, D), A_wqkv, A_wo, B_w_gate, B_w_up, B_w_down)
    return out.reshape(A_x.shape)
```

```python
import functools

import jax
import jax.experimental.pallas as pl
import jax.experimental.pallas.tpu as pltpu
import jax.numpy as jnp
import numpy as np
from jax import lax

CFG = dict(passes=(0, 1, 2, 3), SP=8, FE=4, FR=0, TR=16, QR=2, QD=2, QP=1, UP=((0, 98),), DN=(196, 284), WD=2, WD0=2, PP=16, PR=32, RP=32, WS=1, TS=1, LAG=32, PAD=4, MP=0, WP=512, LR=16, nest=0, fnest=0, nobc=True,
           skipP=0, skipB=False, scopes=False, flags={})

S, D, DF = 2048, 1024, 3584
H, DH, W, DIL = 32, 32, 8, 2
NT = D // 128
TA = 256
NA = S // TA
TF, NF = 512, S // 512
FC = 512
HALO = 16
KS = HALO + S
K, Q, V, O = 0, 1, 2, 3
H0 = 4 * NT * KS
RING = 128
KC = 256
F32, BF16, I32 = jnp.float32, jnp.bfloat16, jnp.int32
P = functools.partial


def _layernorm(x):
    xc = x - jnp.mean(x, axis=-1, keepdims=True)
    return xc * lax.rsqrt(jnp.mean(xc * xc, axis=-1, keepdims=True) + 1e-5)


def _gelu(x):
    c = np.sqrt(2 / np.pi)
    half = 0.5 * x
    return half + half * jnp.tanh(x * (c + (c * 0.044715) * (x * x)))


def _operand(tiles):
    return pltpu.bitcast(jnp.concatenate(tiles, axis=1), BF16)


def _gather_tiles(tiles, sign):
    g = (lax.broadcasted_iota(I32, tiles[0].shape, 1) >> 2) & 7
    cur = [tiles[(sign * m) % NT] for m in range(NT)]
    for b in (1, 2, 4):
        cur = [jnp.where((g & b) != 0, cur[(m + sign * b) % NT], cur[m]) for m in range(NT)]
    return cur


def _shuffle_lanes(u, m):
    lane = lax.broadcasted_iota(I32, u.shape, 1)
    return jnp.take_along_axis(u, (lane & 3) * 32 + (((lane >> 2) - m) & 7) * 4 + (lane >> 5), axis=1)


LHS = ((0, 1, 3), (2, 1, 3), (0, 0, 0), (3, 0, 3), (0, 1, 1), (2, -1, 0), (1, -1, 3))
RHS = ((0, 1, 3), (0, 0, 0), (1, -1, 3), (2, -1, 0), (3, 0, 3), (0, 1, 1), (2, 1, 3))


def _term(rule, quadrant):
    a, sign, b = rule
    if sign == 0:
        return quadrant(a)
    x, y = quadrant(a).astype(F32), quadrant(b).astype(F32)
    return x + y if sign > 0 else x - y


def _terms(rules, *quadrants):
    return [_term(rule, quadrants.__getitem__) for rule in rules]


USES = (((0, 1), (3, 1)), ((2, 1), (3, -1)), ((1, 1), (3, 1)), ((0, 1), (2, 1)), ((1, 1), (0, -1)), ((3, 1),), ((0, 1),))
UP_ORDER = (0, 1, 3, 2, 4, 5, 6)
DOWN_ORDER = (3, 6, 1, 0, 2, 4, 5)


def _quadrants(product, order):
    acc, left = {}, [4, 2, 2, 4]
    for n in order:
        m = product(n)
        for q, sign in USES[n]:
            if q not in acc:
                acc[q] = (sign, m)
            else:
                s, c = acc[q]
                acc[q] = (1, c + m if s == sign else c - m if s > 0 else m - c)
            left[q] -= 1
            if not left[q]:
                yield q, acc[q][1]


def _inner_terms(rules, k, block):
    outer = [_term(rules[k], lambda q: block(q // 2 * 2 + i, q % 2 * 2 + j)) for i in (0, 1) for j in (0, 1)]
    return enumerate(_terms(rules, *outer), 7 * k)


class _Blocks(dict):
    __add__ = lambda a, b: _Blocks({q: a[q] + b[q] for q in a})
    __sub__ = lambda a, b: _Blocks({q: a[q] - b[q] for q in a})


def _sixteenths(product, order):
    for o, blocks in _quadrants(lambda k: _Blocks(_quadrants(lambda n: product(7 * k + n), order)), order):
        yield o, {(o // 2 * 2 + i // 2, o % 2 * 2 + i % 2): block for i, block in blocks.items()}


def _merge(*lists):
    keyed = [((n + 0.5) / len(l), k, t) for k, l in enumerate(lists) for n, t in enumerate(l)]
    return [t for _, _, t in sorted(keyed, key=lambda e: e[:2])]


def _pad(tasks, n, front=0):
    return [lambda: None] * front + tasks + [lambda: None] * n


def _rows(r, n):
    return pl.ds(r if isinstance(r, int) else pl.multiple_of(r, min(n, 16)), n)


def _cols(t):
    return slice(t * 128, (t + 1) * 128)


def _tile(s, t):
    return (s * NT + t) * KS + HALO


def _wterm(s, n, t):
    return ((s * 7 + n) * (NT // 2) + t) * (D // 2)


def _scope(name, fn):
    if CFG['scopes']:
        with jax.named_scope('s_' + name):
            fn()
    else:
        fn()


def _kernel(x_hbm, wqkv_hbm, wo_hbm, wg_hbm, wu_hbm, wd_hbm, out_hbm,
            x_v,
            wk_v,
            wgu2_v, wd2_v,
            t1_v, t2_v, t3_v,
            m_v,
            s_v,
            f_v,
            p_v, o_v,
            g_v, act_v, a_v,
            sems):
    PR, RP, LR = CFG['PR'], CFG['RP'], CFG['LR']
    m_w = m_v.bitcast(I32)
    raw = {Q: S, V: S + D, O: S + 2 * D}

    blocks = lambda lo, hi: (x_hbm.at[pl.ds(lo * TA, (hi - lo) * TA)], x_v.at[pl.ds(lo * TA, (hi - lo) * TA)])
    wk = lambda c: (wqkv_hbm.at[:, pl.ds(D + c * KC, KC)], wk_v.at[:, pl.ds(c * KC, KC)])
    copies = {
        'x0': blocks(0, 1), 'wk0': wk(0), 'x1': blocks(1, 2), 'wk1': wk(1), 'wk2': wk(2), 'wk3': wk(3),
        'x2': blocks(2, 3), 'x3': blocks(3, 5),
        'wq': (wqkv_hbm.at[:, pl.ds(0, D)], x_v.at[pl.ds(raw[Q], D)]),
        'wv': (wqkv_hbm.at[:, pl.ds(2 * D, D)], x_v.at[pl.ds(raw[V], D)]),
        'x5': blocks(5, NA), 'wo': (wo_hbm, x_v.at[pl.ds(raw[O], D)])}
    copies = {name: pltpu.make_async_copy(*c, sems.at[n % 3]) for n, (name, c) in enumerate(copies.items())}

    def start(*names):
        for n in names:
            copies[n].start()

    def wait(*names):
        for n in names:
            _scope('w' + n, copies[n].wait)

    start('x0', 'wk0')
    zero = lax.while_loop(lambda c: c > 0, lambda c: c - 16, 16)

    def pace(y):
        x_v[_rows(zero + S + 3 * D, 16), 0:128] = y[:16, :128].astype(BF16)

    def run(name, *lists):
        def go():
            for task in _merge(*lists):
                task()
        if CFG['skipP'] and name != CFG['skipP']:
            return
        if CFG['nest'] == 1 or (CFG['nest'] == 2 and name == 'step'):
            pl.when(zero == 0)(lambda: _scope(name, go))
        else:
            _scope(name, go)

    def project(s, j, tiles=range(NT), as_given=False):
        held = {}
        lhs_row, w_row, y_row = j * TA // 2, (S + s * D) // 2, _tile(s, 0) + j * TA

        def task(t, r0):
            if r0 == 0:
                lhs = _operand([m_w[k, _rows(lhs_row, TA // 2), :] for k in range(NT)])
                if as_given:
                    w = wk_v[:, _cols(t)]
                else:
                    w = _operand([m_w[t, _rows(w_row, D // 2), :]])
                held['y'] = jnp.dot(lhs, w, preferred_element_type=F32)
            y = held['y'][r0:r0 + RP]
            r = y_row + (t * KS + r0)
            pace(y)
            if as_given:
                t1_v[0, _rows(zero + RING, 8), :] = pltpu.bitcast(y[:8], I32)
            if s != K or j == 5:
                wgu2_v[1][_rows(zero + _wterm(4, 0, 0), 16), :] = y[:16].astype(BF16)
            f_v[_rows(r + zero, RP), :] = y
        return [P(task, t, r0) for t in tiles for r0 in range(0, TA, RP)]

    def lhs_terms(b, get):
        held, row = [], b * (7 * TA // 2)

        def task(r0, t):
            for n, lo, tile, u in held:
                s_v[tile, _rows(row + (n * (TA // 2) + lo), 16), :] = u
            held.clear()
            if r0 < TA // 2:
                blocks = [get(r, c) for r in (r0, r0 + TA // 2) for c in (t, t + NT // 2)]
                held.extend((n, r0, t, u.astype(BF16)) for n, u in enumerate(_terms(LHS, *blocks)))
        return [P(task, r0, t) for r0 in range(0, TA // 2, 16) for t in range(NT // 2)] + [P(task, TA // 2, 0)]

    def norm1(lo, hi):
        def task(j, r0):
            y = _layernorm(x_v[pl.ds(j * TA + r0, 16), :].astype(F32))
            for t in range(NT):
                if j <= 5:
                    m_v[t, pl.ds(j * TA + r0, 16), :] = y[:, _cols(t)].astype(BF16)
                if j >= 2:
                    o_v[zero + j % 2, t, pl.ds(r0, 16), :] = y[:, _cols(t)]
        tasks = []
        for j in range(lo, hi):
            late = lhs_terms(j - 1, lambda r, t, j=j: o_v[(j - 1) % 2, t, pl.ds(r, 16), :]) if j > 2 else []
            tasks += _merge([P(task, j, r) for r in range(0, TA, 16)], late)
        if hi == NA:
            tasks += lhs_terms(NA - 1, lambda r, t: o_v[(NA - 1) % 2, t, pl.ds(r, 16), :])
        return _pad(tasks, 2)

    def weights1(s):
        def task(r0, t):
            blocks = [m_v[c, pl.ds(S + s * D + r, 16), :] for r in (r0, r0 + D // 2) for c in (2 * t, 2 * t + 1)]
            for n, u in enumerate(_terms(RHS, *blocks)):
                wgu2_v[1][pl.ds(_wterm(s, n, t) + r0, 16), :] = u.astype(BF16)
        return [P(task, r0, t) for t in range(NT // 2) for r0 in range(0, D // 2, 16)]

    def hidden(r0, n, cs=range(NT)):
        y = jnp.concatenate([f_v[_rows(_tile(O, t) + r0, n), :] for t in cs], axis=1)
        return x_v[_rows(r0, n), cs[0] * 128:(cs[-1] + 1) * 128].astype(F32) + y

    def norm_stats(stats, j):
        rows = lambda s, t, r: _rows(_tile(s, t) + j * TF + r, 16)

        def center(r):
            y = jnp.concatenate([f_v[rows(O, t, r), :] for t in range(NT)], axis=1)
            h = x_v[_rows(j * TF + r, 16), :].astype(F32) + y
            for t in range(NT):
                f_v[pl.ds(H0 + t * TF + r, 16), :] = h[:, _cols(t)]
            stats[r] = jnp.mean(h, axis=-1, keepdims=True)

        def spread(r):
            hc = jnp.concatenate([f_v[pl.ds(H0 + t * TF + r, 16), :] for t in range(NT)], axis=1) - stats[r]
            stats[r] = (stats[r], lax.rsqrt(jnp.mean(hc * hc, axis=-1, keepdims=True) + 1e-5))

        def scale(r):
            for t in range(NT):
                f_v[pl.ds(H0 + t * TF + r, 16), :] = (f_v[pl.ds(H0 + t * TF + r, 16), :] - stats[r][0]) * stats[r][1]
        return [P(f, r) for f in (center, spread, scale) for r in range(0, TF, 16)]

    def hn2(j, n):
        return j * (13 * TF // 8) + n // 4 * (TF // 8), n % 4 * 2

    def hn2_terms(j):
        def task(r0, t, k):
            for n, u in _inner_terms(LHS, k, lambda r, c: f_v[pl.ds(H0 + (2 * c + t) * TF + r * (TF // 4) + r0, 16), :]):
                row, col = hn2(0, n)
                m_v[col + t, _rows(j * (13 * TF // 4) + (2 * row + r0), 16), :] = u.astype(BF16)
        return [P(task, r0, t, k) for r0 in range(0, TF // 4, 16) for t in range(2) for k in range(7)]

    def staged(c):
        return S + (c & 1) * (D + FC)

    def ffn_copies(c):
        r, f = staged(c), pl.ds(pl.multiple_of(c * FC, FC), FC)
        return [pltpu.make_async_copy(wg_hbm.at[:, f], x_v.at[_rows(r, D), pl.ds(0, FC)], sems.at[0]),
                pltpu.make_async_copy(wu_hbm.at[:, f], x_v.at[_rows(r, D), pl.ds(FC, FC)], sems.at[1]),
                pltpu.make_async_copy(wd_hbm.at[f], x_v.at[_rows(r + D, FC)], sems.at[2])]

    def weights2(p, c, part, parts):
        n = D // 4 // parts
        up_src, down_src = staged(c) + part * n, staged(c) + D + part * (n // 2)
        up_row, down_row = c * (98 * 256) + part * n, c * 128 + part * (n // 2)

        def quad(r0, pitch, col, k):
            return _inner_terms(RHS, k, lambda r, c: x_v[
                _rows(r0 + r * pitch, 16), pl.ds(col + c // 2 * 256, 256)][:, _cols(c % 2)])

        def gate_up(r0, m, k):
            for n, u in quad(up_src + r0, D // 4, m * FC, k):
                wgu2_v[p % 2][_rows(up_row + ((2 * n + m) * 256 + r0), 16), :] = u.astype(BF16)

        def down(r0, t, k):
            for n, u in quad(down_src + r0, FC // 4, t * 512, k):
                wd2_v[p % 2][n, t, _rows(down_row + r0, 16), :] = u.astype(BF16)
        return ([P(gate_up, r, m, k) for r in range(0, n, 16) for m in (0, 1) for k in range(7)]
                + [P(down, r, t, k) for r in range(0, n // 2, 16) for t in (0, 1) for k in range(7)])

    def reorder_cols(s):
        def stage1(r0):
            src = (lambda t: wk_v[pl.ds(2 * r0, 16), _cols(t)]) if s == K else (
                lambda t: x_v[pl.ds(raw[s] + 2 * r0, 16), _cols(t)])
            for m, u in enumerate(_gather_tiles([pltpu.bitcast(src(t), I32) for t in range(NT)], 1)):
                t1_v[m, _rows(zero + r0 % RING, 8), :] = u

        def stage2(r0, m):
            t2_v[m, _rows(zero + r0 % RING, PR), :] = _shuffle_lanes(t1_v[m, pl.ds(r0 % RING, PR), :], m)

        def stage3(r0):
            for t, u in enumerate(_gather_tiles([t2_v[m, pl.ds(r0 % RING, 8), :] for m in range(NT)], -1)):
                m_w[t, pl.ds((S + s * D) // 2 + r0, 8), :] = u
        tasks = []
        for r0 in range(0, D // 2 + 2 * PR, PR):
            tasks += _merge([P(stage1, r) for r in range(r0, r0 + PR, 8) if r < D // 2],
                            [P(stage2, r0 - PR, m) for m in range(NT) if 0 <= r0 - PR < D // 2],
                            [P(stage3, r - 2 * PR) for r in range(r0, r0 + PR, 8) if r >= 2 * PR])
        return _pad(tasks, CFG['PP'])

    def reorder_keys(j):
        held = []

        def task(r0):
            if held:
                lo, tiles = held.pop()
                for t, u in enumerate(tiles):
                    f_v[pl.ds(_tile(K, t) + lo, 8), :] = u
            if r0 < (j + 1) * TA:
                tiles = _gather_tiles([f_v[pl.ds(_tile(K, t) + r0, 8), :] for t in range(NT)], 1)
                held.append((r0, _gather_tiles([_shuffle_lanes(u, m) for m, u in enumerate(tiles)], -1)))
        return [P(task, r) for r in range(j * TA, (j + 1) * TA + 8, 8)]

    def reorder_rows():
        def stage1(t, h0):
            for h in range(h0, h0 + 4):
                t3_v[t % 2, pl.ds(zero + h * (DH + 1), DH), :] = x_v[pl.ds(raw[O] + h * DH, DH), _cols(t)].astype(F32)

        def stage2(t, d0):
            for d in range(d0, d0 + 4):
                m_v[t, pl.ds(S + O * D + d * H, H), :] = t3_v[t % 2, pl.ds(d, H, stride=DH + 1), :].astype(BF16)
        tasks = []
        for t in range(NT + 1):
            tasks += _merge([P(stage1, t, h) for h in range(0, H, 4) if t < NT],
                            [P(stage2, t - 1, d) for d in range(0, DH, 4) if t > 0])
        return _pad(tasks, 4)

    def fill_halo(s, t):
        f_v[pl.ds(_tile(s, t) - HALO, HALO), :] = jnp.broadcast_to(f_v[pl.ds(_tile(s, t), 1), :], (HALO, 128))

    def flush(j):
        return lhs_terms(NA + (j & 3), lambda r, t: o_v[j & 1, t, pl.ds(r, 16), :])

    def attention(i):
        WS, TS, LAG = CFG['WS'], CFG['TS'], CFG['LAG']
        first = isinstance(i, int) and i == 0
        scale = DH ** -0.5

        def scores(parts, r0, ws):
            for t in range(NT):
                q = f_v[_rows(_tile(Q, t) + i * TA + r0, 16), :]
                for w in ws:
                    qk = q * f_v[pl.ds(_tile(K, t) + i * TA + r0 - DIL * w, 16), :]
                    parts[w] = qk if t == 0 else parts[w] + qk
            if len(parts) < W:
                return
            logits = []
            for w in range(W):
                l = parts[w] + pltpu.roll(parts[w], 64, 1)
                l = l + pltpu.roll(l, 32, 1)
                if first and r0 < DIL * w:
                    l = jnp.where(lax.broadcasted_iota(I32, l.shape, 0) + r0 >= DIL * w, l, -1e9 / scale)
                logits.append(l)
            top = functools.reduce(jnp.maximum, logits)
            e = [jnp.exp2((l - top) * (scale * np.log2(np.e))) for l in logits]
            inv = 1.0 / functools.reduce(jnp.add, e)
            for w in range(W):
                p_v[w, pl.ds(r0, 16), :] = e[w] * inv

        def mix(r0, ts):
            p = [p_v[w, pl.ds(r0, 16), :] for w in range(W)]
            for t in ts:
                o_v[i & 1, t, pl.ds(r0, 16), :] = functools.reduce(jnp.add, [
                    p[w] * f_v[pl.ds(_tile(V, t) + i * TA + r0 - DIL * w, 16), :] for w in range(W)])
        tasks = []
        for r0 in range(0, TA + LAG, 16):
            a, b = [], []
            if r0 < TA:
                parts = {}
                a = [P(scores, parts, r0, range(w, w + WS)) for w in range(0, W, WS)]
            if r0 >= LAG:
                b = [P(mix, r0 - LAG, range(t, t + TS)) for t in range(0, NT, TS)]
            tasks += _merge(a, b)
        return _pad(tasks, CFG['PAD'])

    def keys01(lo, hi):
        return sum((project(K, j, [t], True) for t in range(lo, hi) for j in (0, 1)), [])

    wait('x0')
    start('x1')
    run('n0', norm1(0, 1))
    wait('wk0')
    start('wk1')
    run('k0', project(K, 0, range(2), True))
    wait('x1')
    start('wk2')
    run('k0', norm1(1, 2) + project(K, 1, range(2), True))
    wait('wk1')
    start('wk3', 'x2')
    run('k0', keys01(2, 4))
    wait('wk2', 'wk3')
    start('x3')
    run('k1', keys01(4, NT), reorder_cols(K), _pad([P(start, 'wq')], 1, 1))
    wait('x2', 'x3')
    run('k2', norm1(2, 3) + project(K, 2), _pad(reorder_keys(0), 2, 12), _pad(norm1(3, 5), 0, 12), [P(start, 'wv')])
    wait('wq')
    run('k3', project(K, 3), reorder_cols(Q), [P(fill_halo, K, t) for t in range(NT)], [P(start, 'x5')])
    wait('wv')
    start('wo')
    run('k4', project(K, 4), reorder_cols(V))
    wait('x5')
    run('v0', project(V, 0) + project(Q, 0), reorder_keys(1), norm1(5, NA), weights1(K) + weights1(Q),
        _pad([P(fill_halo, V, t) for t in range(NT)], 0, NT))
    wait('wo')
    for copy in ffn_copies(0):
        copy.start()
    run('step0', project(Q, 1) + project(V, 1) + project(K, 5), attention(0),
        _merge(reorder_rows(), weights1(V)) + weights1(O))


    def next_chunk(c, when):
        @pl.when(when)
        def _():
            for copy in ffn_copies(c):
                copy.wait()

            @pl.when(c < DF // FC - 1)
            def _():
                for copy in ffn_copies(c + 1):
                    copy.start()

    def paced(n_slots, parts, *spans):
        slots = [[] for _ in range(n_slots)]
        for tasks, where, reads in spans:
            for n, task in enumerate(tasks):
                slots[where[n * len(where) // len(tasks)]].append((task, reads))

        def product(lhs, rhs):
            y = jnp.dot(_operand(lhs), _operand([rhs]), preferred_element_type=F32)
            for r0 in range(0, y.shape[0], y.shape[0] // parts):
                tasks = slots.pop(0)
                if any(reads is f_v for _, reads in tasks):
                    f_v[_rows(zero + H0 + NT * TF, 8), :] = y[r0:r0 + 8]
                if any(reads is x_v for _, reads in tasks):
                    pace(y[r0:r0 + 16])
                for task, _ in tasks:
                    task()
            return y
        return product

    def project7(product, s, j):
        lhs_row = jnp.where(s == O, NA + (j & 3), j) * (7 * TA // 4)
        s_w, w_w = s_v.bitcast(I32), wgu2_v[1].bitcast(I32)
        w_row, y_row = s * (_wterm(1, 0, 0) // 2), _tile(s, 0) + j * TA
        for t in range(NT // 2):
            for q, y in _quadrants(lambda n: product(
                    [s_w[k, _rows(lhs_row + n * TA // 4, TA // 4), :] for k in range(NT // 2)],
                    w_w[_rows(w_row + _wterm(0, n, t) // 2, D // 4), :]), UP_ORDER):
                f_v[_rows(y_row + ((2 * t + q % 2) * KS + q // 2 * (TA // 2)), TA // 2), :] = y

    def step(i):
        last, late, n, SP = i == NA - 1, i >= NA - 5, i - 1, CFG['SP']
        next_chunk(n >> 2, (n & 3) == 0)
        product = paced(84 * SP, SP, (attention(i), range(84 * SP), f_v), (flush(i - 1), range(CFG['FE'] * SP), CFG['FR'] and f_v),
                        (weights2(0, n >> 2, n & 3, 4), range(82 * SP), x_v))
        project7(product, jnp.where(last, O, Q), jnp.where(last, NA - 4, i + 1))
        project7(product, jnp.where(last, O, V), jnp.where(last, NA - 3, i + 1))
        project7(product, jnp.where(late, O, K), jnp.where(late, jnp.where(last, NA - 2, i + 5 - NA), i + 5))
    lax.fori_loop(1, NA, lambda i, _: _scope('step', P(step, i)), None)

    def tail():
        for task in flush(NA - 1):
            task()
        project7(paced(28 * 8, 8, (weights2(0, 1, 3, 4), range(216), x_v),
                       (norm_stats({}, 0) + hn2_terms(0), range(220), f_v)), O, NA - 1)
    if not CFG['skipP']:
        _scope('wo', tail)

    def ffn(p, j):
        spans = []
        early = [98 * c + n for c in (0, 1) for lo, hi in CFG['UP'] for n in range(lo, hi)]
        down = list(range(*CFG['DN']))
        if p < 2:
            next_chunk(2 * p + 2 + (j >> 1), (j & 1) == 0)
            spans.append((weights2(p + 1, j >> 1, j & 1, 2), early + down[::CFG['WD'] if p else CFG['WD0']], x_v))
        if p == 2:
            next_chunk(2 * p + 2 + zero, j == 0)
            spans.append((weights2(p + 1, 0, j, NF), early + down[::CFG['WD']], x_v))
        if p == 0:
            stats, nxt = {}, jnp.minimum(j + 1, NF - 1)
            spans += [(norm_stats(stats, nxt), early, f_v), (hn2_terms(nxt), down, f_v)]
        product = paced(294, 1, *spans)

        def lhs(n):
            row, col = hn2(j, n)
            return [m_w[col + t, _rows(row, TF // 8), :] for t in range(2)]

        chunks = 2 if p < 3 else 1
        wgu_w, wd_w, a_w = (ref.bitcast(I32) for ref in (wgu2_v[p % 2], wd2_v[p % 2], a_v))
        queue, TR = [], CFG['TR']

        def terms(c, k, r0):
            for n, term in _inner_terms(LHS, k, lambda r, t: act_v[c][4 * r + t, pl.ds(r0, TR), :]):
                a_v[n, c, pl.ds(r0, TR), :] = term.astype(BF16)

        def up_product(c, m, n):
            y = product(lhs(n), wgu_w[pl.ds(((c * 49 + n) * 2 + m) * 128, 128), :])
            if queue and CFG['QP']:
                act_v[queue[0][0]][zero + 16, 0:8, :] = y[:8]
            for task in queue[:3 - chunks]:
                terms(*task)
            del queue[:3 - chunks]
            return y

        def down_product(i, n):
            while any(k == n // 7 for _, k, _ in queue):
                terms(*queue.pop(0))
            y = product([a_w[n, c] for c in range(chunks)], wd_w[n, i, 0:chunks * 64, :])
            if queue and CFG['QP']:
                act_v[queue[0][0]][zero + 16, 0:8, :] = y[:8]
            for task in queue[:CFG['QD']]:
                terms(*task)
            del queue[:CFG['QD']]
            return y
        for c in range(chunks):
            for _, gate in _sixteenths(P(up_product, c, 0), UP_ORDER):
                for (r, t), g in gate.items():
                    g_v[zero + 4 * r + t] = _gelu(g)
            have, todo = set(), list(DOWN_ORDER)
            for q, up in _sixteenths(P(up_product, c, 1), UP_ORDER):
                for (r, t), u in up.items():
                    act_v[c][zero + 4 * r + t] = g_v[4 * r + t] * u
                have.add(q)
                for k in [k for k in todo if {LHS[k][0], LHS[k][2]} <= have]:
                    todo.remove(k)
                    queue += [(c, k, r0) for r0 in range(0, TF // 4, TR)]
        for i in range(2):
            for (r, c), y in (block for _, blocks in _sixteenths(P(down_product, i), DOWN_ORDER)
                              for block in blocks.items()):
                r0, t = j * TF + r * (TF // 4), 4 * i + c
                rows = _rows(_tile(Q, t) + r0, TF // 4)
                acc = f_v[rows, :] + y if p else y
                if p < 3:
                    f_v[rows, :] = acc
                else:
                    block = (_rows(r0, TF // 4), pl.ds(t * 128, 128))
                    x_v[block] = (hidden(r0, TF // 4, [t]) + acc).astype(BF16)
                    pltpu.make_async_copy(x_v.at[block], out_hbm.at[block], sems.at[0]).start()

    for p in CFG['passes']:
        lax.fori_loop(0, NF, lambda j, _: _scope('ffn', P(ffn, p, j)), None)
    pltpu.make_async_copy(x_v.at[pl.ds(0, S)], x_v.at[pl.ds(0, S)], sems.at[0]).wait()


@jax.jit
def pallas_sequential_preLN__sliding_local_dilated__glu_gated_geglu__prompt_kernel(
        A_x, A_wqkv, A_wo, B_x, B_w_gate, B_w_up, B_w_down):
    del B_x
    in_hbm = pl.BlockSpec(memory_space=pl.ANY)
    vmem = pltpu.VMEM
    out = pl.pallas_call(
        _kernel,
        in_specs=[in_hbm] * 6,
        out_specs=in_hbm,
        out_shape=jax.ShapeDtypeStruct((S, D), BF16),
        scratch_shapes=[
            vmem((S + 3 * D + 64, D), BF16),
            vmem((D, D), BF16), [vmem((2 * 49 * 2 * 256, 128), BF16), vmem((_wterm(4, 0, 0) + CFG['WP'], 128), BF16)], [vmem((49, 2, FC // 2, 128), BF16)] * 2,
            vmem((NT, RING + 32, 128), I32), vmem((NT, RING, 128), I32), vmem((2, H * (DH + 4), 128), F32),
            vmem((NT, NF * 13 * TF // 4 + CFG['MP'], 128), BF16), vmem((NT // 2, (NA + 4) * 7 * TA // 2 + CFG['MP'], 128), BF16),
            vmem((H0 + NT * TF + 256, 128), F32),
            vmem((W, TA, 128), F32), vmem((2, NT, TA, 128), F32),
            vmem((16, TF // 4, 128), F32), [vmem((18, TF // 4, 128), F32)] * 2, vmem((49, 2, TF // 4, 128), BF16),
            pltpu.SemaphoreType.DMA((3,)),
        ],
        compiler_params=pltpu.CompilerParams(vmem_limit_bytes=127 * 1024 * 1024, flags=CFG['flags'] or None,
                                             disable_bounds_checks=CFG['nobc']),
    )(A_x.reshape(S, D), A_wqkv, A_wo, B_w_gate, B_w_up, B_w_down)
    return out.reshape(A_x.shape)
```

```python
import functools

import jax
import jax.experimental.pallas as pl
import jax.experimental.pallas.tpu as pltpu
import jax.numpy as jnp
import numpy as np
from jax import lax

S, D, DF = 2048, 1024, 3584
H, DH, W, DIL = 32, 32, 8, 2
NT = D // 128
TA = 256
NA = S // TA
TF, NF = 512, S // 512
FC = 512
HALO = 16
KS = HALO + S
K, Q, V, O = 0, 1, 2, 3
H0 = 4 * NT * KS
PR, RP = 32, 32
RING = 128
KC = 256
F32, BF16, I32 = jnp.float32, jnp.bfloat16, jnp.int32
P = functools.partial


def _layernorm(x):
    xc = x - jnp.mean(x, axis=-1, keepdims=True)
    return xc * lax.rsqrt(jnp.mean(xc * xc, axis=-1, keepdims=True) + 1e-5)


def _gelu(x):
    c = np.sqrt(2 / np.pi)
    half = 0.5 * x
    return half + half * jnp.tanh(x * (c + (c * 0.044715) * (x * x)))


def _operand(tiles):
    return pltpu.bitcast(jnp.concatenate(tiles, axis=1), BF16)


def _gather_tiles(tiles, sign):
    g = (lax.broadcasted_iota(I32, tiles[0].shape, 1) >> 2) & 7
    cur = [tiles[(sign * m) % NT] for m in range(NT)]
    for b in (1, 2, 4):
        cur = [jnp.where((g & b) != 0, cur[(m + sign * b) % NT], cur[m]) for m in range(NT)]
    return cur


def _shuffle_lanes(u, m):
    lane = lax.broadcasted_iota(I32, u.shape, 1)
    return jnp.take_along_axis(u, (lane & 3) * 32 + (((lane >> 2) - m) & 7) * 4 + (lane >> 5), axis=1)


LHS = ((0, 1, 3), (2, 1, 3), (0, 0, 0), (3, 0, 3), (0, 1, 1), (2, -1, 0), (1, -1, 3))
RHS = ((0, 1, 3), (0, 0, 0), (1, -1, 3), (2, -1, 0), (3, 0, 3), (0, 1, 1), (2, 1, 3))


def _term(rule, quadrant):
    a, sign, b = rule
    if sign == 0:
        return quadrant(a)
    x, y = quadrant(a).astype(F32), quadrant(b).astype(F32)
    return x + y if sign > 0 else x - y


def _terms(rules, *quadrants):
    return [_term(rule, quadrants.__getitem__) for rule in rules]


USES = (((0, 1), (3, 1)), ((2, 1), (3, -1)), ((1, 1), (3, 1)), ((0, 1), (2, 1)), ((1, 1), (0, -1)), ((3, 1),), ((0, 1),))
UP_ORDER = (0, 1, 3, 2, 4, 5, 6)
DOWN_ORDER = (3, 6, 1, 0, 2, 4, 5)


def _combine(products, order):
    acc, left = {}, [4, 2, 2, 4]
    for n in order:
        for part, m in products(n):
            for q, sign in USES[n]:
                if (q, part) not in acc:
                    acc[q, part] = (sign, m)
                else:
                    s, c = acc[q, part]
                    acc[q, part] = (1, c + m if s == sign else c - m if s > 0 else m - c)
                if left[q] == 1:
                    yield q, part, acc[q, part][1]
        for q, _ in USES[n]:
            left[q] -= 1


def _quadrants(product, order):
    return ((q, y) for q, _, y in _combine(lambda n: [(0, product(n))], order))


def _inner_terms(rules, k, block):
    outer = [_term(rules[k], lambda q: block(q // 2 * 2 + i, q % 2 * 2 + j)) for i in (0, 1) for j in (0, 1)]
    return enumerate(_terms(rules, *outer), 7 * k)


def _sixteenths(product, order):
    for o, i, y in _combine(lambda k: _quadrants(lambda n: product(7 * k + n), order), order):
        yield o // 2 * 2 + i // 2, o % 2 * 2 + i % 2, y


def _merge(*lists):
    keyed = [((n + 0.5) / len(l), k, t) for k, l in enumerate(lists) for n, t in enumerate(l)]
    return [t for _, _, t in sorted(keyed, key=lambda e: e[:2])]


def _pad(tasks, n, front=0):
    return [lambda: None] * front + tasks + [lambda: None] * n


def _rows(r, n):
    return pl.ds(r if isinstance(r, int) else pl.multiple_of(r, min(n, 16)), n)


def _cols(t):
    return slice(t * 128, (t + 1) * 128)


def _tile(s, t):
    return (s * NT + t) * KS + HALO


def _wterm(s, n, t):
    return ((s * 7 + n) * (NT // 2) + t) * (D // 2)


def _kernel(x_hbm, wqkv_hbm, wo_hbm, wg_hbm, wu_hbm, wd_hbm, out_hbm,
            x_v,
            wk_v,
            wgu2_v, wd2_v,
            t1_v, t2_v, t3_v,
            m_v,
            s_v,
            f_v,
            p_v, o_v,
            g_v, act_v, a_v,
            sems):
    m_w = m_v.bitcast(I32)
    raw = {Q: S, V: S + D, O: S + 2 * D}

    blocks = lambda lo, hi: (x_hbm.at[pl.ds(lo * TA, (hi - lo) * TA)], x_v.at[pl.ds(lo * TA, (hi - lo) * TA)])
    wk = lambda c: (wqkv_hbm.at[:, pl.ds(D + c * KC, KC)], wk_v.at[:, pl.ds(c * KC, KC)])
    copies = {
        'x0': blocks(0, 1), 'wk0': wk(0), 'x1': blocks(1, 2), 'wk1': wk(1), 'wk2': wk(2), 'wk3': wk(3),
        'x2': blocks(2, 3), 'x3': blocks(3, 5),
        'wq': (wqkv_hbm.at[:, pl.ds(0, D)], x_v.at[pl.ds(raw[Q], D)]),
        'wv': (wqkv_hbm.at[:, pl.ds(2 * D, D)], x_v.at[pl.ds(raw[V], D)]),
        'x5': blocks(5, NA), 'wo': (wo_hbm, x_v.at[pl.ds(raw[O], D)])}
    copies = {name: pltpu.make_async_copy(*c, sems.at[n % 3]) for n, (name, c) in enumerate(copies.items())}

    def start(*names):
        for n in names:
            copies[n].start()

    def wait(*names):
        for n in names:
            copies[n].wait()

    start('x0', 'wk0')
    zero = lax.while_loop(lambda c: c > 0, lambda c: c - 16, 16)

    def pace(y):
        x_v[_rows(zero + S + 3 * D, 16), 0:128] = y[:16, :128].astype(BF16)

    def run(*lists):
        for task in _merge(*lists):
            task()

    def project(s, j, tiles=range(NT), as_given=False):
        held = {}
        lhs_row, w_row, y_row = j * TA // 2, (S + s * D) // 2, _tile(s, 0) + j * TA

        def task(t, r0):
            if r0 == 0:
                lhs = _operand([m_w[k, _rows(lhs_row, TA // 2), :] for k in range(NT)])
                if as_given:
                    w = wk_v[:, _cols(t)]
                else:
                    w = _operand([m_w[t, _rows(w_row, D // 2), :]])
                held['y'] = jnp.dot(lhs, w, preferred_element_type=F32)
            y = held['y'][r0:r0 + RP]
            r = y_row + (t * KS + r0)
            pace(y)
            if as_given:
                t1_v[0, _rows(zero + RING, 8), :] = pltpu.bitcast(y[:8], I32)
            if s != K or j == 5:
                wgu2_v[1][_rows(zero + _wterm(4, 0, 0), 16), :] = y[:16].astype(BF16)
            f_v[_rows(r + zero, RP), :] = y
        return [P(task, t, r0) for t in tiles for r0 in range(0, TA, RP)]

    def lhs_terms(b, get):
        held, row = [], b * (7 * TA // 2)

        def task(r0, t):
            for n, lo, tile, u in held:
                s_v[tile, _rows(row + (n * (TA // 2) + lo), 16), :] = u
            held.clear()
            if r0 < TA // 2:
                blocks = [get(r, c) for r in (r0, r0 + TA // 2) for c in (t, t + NT // 2)]
                held.extend((n, r0, t, u.astype(BF16)) for n, u in enumerate(_terms(LHS, *blocks)))
        return [P(task, r0, t) for r0 in range(0, TA // 2, 16) for t in range(NT // 2)] + [P(task, TA // 2, 0)]

    def norm1(lo, hi):
        def task(j, r0):
            y = _layernorm(x_v[pl.ds(j * TA + r0, 16), :].astype(F32))
            for t in range(NT):
                if j <= 5:
                    m_v[t, pl.ds(j * TA + r0, 16), :] = y[:, _cols(t)].astype(BF16)
                if j >= 2:
                    o_v[zero + j % 2, t, pl.ds(r0, 16), :] = y[:, _cols(t)]
        tasks = []
        for j in range(lo, hi):
            late = lhs_terms(j - 1, lambda r, t, j=j: o_v[(j - 1) % 2, t, pl.ds(r, 16), :]) if j > 2 else []
            tasks += _merge([P(task, j, r) for r in range(0, TA, 16)], late)
        if hi == NA:
            tasks += lhs_terms(NA - 1, lambda r, t: o_v[(NA - 1) % 2, t, pl.ds(r, 16), :])
        return _pad(tasks, 2)

    def weights1(s):
        def task(r0, t):
            blocks = [m_v[c, pl.ds(S + s * D + r, 16), :] for r in (r0, r0 + D // 2) for c in (2 * t, 2 * t + 1)]
            for n, u in enumerate(_terms(RHS, *blocks)):
                wgu2_v[1][pl.ds(_wterm(s, n, t) + r0, 16), :] = u.astype(BF16)
        return [P(task, r0, t) for t in range(NT // 2) for r0 in range(0, D // 2, 16)]

    def hidden(r0, n, cs=range(NT)):
        y = jnp.concatenate([f_v[_rows(_tile(O, t) + r0, n), :] for t in cs], axis=1)
        return x_v[_rows(r0, n), cs[0] * 128:(cs[-1] + 1) * 128].astype(F32) + y

    def norm2(j):
        stats = {}

        def center(r):
            h = hidden(j * TF + r, 16)
            for t in range(NT):
                f_v[pl.ds(H0 + t * TF + r, 16), :] = h[:, _cols(t)]
            stats[r] = jnp.mean(h, axis=-1, keepdims=True)

        def spread(r):
            hc = jnp.concatenate([f_v[pl.ds(H0 + t * TF + r, 16), :] for t in range(NT)], axis=1) - stats[r]
            stats[r] = (stats[r], lax.rsqrt(jnp.mean(hc * hc, axis=-1, keepdims=True) + 1e-5))

        def scale(r):
            for t in range(NT):
                f_v[pl.ds(H0 + t * TF + r, 16), :] = (f_v[pl.ds(H0 + t * TF + r, 16), :] - stats[r][0]) * stats[r][1]
        return [P(f, r) for f in (center, spread, scale) for r in range(0, TF, 16)]

    def hn2(j, n):
        return j * (13 * TF // 8) + n // 4 * (TF // 8), n % 4 * 2

    def norm2_terms(j):
        def task(r0, t, k):
            for n, u in _inner_terms(LHS, k, lambda r, c: f_v[pl.ds(H0 + (2 * c + t) * TF + r * (TF // 4) + r0, 16), :]):
                row, col = hn2(0, n)
                m_v[col + t, _rows(j * (13 * TF // 4) + (2 * row + r0), 16), :] = u.astype(BF16)
        return [P(task, r0, t, k) for r0 in range(0, TF // 4, 16) for t in range(2) for k in range(7)]

    def staged(c):
        return S + (c & 1) * (D + FC)

    def ffn_copies(c):
        r, f = staged(c), pl.ds(pl.multiple_of(c * FC, FC), FC)
        return [pltpu.make_async_copy(wg_hbm.at[:, f], x_v.at[_rows(r, D), pl.ds(0, FC)], sems.at[0]),
                pltpu.make_async_copy(wu_hbm.at[:, f], x_v.at[_rows(r, D), pl.ds(FC, FC)], sems.at[1]),
                pltpu.make_async_copy(wd_hbm.at[f], x_v.at[_rows(r + D, FC)], sems.at[2])]

    def weights2(p, c, part, parts):
        n = D // 4 // parts
        up_src, down_src = staged(c) + part * n, staged(c) + D + part * (n // 2)
        up_row, down_row = c * (98 * 256) + part * n, c * 128 + part * (n // 2)

        def quad(r0, pitch, col, k):
            return _inner_terms(RHS, k, lambda r, c: x_v[
                _rows(r0 + r * pitch, 16), pl.ds(col + c // 2 * 256, 256)][:, _cols(c % 2)])

        def gate_up(r0, m, k):
            for n, u in quad(up_src + r0, D // 4, m * FC, k):
                wgu2_v[p % 2][_rows(up_row + ((2 * n + m) * 256 + r0), 16), :] = u.astype(BF16)

        def down(r0, t, k):
            for n, u in quad(down_src + r0, FC // 4, t * 512, k):
                wd2_v[p % 2][n, t, _rows(down_row + r0, 16), :] = u.astype(BF16)
        return ([P(gate_up, r, m, k) for r in range(0, n, 16) for m in (0, 1) for k in range(7)]
                + [P(down, r, t, k) for r in range(0, n // 2, 16) for t in (0, 1) for k in range(7)])

    def reorder_cols(s):
        def stage1(r0):
            src = (lambda t: wk_v[pl.ds(2 * r0, 16), _cols(t)]) if s == K else (
                lambda t: x_v[pl.ds(raw[s] + 2 * r0, 16), _cols(t)])
            for m, u in enumerate(_gather_tiles([pltpu.bitcast(src(t), I32) for t in range(NT)], 1)):
                t1_v[m, _rows(zero + r0 % RING, 8), :] = u

        def stage2(r0, m):
            t2_v[m, _rows(zero + r0 % RING, PR), :] = _shuffle_lanes(t1_v[m, pl.ds(r0 % RING, PR), :], m)

        def stage3(r0):
            for t, u in enumerate(_gather_tiles([t2_v[m, pl.ds(r0 % RING, 8), :] for m in range(NT)], -1)):
                m_w[t, pl.ds((S + s * D) // 2 + r0, 8), :] = u
        tasks = []
        for r0 in range(0, D // 2 + 2 * PR, PR):
            tasks += _merge([P(stage1, r) for r in range(r0, r0 + PR, 8) if r < D // 2],
                            [P(stage2, r0 - PR, m) for m in range(NT) if 0 <= r0 - PR < D // 2],
                            [P(stage3, r - 2 * PR) for r in range(r0, r0 + PR, 8) if r >= 2 * PR])
        return _pad(tasks, 16)

    def reorder_keys(j):
        held = []

        def task(r0):
            if held:
                lo, tiles = held.pop()
                for t, u in enumerate(tiles):
                    f_v[pl.ds(_tile(K, t) + lo, 8), :] = u
            if r0 < (j + 1) * TA:
                tiles = _gather_tiles([f_v[pl.ds(_tile(K, t) + r0, 8), :] for t in range(NT)], 1)
                held.append((r0, _gather_tiles([_shuffle_lanes(u, m) for m, u in enumerate(tiles)], -1)))
        return [P(task, r) for r in range(j * TA, (j + 1) * TA + 8, 8)]

    def reorder_rows():
        def stage1(t, h0):
            for h in range(h0, h0 + 4):
                t3_v[t % 2, pl.ds(zero + h * (DH + 1), DH), :] = x_v[pl.ds(raw[O] + h * DH, DH), _cols(t)].astype(F32)

        def stage2(t, d0):
            for d in range(d0, d0 + 4):
                m_v[t, pl.ds(S + O * D + d * H, H), :] = t3_v[t % 2, pl.ds(d, H, stride=DH + 1), :].astype(BF16)
        tasks = []
        for t in range(NT + 1):
            tasks += _merge([P(stage1, t, h) for h in range(0, H, 4) if t < NT],
                            [P(stage2, t - 1, d) for d in range(0, DH, 4) if t > 0])
        return _pad(tasks, 4)

    def fill_halo(s, t):
        f_v[pl.ds(_tile(s, t) - HALO, HALO), :] = jnp.broadcast_to(f_v[pl.ds(_tile(s, t), 1), :], (HALO, 128))

    def flush(j):
        return lhs_terms(NA + (j & 3), lambda r, t: o_v[j & 1, t, pl.ds(r, 16), :])

    def attention(i):
        lag = 32
        first = isinstance(i, int) and i == 0
        scale = DH ** -0.5

        def scores(parts, r0, ws):
            for t in range(NT):
                q = f_v[_rows(_tile(Q, t) + i * TA + r0, 16), :]
                for w in ws:
                    qk = q * f_v[pl.ds(_tile(K, t) + i * TA + r0 - DIL * w, 16), :]
                    parts[w] = qk if t == 0 else parts[w] + qk
            if len(parts) < W:
                return
            logits = []
            for w in range(W):
                l = parts[w] + pltpu.roll(parts[w], 64, 1)
                l = l + pltpu.roll(l, 32, 1)
                if first and r0 < DIL * w:
                    l = jnp.where(lax.broadcasted_iota(I32, l.shape, 0) + r0 >= DIL * w, l, -1e9 / scale)
                logits.append(l)
            top = functools.reduce(jnp.maximum, logits)
            e = [jnp.exp2((l - top) * (scale * np.log2(np.e))) for l in logits]
            inv = 1.0 / functools.reduce(jnp.add, e)
            for w in range(W):
                p_v[w, pl.ds(r0, 16), :] = e[w] * inv

        def mix(r0, ts):
            p = [p_v[w, pl.ds(r0, 16), :] for w in range(W)]
            for t in ts:
                o_v[i & 1, t, pl.ds(r0, 16), :] = functools.reduce(jnp.add, [
                    p[w] * f_v[pl.ds(_tile(V, t) + i * TA + r0 - DIL * w, 16), :] for w in range(W)])
        tasks = []
        for r0 in range(0, TA + lag, 16):
            a, b = [], []
            if r0 < TA:
                parts = {}
                a = [P(scores, parts, r0, [w]) for w in range(W)]
            if r0 >= lag:
                b = [P(mix, r0 - lag, [t]) for t in range(NT)]
            tasks += _merge(a, b)
        return _pad(tasks, 4)

    def keys01(lo, hi):
        return sum((project(K, j, [t], True) for t in range(lo, hi) for j in (0, 1)), [])

    wait('x0')
    start('x1')
    run(norm1(0, 1))
    wait('wk0')
    start('wk1')
    run(project(K, 0, range(2), True))
    wait('x1')
    start('wk2')
    run(norm1(1, 2) + project(K, 1, range(2), True))
    wait('wk1')
    start('wk3', 'x2')
    run(keys01(2, 4))
    wait('wk2', 'wk3')
    start('x3')
    run(keys01(4, NT), reorder_cols(K), _pad([P(start, 'wq')], 1, 1))
    wait('x2', 'x3')
    run(norm1(2, 3) + project(K, 2), _pad(reorder_keys(0), 2, 12), _pad(norm1(3, 5), 0, 12), [P(start, 'wv')])
    wait('wq')
    run(project(K, 3), reorder_cols(Q), [P(fill_halo, K, t) for t in range(NT)], [P(start, 'x5')])
    wait('wv')
    start('wo')
    run(project(K, 4), reorder_cols(V))
    wait('x5')
    run(project(V, 0) + project(Q, 0), reorder_keys(1), norm1(5, NA), weights1(K) + weights1(Q),
        _pad([P(fill_halo, V, t) for t in range(NT)], 0, NT))
    wait('wo')
    for copy in ffn_copies(0):
        copy.start()
    run(project(Q, 1) + project(V, 1) + project(K, 5), attention(0),
        _merge(reorder_rows(), weights1(V)) + weights1(O))


    def next_chunk(c, when):
        @pl.when(when)
        def _():
            for copy in ffn_copies(c):
                copy.wait()

            @pl.when(c < DF // FC - 1)
            def _():
                for copy in ffn_copies(c + 1):
                    copy.start()

    def paced(n_slots, parts, *spans):
        slots = [[] for _ in range(n_slots)]
        for tasks, where, reads in spans:
            for n, task in enumerate(tasks):
                slots[where[n * len(where) // len(tasks)]].append((task, reads))

        def product(lhs, rhs):
            y = jnp.dot(_operand(lhs), _operand([rhs]), preferred_element_type=F32)
            for r0 in range(0, y.shape[0], y.shape[0] // parts):
                tasks = slots.pop(0)
                if any(reads is f_v for _, reads in tasks):
                    f_v[_rows(zero + H0 + NT * TF, 8), :] = y[r0:r0 + 8]
                if any(reads is x_v for _, reads in tasks):
                    pace(y[r0:r0 + 16])
                for task, _ in tasks:
                    task()
            return y
        return product

    def project7(product, s, j):
        lhs_row = jnp.where(s == O, NA + (j & 3), j) * (7 * TA // 4)
        s_w, w_w = s_v.bitcast(I32), wgu2_v[1].bitcast(I32)
        w_row, y_row = s * (_wterm(1, 0, 0) // 2), _tile(s, 0) + j * TA
        for t in range(NT // 2):
            for q, y in _quadrants(lambda n: product(
                    [s_w[k, _rows(lhs_row + n * TA // 4, TA // 4), :] for k in range(NT // 2)],
                    w_w[_rows(w_row + _wterm(0, n, t) // 2, D // 4), :]), UP_ORDER):
                f_v[_rows(y_row + ((2 * t + q % 2) * KS + q // 2 * (TA // 2)), TA // 2), :] = y

    def step(i, _):
        last, late, n = i == NA - 1, i >= NA - 5, i - 1
        next_chunk(n >> 2, (n & 3) == 0)
        product = paced(84 * 8, 8, (attention(i), range(84 * 8), f_v), (flush(i - 1), range(4 * 8), None),
                        (weights2(0, n >> 2, n & 3, 4), range(82 * 8), x_v))
        project7(product, jnp.where(last, O, Q), jnp.where(last, NA - 4, i + 1))
        project7(product, jnp.where(last, O, V), jnp.where(last, NA - 3, i + 1))
        project7(product, jnp.where(late, O, K), jnp.where(late, jnp.where(last, NA - 2, i + 5 - NA), i + 5))
    lax.fori_loop(1, NA, step, None)
    run(flush(NA - 1))
    project7(paced(28 * 8, 8, (weights2(0, 1, 3, 4), range(216), x_v), (norm2(0) + norm2_terms(0), range(220), f_v)),
             O, NA - 1)

    def ffn(p, j, _):
        spans = []
        early, down = list(range(196)), list(range(196, 284))
        if p < 2:
            next_chunk(2 * p + 2 + (j >> 1), (j & 1) == 0)
            spans.append((weights2(p + 1, j >> 1, j & 1, 2), early + down[::2], x_v))
        if p == 2:
            next_chunk(2 * p + 2 + zero, j == 0)
            spans.append((weights2(p + 1, 0, j, NF), early + down[::2], x_v))
        if p == 0:
            nxt = jnp.minimum(j + 1, NF - 1)
            spans += [(norm2(nxt), early, f_v), (norm2_terms(nxt), down, f_v)]
        product = paced(294, 1, *spans)

        def lhs(n):
            row, col = hn2(j, n)
            return [m_w[col + t, _rows(row, TF // 8), :] for t in range(2)]

        chunks = 2 if p < 3 else 1
        wgu_w, wd_w, a_w = (ref.bitcast(I32) for ref in (wgu2_v[p % 2], wd2_v[p % 2], a_v))
        queue = []

        def terms(c, k, r0):
            for n, term in _inner_terms(LHS, k, lambda r, t: act_v[c][4 * r + t, pl.ds(r0, 16), :]):
                a_v[n, c, pl.ds(r0, 16), :] = term.astype(BF16)

        def up_product(c, m, n):
            y = product(lhs(n), wgu_w[pl.ds(((c * 49 + n) * 2 + m) * 128, 128), :])
            if queue:
                act_v[queue[0][0]][zero + 16, 0:8, :] = y[:8]
            for task in queue[:3 - chunks]:
                terms(*task)
            del queue[:3 - chunks]
            return y

        def down_product(i, n):
            while any(k == n // 7 for _, k, _ in queue):
                terms(*queue.pop(0))
            y = product([a_w[n, c] for c in range(chunks)], wd_w[n, i, 0:chunks * 64, :])
            if queue:
                act_v[queue[0][0]][zero + 16, 0:8, :] = y[:8]
            for task in queue[:2 * (3 - chunks)]:
                terms(*task)
            del queue[:2 * (3 - chunks)]
            return y
        for c in range(chunks):
            for r, t, g in _sixteenths(P(up_product, c, 0), UP_ORDER):
                g_v[zero + 4 * r + t] = _gelu(g)
            have, todo = [0] * 4, list(DOWN_ORDER)
            for r, t, u in _sixteenths(P(up_product, c, 1), UP_ORDER):
                act_v[c][zero + 4 * r + t] = g_v[4 * r + t] * u
                have[r // 2 * 2 + t // 2] += 1
                for k in [k for k in todo if have[LHS[k][0]] == have[LHS[k][2]] == 4]:
                    todo.remove(k)
                    queue += [(c, k, r0) for r0 in range(0, TF // 4, 16)]
        for i in range(2):
            rows = lambda r, c: _rows(_tile(Q, 4 * i + c) + j * TF + r * (TF // 4), TF // 4)
            for r, c, y in _sixteenths(P(down_product, i), DOWN_ORDER):
                if p < 3:
                    f_v[rows(r, c), :] = y + f_v[rows(r, c), :] if p else y
                else:
                    y = y + (f_v[rows(r, c), :] + hidden(j * TF + r * (TF // 4), TF // 4, [4 * i + c]))
                    block = (_rows(j * TF + r * (TF // 4), TF // 4), pl.ds((4 * i + c) * 128, 128))
                    x_v[block] = y.astype(BF16)
                    pltpu.make_async_copy(x_v.at[block], out_hbm.at[block], sems.at[0]).start()

    for p in range(4):
        lax.fori_loop(0, NF, P(ffn, p), None)
    pltpu.make_async_copy(x_v.at[pl.ds(0, S)], x_v.at[pl.ds(0, S)], sems.at[0]).wait()


@jax.jit
def pallas_sequential_preLN__sliding_local_dilated__glu_gated_geglu__prompt_kernel(
        A_x, A_wqkv, A_wo, B_x, B_w_gate, B_w_up, B_w_down):
    del B_x
    in_hbm = pl.BlockSpec(memory_space=pl.ANY)
    vmem = pltpu.VMEM
    out = pl.pallas_call(
        _kernel,
        in_specs=[in_hbm] * 6,
        out_specs=in_hbm,
        out_shape=jax.ShapeDtypeStruct((S, D), BF16),
        scratch_shapes=[
            vmem((S + 3 * D + 64, D), BF16),
            vmem((D, D), BF16), [vmem((2 * 49 * 2 * 256, 128), BF16), vmem((_wterm(4, 0, 0) + 512, 128), BF16)], [vmem((49, 2, FC // 2, 128), BF16)] * 2,
            vmem((NT, RING + 32, 128), I32), vmem((NT, RING, 128), I32), vmem((2, H * (DH + 4), 128), F32),
            vmem((NT, NF * 13 * TF // 4, 128), BF16), vmem((NT // 2, (NA + 4) * 7 * TA // 2, 128), BF16),
            vmem((H0 + NT * TF + 256, 128), F32),
            vmem((W, TA, 128), F32), vmem((2, NT, TA, 128), F32),
            vmem((16, TF // 4, 128), F32), [vmem((18, TF // 4, 128), F32)] * 2, vmem((49, 2, TF // 4, 128), BF16),
            pltpu.SemaphoreType.DMA((3,)),
        ],
        compiler_params=pltpu.CompilerParams(vmem_limit_bytes=127 * 1024 * 1024, disable_bounds_checks=True),
    )(A_x.reshape(S, D), A_wqkv, A_wo, B_w_gate, B_w_up, B_w_down)
    return out.reshape(A_x.shape)
```

```python
import functools

import jax
import jax.experimental.pallas as pl
import jax.experimental.pallas.tpu as pltpu
import jax.numpy as jnp
import numpy as np
from jax import lax

S, D, DF = 2048, 1024, 3584
H, DH, W, DIL = 32, 32, 8, 2
NT = D // 128
TA = 256
NA = S // TA
TF, NF = 512, S // 512
FC = 512
HALO = 16
KS = HALO + S
K, Q, V, O = 0, 1, 2, 3
H0 = 4 * NT * KS
PR, RP = 32, 32
RING = 128
KC = 256
F32, BF16, I32 = jnp.float32, jnp.bfloat16, jnp.int32
P = functools.partial


def _layernorm(x):
    xc = x - jnp.mean(x, axis=-1, keepdims=True)
    return xc * lax.rsqrt(jnp.mean(xc * xc, axis=-1, keepdims=True) + 1e-5)


def _gelu(x):
    c = np.sqrt(2 / np.pi)
    half = 0.5 * x
    return half + half * jnp.tanh(x * (c + (c * 0.044715) * (x * x)))


def _operand(tiles):
    return pltpu.bitcast(jnp.concatenate(tiles, axis=1), BF16)


def _gather_tiles(tiles, sign):
    g = (lax.broadcasted_iota(I32, tiles[0].shape, 1) >> 2) & 7
    cur = [tiles[(sign * m) % NT] for m in range(NT)]
    for b in (1, 2, 4):
        cur = [jnp.where((g & b) != 0, cur[(m + sign * b) % NT], cur[m]) for m in range(NT)]
    return cur


def _shuffle_lanes(u, m):
    lane = lax.broadcasted_iota(I32, u.shape, 1)
    return jnp.take_along_axis(u, (lane & 3) * 32 + (((lane >> 2) - m) & 7) * 4 + (lane >> 5), axis=1)


LHS = ((0, 1, 3), (2, 1, 3), (0, 0, 0), (3, 0, 3), (0, 1, 1), (2, -1, 0), (1, -1, 3))
RHS = ((0, 1, 3), (0, 0, 0), (1, -1, 3), (2, -1, 0), (3, 0, 3), (0, 1, 1), (2, 1, 3))


def _term(rule, quadrant):
    a, sign, b = rule
    if sign == 0:
        return quadrant(a)
    x, y = quadrant(a).astype(F32), quadrant(b).astype(F32)
    return x + y if sign > 0 else x - y


def _terms(rules, *quadrants):
    return [_term(rule, quadrants.__getitem__) for rule in rules]


USES = (((0, 1), (3, 1)), ((2, 1), (3, -1)), ((1, 1), (3, 1)), ((0, 1), (2, 1)), ((1, 1), (0, -1)), ((3, 1),), ((0, 1),))
UP_ORDER = (3, 1, 0, 5, 2, 4, 6)
DOWN_ORDER = (3, 1, 6, 0, 4, 2, 5)


def _combine(products, order):
    acc, left = {}, [4, 2, 2, 4]
    for n in order:
        for part, m in products(n):
            for q, sign in USES[n]:
                if (q, part) not in acc:
                    acc[q, part] = (sign, m)
                else:
                    s, c = acc[q, part]
                    acc[q, part] = (1, c + m if s == sign else c - m if s > 0 else m - c)
                if left[q] == 1:
                    yield q, part, acc[q, part][1]
        for q, _ in USES[n]:
            left[q] -= 1


def _quadrants(product, order):
    return ((q, y) for q, _, y in _combine(lambda n: [(0, product(n))], order))


def _inner_terms(rules, k, block):
    outer = [_term(rules[k], lambda q: block(q // 2 * 2 + i, q % 2 * 2 + j)) for i in (0, 1) for j in (0, 1)]
    return enumerate(_terms(rules, *outer), 7 * k)


def _sixteenths(product, order):
    for o, i, y in _combine(lambda k: _quadrants(lambda n: product(7 * k + n), UP_ORDER), order):
        yield o // 2 * 2 + i // 2, o % 2 * 2 + i % 2, y


def _merge(*lists):
    keyed = [((n + 0.5) / len(l), k, t) for k, l in enumerate(lists) for n, t in enumerate(l)]
    return [t for _, _, t in sorted(keyed, key=lambda e: e[:2])]


def _pad(tasks, n, front=0):
    return [lambda: None] * front + tasks + [lambda: None] * n


def _rows(r, n):
    return pl.ds(r if isinstance(r, int) else pl.multiple_of(r, min(n, 16)), n)


def _cols(t):
    return slice(t * 128, (t + 1) * 128)


def _tile(s, t):
    return (s * NT + t) * KS + HALO


def _wterm(s, n, t):
    return ((s * 7 + n) * (NT // 2) + t) * (D // 2)


def _kernel(x_hbm, wqkv_hbm, wo_hbm, wg_hbm, wu_hbm, wd_hbm, out_hbm,
            x_v,
            wk_v,
            wgu2_v, wd2_v,
            t1_v, t2_v, t3_v,
            m_v,
            s_v,
            f_v,
            p_v, o_v,
            g_v, act_v, a_v,
            sems):
    m_w = m_v.bitcast(I32)
    raw = {Q: S, V: S + D, O: S + 2 * D}

    blocks = lambda lo, hi: (x_hbm.at[pl.ds(lo * TA, (hi - lo) * TA)], x_v.at[pl.ds(lo * TA, (hi - lo) * TA)])
    wk = lambda c: (wqkv_hbm.at[:, pl.ds(D + c * KC, KC)], wk_v.at[:, pl.ds(c * KC, KC)])
    copies = {
        'x0': blocks(0, 1), 'wk0': wk(0), 'x1': blocks(1, 2), 'wk1': wk(1), 'wk2': wk(2), 'wk3': wk(3),
        'x2': blocks(2, 3), 'x3': blocks(3, 5),
        'wq': (wqkv_hbm.at[:, pl.ds(0, D)], x_v.at[pl.ds(raw[Q], D)]),
        'wv': (wqkv_hbm.at[:, pl.ds(2 * D, D)], x_v.at[pl.ds(raw[V], D)]),
        'x5': blocks(5, NA), 'wo': (wo_hbm, x_v.at[pl.ds(raw[O], D)])}
    copies = {name: pltpu.make_async_copy(*c, sems.at[n % 3]) for n, (name, c) in enumerate(copies.items())}

    def start(*names):
        for n in names:
            copies[n].start()

    def wait(*names):
        for n in names:
            copies[n].wait()

    start('x0', 'wk0')
    zero = lax.while_loop(lambda c: c > 0, lambda c: c - 16, 16)

    def pace(y):
        x_v[_rows(zero + S + 3 * D, 16), 0:128] = y[:16, :128].astype(BF16)

    def run(*lists):
        for task in _merge(*lists):
            task()

    def project(s, j, tiles=range(NT), as_given=False):
        held = {}
        lhs_row, w_row, y_row = j * TA // 2, (S + s * D) // 2, _tile(s, 0) + j * TA

        def task(t, r0):
            if r0 == 0:
                lhs = _operand([m_w[k, _rows(lhs_row, TA // 2), :] for k in range(NT)])
                if as_given:
                    w = wk_v[:, _cols(t)]
                else:
                    w = _operand([m_w[t, _rows(w_row, D // 2), :]])
                held['y'] = jnp.dot(lhs, w, preferred_element_type=F32)
            y = held['y'][r0:r0 + RP]
            r = y_row + (t * KS + r0)
            pace(y)
            if as_given:
                t1_v[0, _rows(zero + RING, 8), :] = pltpu.bitcast(y[:8], I32)
            if s != K or j == 5:
                wgu2_v[1][_rows(zero + _wterm(4, 0, 0), 16), :] = y[:16].astype(BF16)
            f_v[_rows(r + zero, RP), :] = y
        return [P(task, t, r0) for t in tiles for r0 in range(0, TA, RP)]

    def lhs_terms(b, get):
        held, row = [], b * (7 * TA // 2)

        def task(r0, t):
            for n, lo, tile, u in held:
                s_v[tile, _rows(row + (n * (TA // 2) + lo), 16), :] = u
            held.clear()
            if r0 < TA // 2:
                blocks = [get(r, c) for r in (r0, r0 + TA // 2) for c in (t, t + NT // 2)]
                held.extend((n, r0, t, u.astype(BF16)) for n, u in enumerate(_terms(LHS, *blocks)))
        return [P(task, r0, t) for r0 in range(0, TA // 2, 16) for t in range(NT // 2)] + [P(task, TA // 2, 0)]

    def norm1(lo, hi):
        def task(j, r0):
            y = _layernorm(x_v[pl.ds(j * TA + r0, 16), :].astype(F32))
            for t in range(NT):
                if j <= 5:
                    m_v[t, pl.ds(j * TA + r0, 16), :] = y[:, _cols(t)].astype(BF16)
                if j >= 2:
                    o_v[zero + j % 2, t, pl.ds(r0, 16), :] = y[:, _cols(t)]
        tasks = []
        for j in range(lo, hi):
            late = lhs_terms(j - 1, lambda r, t, j=j: o_v[(j - 1) % 2, t, pl.ds(r, 16), :]) if j > 2 else []
            tasks += _merge([P(task, j, r) for r in range(0, TA, 16)], late)
        if hi == NA:
            tasks += lhs_terms(NA - 1, lambda r, t: o_v[(NA - 1) % 2, t, pl.ds(r, 16), :])
        return _pad(tasks, 2)

    def weights1(s):
        def task(r0, t):
            blocks = [m_v[c, pl.ds(S + s * D + r, 16), :] for r in (r0, r0 + D // 2) for c in (2 * t, 2 * t + 1)]
            for n, u in enumerate(_terms(RHS, *blocks)):
                wgu2_v[1][pl.ds(_wterm(s, n, t) + r0, 16), :] = u.astype(BF16)
        return [P(task, r0, t) for t in range(NT // 2) for r0 in range(0, D // 2, 16)]

    def hidden(r0, n, cs=range(NT)):
        y = jnp.concatenate([f_v[_rows(_tile(O, t) + r0, n), :] for t in cs], axis=1)
        return x_v[_rows(r0, n), cs[0] * 128:(cs[-1] + 1) * 128].astype(F32) + y

    def norm2(j):
        stats = {}

        def center(r):
            h = hidden(j * TF + r, 16)
            for t in range(NT):
                f_v[pl.ds(H0 + t * TF + r, 16), :] = h[:, _cols(t)]
            stats[r] = jnp.mean(h, axis=-1, keepdims=True)

        def spread(r):
            hc = jnp.concatenate([f_v[pl.ds(H0 + t * TF + r, 16), :] for t in range(NT)], axis=1) - stats[r]
            stats[r] = (stats[r], lax.rsqrt(jnp.mean(hc * hc, axis=-1, keepdims=True) + 1e-5))

        def scale(r):
            for t in range(NT):
                f_v[pl.ds(H0 + t * TF + r, 16), :] = (f_v[pl.ds(H0 + t * TF + r, 16), :] - stats[r][0]) * stats[r][1]
        return [P(f, r) for f in (center, spread, scale) for r in range(0, TF, 16)]

    def hn2(j, n):
        return j * (13 * TF // 8) + n // 4 * (TF // 8), n % 4 * 2

    def norm2_terms(j):
        def task(r0, t, k):
            for n, u in _inner_terms(LHS, k, lambda r, c: f_v[pl.ds(H0 + (2 * c + t) * TF + r * (TF // 4) + r0, 16), :]):
                row, col = hn2(0, n)
                m_v[col + t, _rows(j * (13 * TF // 4) + (2 * row + r0), 16), :] = u.astype(BF16)
        return [P(task, r0, t, k) for r0 in range(0, TF // 4, 16) for t in range(2) for k in range(7)]

    def staged(c):
        return S + (c & 1) * (D + FC)

    def ffn_copies(c):
        r, f = staged(c), pl.ds(c * FC if isinstance(c, int) else pl.multiple_of(c * FC, FC), FC)
        return [pltpu.make_async_copy(wg_hbm.at[:, f], x_v.at[_rows(r, D), pl.ds(0, FC)], sems.at[0]),
                pltpu.make_async_copy(wu_hbm.at[:, f], x_v.at[_rows(r, D), pl.ds(FC, FC)], sems.at[1]),
                pltpu.make_async_copy(wd_hbm.at[f], x_v.at[_rows(r + D, FC)], sems.at[2])]

    def weights2(p, c, part, parts):
        n = D // 4 // parts
        up_src, down_src = staged(c) + part * n, staged(c) + D + part * (n // 2)
        up_row, down_row = c * (98 * 256) + part * n, c * 128 + part * (n // 2)

        def quad(r0, pitch, col, k):
            return _inner_terms(RHS, k, lambda r, c: x_v[
                _rows(r0 + r * pitch, 16), pl.ds(col + c // 2 * 256, 256)][:, _cols(c % 2)])

        def gate_up(r0, m, k):
            for n, u in quad(up_src + r0, D // 4, m * FC, k):
                wgu2_v[p % 2][_rows(up_row + ((2 * n + m) * 256 + r0), 16), :] = u.astype(BF16)

        def down(r0, t, k):
            for n, u in quad(down_src + r0, FC // 4, t * 512, k):
                wd2_v[p % 2][n, t, _rows(down_row + r0, 16), :] = u.astype(BF16)
        return ([P(gate_up, r, m, k) for r in range(0, n, 16) for m in (0, 1) for k in range(7)]
                + [P(down, r, t, k) for r in range(0, n // 2, 16) for t in (0, 1) for k in range(7)])

    def reorder_cols(s):
        def stage1(r0):
            src = (lambda t: wk_v[pl.ds(2 * r0, 16), _cols(t)]) if s == K else (
                lambda t: x_v[pl.ds(raw[s] + 2 * r0, 16), _cols(t)])
            for m, u in enumerate(_gather_tiles([pltpu.bitcast(src(t), I32) for t in range(NT)], 1)):
                t1_v[m, _rows(zero + r0 % RING, 8), :] = u

        def stage2(r0, m):
            t2_v[m, _rows(zero + r0 % RING, PR), :] = _shuffle_lanes(t1_v[m, pl.ds(r0 % RING, PR), :], m)

        def stage3(r0):
            for t, u in enumerate(_gather_tiles([t2_v[m, pl.ds(r0 % RING, 8), :] for m in range(NT)], -1)):
                m_w[t, pl.ds((S + s * D) // 2 + r0, 8), :] = u
        tasks = []
        for r0 in range(0, D // 2 + 2 * PR, PR):
            tasks += _merge([P(stage1, r) for r in range(r0, r0 + PR, 8) if r < D // 2],
                            [P(stage2, r0 - PR, m) for m in range(NT) if 0 <= r0 - PR < D // 2],
                            [P(stage3, r - 2 * PR) for r in range(r0, r0 + PR, 8) if r >= 2 * PR])
        return _pad(tasks, 16)

    def reorder_keys(j):
        held = []

        def task(r0):
            if held:
                lo, tiles = held.pop()
                for t, u in enumerate(tiles):
                    f_v[pl.ds(_tile(K, t) + lo, 8), :] = u
            if r0 < (j + 1) * TA:
                tiles = _gather_tiles([f_v[pl.ds(_tile(K, t) + r0, 8), :] for t in range(NT)], 1)
                held.append((r0, _gather_tiles([_shuffle_lanes(u, m) for m, u in enumerate(tiles)], -1)))
        return [P(task, r) for r in range(j * TA, (j + 1) * TA + 8, 8)]

    def reorder_rows():
        def stage1(t, h0):
            for h in range(h0, h0 + 4):
                t3_v[pl.ds(zero + (t % 2 * H * (DH + 4) + h * (DH + 1)), DH), :] = x_v[pl.ds(raw[O] + h * DH, DH), _cols(t)].astype(F32)

        def stage2(t, d0):
            for d in range(d0, d0 + 4):
                m_v[t, pl.ds(S + O * D + d * H, H), :] = t3_v[pl.ds(t % 2 * H * (DH + 4) + d, H, stride=DH + 1), :].astype(BF16)
        tasks = []
        for t in range(NT + 1):
            tasks += _merge([P(stage1, t, h) for h in range(0, H, 4) if t < NT],
                            [P(stage2, t - 1, d) for d in range(0, DH, 4) if t > 0])
        return _pad(tasks, 4)

    def fill_halo(s, t):
        f_v[pl.ds(_tile(s, t) - HALO, HALO), :] = jnp.broadcast_to(f_v[pl.ds(_tile(s, t), 1), :], (HALO, 128))

    def flush(j):
        return lhs_terms(NA + (j & 3), lambda r, t: o_v[j & 1, t, pl.ds(r, 16), :])

    def attention(i):
        lag = 32
        first = isinstance(i, int) and i == 0
        scale = DH ** -0.5

        def scores(parts, r0, ws):
            for t in range(NT):
                q = f_v[_rows(_tile(Q, t) + i * TA + r0, 16), :]
                for w in ws:
                    qk = q * f_v[pl.ds(_tile(K, t) + i * TA + r0 - DIL * w, 16), :]
                    parts[w] = qk if t == 0 else parts[w] + qk
            if len(parts) < W:
                return
            logits = []
            for w in range(W):
                l = parts[w] + pltpu.roll(parts[w], 64, 1)
                l = l + pltpu.roll(l, 32, 1)
                if first and r0 < DIL * w:
                    l = jnp.where(lax.broadcasted_iota(I32, l.shape, 0) + r0 >= DIL * w, l, -1e9 / scale)
                logits.append(l)
            top = functools.reduce(jnp.maximum, logits)
            e = [jnp.exp2((l - top) * (scale * np.log2(np.e))) for l in logits]
            inv = 1.0 / functools.reduce(jnp.add, e)
            for w in range(W):
                p_v[w, pl.ds(r0, 16), :] = e[w] * inv

        def mix(r0, ts):
            p = [p_v[w, pl.ds(r0, 16), :] for w in range(W)]
            for t in ts:
                o_v[i & 1, t, pl.ds(r0, 16), :] = functools.reduce(jnp.add, [
                    p[w] * f_v[pl.ds(_tile(V, t) + i * TA + r0 - DIL * w, 16), :] for w in range(W)])
        tasks = []
        for r0 in range(0, TA + lag, 16):
            a, b = [], []
            if r0 < TA:
                parts = {}
                a = [P(scores, parts, r0, [w]) for w in range(W)]
            if r0 >= lag:
                b = [P(mix, r0 - lag, [t]) for t in range(NT)]
            tasks += _merge(a, b)
        return _pad(tasks, 4)

    def keys01(lo, hi):
        return sum((project(K, j, [t], True) for t in range(lo, hi) for j in (0, 1)), [])

    wait('x0')
    start('x1')
    run(norm1(0, 1))
    wait('wk0')
    start('wk1')
    run(project(K, 0, range(2), True))
    wait('x1')
    start('wk2')
    run(norm1(1, 2) + project(K, 1, range(2), True))
    wait('wk1')
    start('wk3', 'x2')
    run(keys01(2, 4))
    wait('wk2', 'wk3')
    start('x3')
    run(keys01(4, NT), reorder_cols(K), _pad([P(start, 'wq')], 1, 1))
    wait('x2', 'x3')
    run(norm1(2, 3) + project(K, 2), _pad(reorder_keys(0), 2, 12), _pad(norm1(3, 5), 0, 12), [P(start, 'wv')])
    wait('wq')
    run(project(K, 3), reorder_cols(Q), [P(fill_halo, K, t) for t in range(NT)], [P(start, 'x5')])
    wait('wv')
    start('wo')
    run(project(K, 4), reorder_cols(V))
    wait('x5')
    run(project(V, 0) + project(Q, 0), reorder_keys(1), norm1(5, NA), weights1(K) + weights1(Q),
        _pad([P(fill_halo, V, t) for t in range(NT)], 0, NT))
    wait('wo')
    for copy in ffn_copies(0):
        copy.start()
    run(project(Q, 1) + project(V, 1) + project(K, 5), attention(0),
        _merge(reorder_rows(), weights1(V)) + weights1(O))


    def next_chunk(c, when):
        @pl.when(when)
        def _():
            for copy in ffn_copies(c):
                copy.wait()

            @pl.when(c < DF // FC - 1)
            def _():
                for copy in ffn_copies(c + 1):
                    copy.start()

    def paced(n_slots, parts, *spans):
        slots = [[] for _ in range(n_slots)]
        for tasks, where, reads in spans:
            for n, task in enumerate(tasks):
                slots[where[n * len(where) // len(tasks)]].append((task, reads))

        def product(lhs, rhs):
            y = jnp.dot(_operand(lhs), _operand([rhs]), preferred_element_type=F32)
            for r0 in range(0, y.shape[0], y.shape[0] // parts):
                tasks = slots.pop(0)
                if any(reads is f_v for _, reads in tasks):
                    f_v[_rows(zero + H0 + NT * TF, 8), :] = y[r0:r0 + 8]
                if any(reads is x_v for _, reads in tasks):
                    pace(y[r0:r0 + 16])
                for task, _ in tasks:
                    task()
            return y
        return product

    def project7(product, s, j):
        lhs_row = jnp.where(s == O, NA + (j & 3), j) * (7 * TA // 4)
        s_w, w_w = s_v.bitcast(I32), wgu2_v[1].bitcast(I32)
        w_row, y_row = s * (_wterm(1, 0, 0) // 2), _tile(s, 0) + j * TA
        for t in range(NT // 2):
            for q, y in _quadrants(lambda n: product(
                    [s_w[k, _rows(lhs_row + n * TA // 4, TA // 4), :] for k in range(NT // 2)],
                    w_w[_rows(w_row + _wterm(0, n, t) // 2, D // 4), :]), UP_ORDER):
                f_v[_rows(y_row + ((2 * t + q % 2) * KS + q // 2 * (TA // 2)), TA // 2), :] = y

    def step(i, _):
        last, late, n = i == NA - 1, i >= NA - 5, i - 1
        next_chunk(n >> 2, (n & 3) == 0)
        product = paced(84 * 8, 8, (attention(i), range(84 * 8), f_v), (flush(i - 1), range(4 * 8), None),
                        (weights2(0, n >> 2, n & 3, 4), range(82 * 8), x_v))
        project7(product, jnp.where(last, O, Q), jnp.where(last, NA - 4, i + 1))
        project7(product, jnp.where(last, O, V), jnp.where(last, NA - 3, i + 1))
        project7(product, jnp.where(late, O, K), jnp.where(late, jnp.where(last, NA - 2, i + 5 - NA), i + 5))
    lax.fori_loop(1, NA, step, None)
    run(flush(NA - 1))
    project7(paced(28 * 8, 8, (weights2(0, 1, 3, 4), range(130), x_v), (norm2(0) + norm2_terms(0), range(220), f_v)),
             O, NA - 1)

    def ffn(p, j, _):
        spans = []
        early, down = list(range(392)), list(range(392, 568))
        if p < 2:
            next_chunk(2 * p + 2 + (j >> 1), (j & 1) == 0)
            spans.append((weights2(p + 1, j >> 1, j & 1, 2), early + down[::2], x_v))
        if p == 2:
            next_chunk(2 * p + 2 + zero, j == 0)
            spans.append((weights2(p + 1, 0, j, NF), early + down[::2], x_v))
        if p == 0:
            nxt = jnp.minimum(j + 1, NF - 1)
            spans += [(norm2(nxt), early, f_v), (norm2_terms(nxt), range(420, 580), f_v)]
        product = paced(588, 2, *spans)

        def lhs(n):
            row, col = hn2(j, n)
            return [m_w[col + t, _rows(row, TF // 8), :] for t in range(2)]

        chunks = 2 if p < 3 else 1
        wgu_w, wd_w, a_w = (ref.bitcast(I32) for ref in (wgu2_v[p % 2], wd2_v[p % 2], a_v))
        queue = []

        def terms(c, k, r0):
            for n, term in _inner_terms(LHS, k, lambda r, t: act_v[c][4 * r + t, pl.ds(r0, 16), :]):
                a_v[n, c, pl.ds(r0, 16), :] = term.astype(BF16)

        def up_product(c, m, n):
            y = product(lhs(n), wgu_w[pl.ds(((c * 49 + n) * 2 + m) * 128, 128), :])
            if queue:
                act_v[queue[0][0]][zero + 16, 0:8, :] = y[:8]
            for task in queue[:3 - chunks]:
                terms(*task)
            del queue[:3 - chunks]
            return y

        def down_product(i, n):
            while any(k == n // 7 for _, k, _ in queue):
                terms(*queue.pop(0))
            y = product([a_w[n, c] for c in range(chunks)], wd_w[n, i, 0:chunks * 64, :])
            if queue:
                act_v[queue[0][0]][zero + 16, 0:8, :] = y[:8]
            for task in queue[:2 * (3 - chunks)]:
                terms(*task)
            del queue[:2 * (3 - chunks)]
            return y
        for c in range(chunks):
            for r, t, g in _sixteenths(P(up_product, c, 0), UP_ORDER):
                g_v[zero + 4 * r + t] = _gelu(g)
            have, todo = [0] * 4, list(DOWN_ORDER)
            for r, t, u in _sixteenths(P(up_product, c, 1), UP_ORDER):
                act_v[c][zero + 4 * r + t] = g_v[4 * r + t] * u
                have[r // 2 * 2 + t // 2] += 1
                for k in [k for k in todo if have[LHS[k][0]] == have[LHS[k][2]] == 4]:
                    todo.remove(k)
                    queue += [(c, k, r0) for r0 in range(0, TF // 4, 16)]
        for i in range(2):
            rows = lambda r, c: _rows(_tile(Q, 4 * i + c) + j * TF + r * (TF // 4), TF // 4)
            for r, c, y in _sixteenths(P(down_product, i), DOWN_ORDER):
                if p < 3:
                    f_v[rows(r, c), :] = y + f_v[rows(r, c), :] if p else y
                else:
                    y = y + (f_v[rows(r, c), :] + hidden(j * TF + r * (TF // 4), TF // 4, [4 * i + c]))
                    block = (_rows(j * TF + r * (TF // 4), TF // 4), pl.ds((4 * i + c) * 128, 128))
                    x_v[block] = y.astype(BF16)
                    pltpu.make_async_copy(x_v.at[block], out_hbm.at[block], sems.at[0]).start()

    for p in range(4):
        lax.fori_loop(0, NF, P(ffn, p), None)
    pltpu.make_async_copy(x_v.at[pl.ds(0, S)], x_v.at[pl.ds(0, S)], sems.at[0]).wait()


@jax.jit
def pallas_sequential_preLN__sliding_local_dilated__glu_gated_geglu__prompt_kernel(
        A_x, A_wqkv, A_wo, B_x, B_w_gate, B_w_up, B_w_down):
    del B_x
    in_hbm = pl.BlockSpec(memory_space=pl.ANY)
    vmem = pltpu.VMEM
    out = pl.pallas_call(
        _kernel,
        in_specs=[in_hbm] * 6,
        out_specs=in_hbm,
        out_shape=jax.ShapeDtypeStruct((S, D), BF16),
        scratch_shapes=[
            vmem((S + 3 * D + 64, D), BF16),
            vmem((D, D), BF16), [vmem((2 * 49 * 2 * 256, 128), BF16), vmem((_wterm(4, 0, 0) + 512, 128), BF16)], [vmem((49, 2, FC // 2, 128), BF16)] * 2,
            vmem((NT, RING + 32, 128), I32), vmem((NT, RING, 128), I32), vmem((2 * H * (DH + 4), 128), F32),
            vmem((NT, NF * 13 * TF // 4, 128), BF16), vmem((NT // 2, (NA + 4) * 7 * TA // 2, 128), BF16),
            vmem((H0 + NT * TF + 256, 128), F32),
            vmem((W, TA, 128), F32), vmem((2, NT, TA, 128), F32),
            vmem((16, TF // 4, 128), F32), [vmem((18, TF // 4, 128), F32)] * 2, vmem((49, 2, TF // 4, 128), BF16),
            pltpu.SemaphoreType.DMA((3,)),
        ],
        compiler_params=pltpu.CompilerParams(vmem_limit_bytes=127 * 1024 * 1024, disable_bounds_checks=True),
    )(A_x.reshape(S, D), A_wqkv, A_wo, B_w_gate, B_w_up, B_w_down)
    return out.reshape(A_x.shape)
```

```python
import functools

import jax
import jax.experimental.pallas as pl
import jax.experimental.pallas.tpu as pltpu
import jax.numpy as jnp
import numpy as np
from jax import lax

S, D, DF = 2048, 1024, 3584
H, DH, W, DIL = 32, 32, 8, 2
NT = D // 128
TA = 256
NA = S // TA
TF, NF = 512, S // 512
FC = 512
HALO = 16
KS = HALO + S
K, Q, V, O = 0, 1, 2, 3
H0 = 4 * NT * KS
PR, RP = 32, 32
RING = 128
KC = 256
F32, BF16, I32 = jnp.float32, jnp.bfloat16, jnp.int32
P = functools.partial


def _layernorm(x):
    xc = x - jnp.mean(x, axis=-1, keepdims=True)
    return xc * lax.rsqrt(jnp.mean(xc * xc, axis=-1, keepdims=True) + 1e-5)


def _gelu(x):
    c = np.sqrt(2 / np.pi)
    half = 0.5 * x
    return half + half * jnp.tanh(x * (c + (c * 0.044715) * (x * x)))


def _operand(tiles):
    return pltpu.bitcast(jnp.concatenate(tiles, axis=1), BF16)


def _gather_tiles(tiles, sign):
    g = (lax.broadcasted_iota(I32, tiles[0].shape, 1) >> 2) & 7
    cur = [tiles[(sign * m) % NT] for m in range(NT)]
    for b in (1, 2, 4):
        cur = [jnp.where((g & b) != 0, cur[(m + sign * b) % NT], cur[m]) for m in range(NT)]
    return cur


def _shuffle_lanes(u, m):
    lane = lax.broadcasted_iota(I32, u.shape, 1)
    return jnp.take_along_axis(u, (lane & 3) * 32 + (((lane >> 2) - m) & 7) * 4 + (lane >> 5), axis=1)


LHS = ((0, 1, 3), (2, 1, 3), (0, 0, 0), (3, 0, 3), (0, 1, 1), (2, -1, 0), (1, -1, 3))
RHS = ((0, 1, 3), (0, 0, 0), (1, -1, 3), (2, -1, 0), (3, 0, 3), (0, 1, 1), (2, 1, 3))


def _term(rule, quadrant):
    a, sign, b = rule
    if sign == 0:
        return quadrant(a)
    x, y = quadrant(a).astype(F32), quadrant(b).astype(F32)
    return x + y if sign > 0 else x - y


def _terms(rules, *quadrants):
    return [_term(rule, quadrants.__getitem__) for rule in rules]


USES = (((0, 1), (3, 1)), ((2, 1), (3, -1)), ((1, 1), (3, 1)), ((0, 1), (2, 1)), ((1, 1), (0, -1)), ((3, 1),), ((0, 1),))
GATE_ORDER = (6, 3, 1, 0, 4, 2, 5)
UP_ORDER = (3, 1, 0, 5, 2, 4, 6)
DOWN_ORDER = (3, 1, 6, 0, 4, 2, 5)


def _combine(products, order):
    acc, left = {}, [4, 2, 2, 4]
    for n in order:
        for part, m in products(n):
            for q, sign in USES[n]:
                if (q, part) not in acc:
                    acc[q, part] = (sign, m)
                else:
                    s, c = acc[q, part]
                    acc[q, part] = (1, c + m if s == sign else c - m if s > 0 else m - c)
                if left[q] == 1:
                    yield q, part, acc[q, part][1]
        for q, _ in USES[n]:
            left[q] -= 1


def _quadrants(product, order):
    return ((q, y) for q, _, y in _combine(lambda n: [(0, product(n))], order))


def _inner_terms(rules, k, block):
    outer = [_term(rules[k], lambda q: block(q // 2 * 2 + i, q % 2 * 2 + j)) for i in (0, 1) for j in (0, 1)]
    return enumerate(_terms(rules, *outer), 7 * k)


def _sixteenths(product, order):
    for o, i, y in _combine(lambda k: _quadrants(lambda n: product(7 * k + n), UP_ORDER), order):
        yield o // 2 * 2 + i // 2, o % 2 * 2 + i % 2, y


def _merge(*lists):
    keyed = [((n + 0.5) / len(l), k, t) for k, l in enumerate(lists) for n, t in enumerate(l)]
    return [t for _, _, t in sorted(keyed, key=lambda e: e[:2])]


def _pad(tasks, n, front=0):
    return [lambda: None] * front + tasks + [lambda: None] * n


def _rows(r, n):
    return pl.ds(r if isinstance(r, int) else pl.multiple_of(r, min(n, 16)), n)


def _cols(t):
    return slice(t * 128, (t + 1) * 128)


def _tile(s, t):
    return (s * NT + t) * KS + HALO


def _wterm(s, n, t):
    return ((s * 7 + n) * (NT // 2) + t) * (D // 2)


def _kernel(x_hbm, wqkv_hbm, wo_hbm, wg_hbm, wu_hbm, wd_hbm, out_hbm,
            x_v,
            wk_v,
            wgu2_v, wd2_v,
            t1_v, t2_v, t3_v,
            m_v,
            s_v,
            f_v,
            p_v, o_v,
            g_v, act_v, a_v,
            sems):
    m_w = m_v.bitcast(I32)
    raw = {Q: S, V: S + D, O: S + 2 * D}

    blocks = lambda lo, hi: (x_hbm.at[pl.ds(lo * TA, (hi - lo) * TA)], x_v.at[pl.ds(lo * TA, (hi - lo) * TA)])
    wk = lambda c: (wqkv_hbm.at[:, pl.ds(D + c * KC, KC)], wk_v.at[:, pl.ds(c * KC, KC)])
    copies = {
        'x0': blocks(0, 1), 'wk0': wk(0), 'x1': blocks(1, 2), 'wk1': wk(1), 'wk2': wk(2), 'wk3': wk(3),
        'x2': blocks(2, 3), 'x3': blocks(3, 5),
        'wq': (wqkv_hbm.at[:, pl.ds(0, D)], x_v.at[pl.ds(raw[Q], D)]),
        'wv': (wqkv_hbm.at[:, pl.ds(2 * D, D)], x_v.at[pl.ds(raw[V], D)]),
        'x5': blocks(5, NA), 'wo': (wo_hbm, x_v.at[pl.ds(raw[O], D)])}
    copies = {name: pltpu.make_async_copy(*c, sems.at[n % 3]) for n, (name, c) in enumerate(copies.items())}

    def start(*names):
        for n in names:
            copies[n].start()

    def wait(*names):
        for n in names:
            copies[n].wait()

    start('x0', 'wk0')
    zero = lax.while_loop(lambda c: c > 0, lambda c: c - 16, 16)

    def pace(y):
        x_v[_rows(zero + S + 3 * D, 16), 0:128] = y[:16, :128].astype(BF16)

    def run(*lists):
        for task in _merge(*lists):
            task()

    def project(s, j, tiles=range(NT), as_given=False):
        held = {}
        lhs_row, w_row, y_row = j * TA // 2, (S + s * D) // 2, _tile(s, 0) + j * TA

        def task(t, r0):
            if r0 == 0:
                lhs = _operand([m_w[k, _rows(lhs_row, TA // 2), :] for k in range(NT)])
                if as_given:
                    w = wk_v[:, _cols(t)]
                else:
                    w = _operand([m_w[t, _rows(w_row, D // 2), :]])
                held['y'] = jnp.dot(lhs, w, preferred_element_type=F32)
            y = held['y'][r0:r0 + RP]
            r = y_row + (t * KS + r0)
            pace(y)
            if as_given:
                t1_v[0, _rows(zero + RING, 8), :] = pltpu.bitcast(y[:8], I32)
            if s != K or j == 5:
                wgu2_v[1][_rows(zero + _wterm(4, 0, 0), 16), :] = y[:16].astype(BF16)
            f_v[_rows(r + zero, RP), :] = y
        return [P(task, t, r0) for t in tiles for r0 in range(0, TA, RP)]

    def lhs_terms(b, get):
        held, row = [], b * (7 * TA // 2)

        def task(r0, t):
            for n, lo, tile, u in held:
                s_v[tile, _rows(row + (n * (TA // 2) + lo), 16), :] = u
            held.clear()
            if r0 < TA // 2:
                blocks = [get(r, c) for r in (r0, r0 + TA // 2) for c in (t, t + NT // 2)]
                held.extend((n, r0, t, u.astype(BF16)) for n, u in enumerate(_terms(LHS, *blocks)))
        return [P(task, r0, t) for r0 in range(0, TA // 2, 16) for t in range(NT // 2)] + [P(task, TA // 2, 0)]

    def norm1(lo, hi):
        def task(j, r0):
            y = _layernorm(x_v[pl.ds(j * TA + r0, 16), :].astype(F32))
            for t in range(NT):
                if j <= 5:
                    m_v[t, pl.ds(j * TA + r0, 16), :] = y[:, _cols(t)].astype(BF16)
                if j >= 2:
                    o_v[zero + j % 2, t, pl.ds(r0, 16), :] = y[:, _cols(t)]
        tasks = []
        for j in range(lo, hi):
            late = lhs_terms(j - 1, lambda r, t, j=j: o_v[(j - 1) % 2, t, pl.ds(r, 16), :]) if j > 2 else []
            tasks += _merge([P(task, j, r) for r in range(0, TA, 16)], late)
        if hi == NA:
            tasks += lhs_terms(NA - 1, lambda r, t: o_v[(NA - 1) % 2, t, pl.ds(r, 16), :])
        return _pad(tasks, 2)

    def weights1(s):
        def task(r0, t):
            blocks = [m_v[c, pl.ds(S + s * D + r, 16), :] for r in (r0, r0 + D // 2) for c in (2 * t, 2 * t + 1)]
            for n, u in enumerate(_terms(RHS, *blocks)):
                wgu2_v[1][pl.ds(_wterm(s, n, t) + r0, 16), :] = u.astype(BF16)
        return [P(task, r0, t) for t in range(NT // 2) for r0 in range(0, D // 2, 16)]

    def hidden(r0, n, cs=range(NT)):
        y = jnp.concatenate([f_v[_rows(_tile(O, t) + r0, n), :] for t in cs], axis=1)
        return x_v[_rows(r0, n), cs[0] * 128:(cs[-1] + 1) * 128].astype(F32) + y

    def norm2(j):
        stats = {}

        def center(r):
            h = hidden(j * TF + r, 16)
            for t in range(NT):
                f_v[pl.ds(H0 + t * TF + r, 16), :] = h[:, _cols(t)]
            stats[r] = jnp.mean(h, axis=-1, keepdims=True)

        def spread(r):
            hc = jnp.concatenate([f_v[pl.ds(H0 + t * TF + r, 16), :] for t in range(NT)], axis=1) - stats[r]
            stats[r] = (stats[r], lax.rsqrt(jnp.mean(hc * hc, axis=-1, keepdims=True) + 1e-5))

        def scale(r):
            for t in range(NT):
                f_v[pl.ds(H0 + t * TF + r, 16), :] = (f_v[pl.ds(H0 + t * TF + r, 16), :] - stats[r][0]) * stats[r][1]
        return [P(f, r) for f in (center, spread, scale) for r in range(0, TF, 16)]

    def hn2(j, n):
        return j * (13 * TF // 8) + n // 4 * (TF // 8), n % 4 * 2

    def norm2_terms(j):
        def task(r0, t, k):
            for n, u in _inner_terms(LHS, k, lambda r, c: f_v[pl.ds(H0 + (2 * c + t) * TF + r * (TF // 4) + r0, 16), :]):
                row, col = hn2(0, n)
                m_v[col + t, _rows(j * (13 * TF // 4) + (2 * row + r0), 16), :] = u.astype(BF16)
        return [P(task, r0, t, k) for r0 in range(0, TF // 4, 16) for t in range(2) for k in range(7)]

    def staged(c):
        return S + (c & 1) * (D + FC)

    def ffn_copies(c):
        r, f = staged(c), pl.ds(c * FC if isinstance(c, int) else pl.multiple_of(c * FC, FC), FC)
        return [pltpu.make_async_copy(wg_hbm.at[:, f], x_v.at[_rows(r, D), pl.ds(0, FC)], sems.at[0]),
                pltpu.make_async_copy(wu_hbm.at[:, f], x_v.at[_rows(r, D), pl.ds(FC, FC)], sems.at[1]),
                pltpu.make_async_copy(wd_hbm.at[f], x_v.at[_rows(r + D, FC)], sems.at[2])]

    def weights2(p, c, part, parts):
        n = D // 4 // parts
        up_src, down_src = staged(c) + part * n, staged(c) + D + part * (n // 2)
        up_row, down_row = c * (98 * 256) + part * n, c * 128 + part * (n // 2)

        def quad(r0, pitch, col, k):
            return _inner_terms(RHS, k, lambda r, c: x_v[
                _rows(r0 + r * pitch, 16), pl.ds(col + c // 2 * 256, 256)][:, _cols(c % 2)])

        def gate_up(r0, m, k):
            for n, u in quad(up_src + r0, D // 4, m * FC, k):
                wgu2_v[p % 2][_rows(up_row + ((2 * n + m) * 256 + r0), 16), :] = u.astype(BF16)

        def down(r0, t, k):
            for n, u in quad(down_src + r0, FC // 4, t * 512, k):
                wd2_v[p % 2][n, t, _rows(down_row + r0, 16), :] = u.astype(BF16)
        return ([P(gate_up, r, m, k) for r in range(0, n, 16) for m in (0, 1) for k in range(7)]
                + [P(down, r, t, k) for r in range(0, n // 2, 16) for t in (0, 1) for k in range(7)])

    def reorder_cols(s):
        def stage1(r0):
            src = (lambda t: wk_v[pl.ds(2 * r0, 16), _cols(t)]) if s == K else (
                lambda t: x_v[pl.ds(raw[s] + 2 * r0, 16), _cols(t)])
            for m, u in enumerate(_gather_tiles([pltpu.bitcast(src(t), I32) for t in range(NT)], 1)):
                t1_v[m, _rows(zero + r0 % RING, 8), :] = u

        def stage2(r0, m):
            t2_v[m, _rows(zero + r0 % RING, PR), :] = _shuffle_lanes(t1_v[m, pl.ds(r0 % RING, PR), :], m)

        def stage3(r0):
            for t, u in enumerate(_gather_tiles([t2_v[m, pl.ds(r0 % RING, 8), :] for m in range(NT)], -1)):
                m_w[t, pl.ds((S + s * D) // 2 + r0, 8), :] = u
        tasks = []
        for r0 in range(0, D // 2 + 2 * PR, PR):
            tasks += _merge([P(stage1, r) for r in range(r0, r0 + PR, 8) if r < D // 2],
                            [P(stage2, r0 - PR, m) for m in range(NT) if 0 <= r0 - PR < D // 2],
                            [P(stage3, r - 2 * PR) for r in range(r0, r0 + PR, 8) if r >= 2 * PR])
        return _pad(tasks, 16)

    def reorder_keys(j):
        held = []

        def task(r0):
            if held:
                lo, tiles = held.pop()
                for t, u in enumerate(tiles):
                    f_v[pl.ds(_tile(K, t) + lo, 8), :] = u
            if r0 < (j + 1) * TA:
                tiles = _gather_tiles([f_v[pl.ds(_tile(K, t) + r0, 8), :] for t in range(NT)], 1)
                held.append((r0, _gather_tiles([_shuffle_lanes(u, m) for m, u in enumerate(tiles)], -1)))
        return [P(task, r) for r in range(j * TA, (j + 1) * TA + 8, 8)]

    def reorder_rows():
        def stage1(t, h0):
            for h in range(h0, h0 + 4):
                t3_v[pl.ds(zero + (t % 2 * H * (DH + 4) + h * (DH + 1)), DH), :] = x_v[pl.ds(raw[O] + h * DH, DH), _cols(t)].astype(F32)

        def stage2(t, d0):
            for d in range(d0, d0 + 4):
                m_v[t, pl.ds(S + O * D + d * H, H), :] = t3_v[pl.ds(t % 2 * H * (DH + 4) + d, H, stride=DH + 1), :].astype(BF16)
        tasks = []
        for t in range(NT + 1):
            tasks += _merge([P(stage1, t, h) for h in range(0, H, 4) if t < NT],
                            [P(stage2, t - 1, d) for d in range(0, DH, 4) if t > 0])
        return _pad(tasks, 4)

    def fill_halo(s, t):
        f_v[pl.ds(_tile(s, t) - HALO, HALO), :] = jnp.broadcast_to(f_v[pl.ds(_tile(s, t), 1), :], (HALO, 128))

    def flush(j):
        return lhs_terms(NA + (j & 3), lambda r, t: o_v[j & 1, t, pl.ds(r, 16), :])

    def attention(i):
        lag = 32
        first = isinstance(i, int) and i == 0
        scale = DH ** -0.5

        def scores(parts, r0, ws):
            for t in range(NT):
                q = f_v[_rows(_tile(Q, t) + i * TA + r0, 16), :]
                for w in ws:
                    qk = q * f_v[pl.ds(_tile(K, t) + i * TA + r0 - DIL * w, 16), :]
                    parts[w] = qk if t == 0 else parts[w] + qk
            if len(parts) < W:
                return
            logits = []
            for w in range(W):
                l = parts[w] + pltpu.roll(parts[w], 64, 1)
                l = l + pltpu.roll(l, 32, 1)
                if first and r0 < DIL * w:
                    l = jnp.where(lax.broadcasted_iota(I32, l.shape, 0) + r0 >= DIL * w, l, -1e9 / scale)
                logits.append(l)
            top = functools.reduce(jnp.maximum, logits)
            e = [jnp.exp2((l - top) * (scale * np.log2(np.e))) for l in logits]
            inv = 1.0 / functools.reduce(jnp.add, e)
            for w in range(W):
                p_v[w, pl.ds(r0, 16), :] = e[w] * inv

        def mix(r0, ts):
            p = [p_v[w, pl.ds(r0, 16), :] for w in range(W)]
            for t in ts:
                o_v[i & 1, t, pl.ds(r0, 16), :] = functools.reduce(jnp.add, [
                    p[w] * f_v[pl.ds(_tile(V, t) + i * TA + r0 - DIL * w, 16), :] for w in range(W)])
        tasks = []
        for r0 in range(0, TA + lag, 16):
            a, b = [], []
            if r0 < TA:
                parts = {}
                a = [P(scores, parts, r0, [w]) for w in range(W)]
            if r0 >= lag:
                b = [P(mix, r0 - lag, [t]) for t in range(NT)]
            tasks += _merge(a, b)
        return _pad(tasks, 4)

    def keys01(lo, hi):
        return sum((project(K, j, [t], True) for t in range(lo, hi) for j in (0, 1)), [])

    wait('x0')
    start('x1')
    run(norm1(0, 1))
    wait('wk0')
    start('wk1')
    run(project(K, 0, range(2), True))
    wait('x1')
    start('wk2')
    run(norm1(1, 2) + project(K, 1, range(2), True))
    wait('wk1')
    start('wk3', 'x2')
    run(keys01(2, 4))
    wait('wk2', 'wk3')
    start('x3')
    run(keys01(4, NT), reorder_cols(K), _pad([P(start, 'wq')], 1, 1))
    wait('x2', 'x3')
    run(norm1(2, 3) + project(K, 2), _pad(reorder_keys(0), 2, 12), _pad(norm1(3, 5), 0, 12), [P(start, 'wv')])
    wait('wq')
    run(project(K, 3), reorder_cols(Q), [P(fill_halo, K, t) for t in range(NT)], [P(start, 'x5')])
    wait('wv')
    start('wo')
    run(project(K, 4), reorder_cols(V))
    wait('x5')
    run(project(V, 0) + project(Q, 0), reorder_keys(1), norm1(5, NA), weights1(K) + weights1(Q),
        _pad([P(fill_halo, V, t) for t in range(NT)], 0, NT))
    wait('wo')
    for copy in ffn_copies(0):
        copy.start()
    run(project(Q, 1) + project(V, 1) + project(K, 5), attention(0),
        _merge(reorder_rows(), weights1(V)) + weights1(O))

    def next_chunk(c, when):
        @pl.when(when)
        def _():
            for copy in ffn_copies(c):
                copy.wait()

            @pl.when(c < DF // FC - 1)
            def _():
                for copy in ffn_copies(c + 1):
                    copy.start()

    def paced(n_slots, parts, *spans):
        slots = [[] for _ in range(n_slots)]
        for tasks, where, reads in spans:
            for n, task in enumerate(tasks):
                slots[where[n * len(where) // len(tasks)]].append((task, reads))

        def product(lhs, rhs):
            y = jnp.dot(_operand(lhs), _operand([rhs]), preferred_element_type=F32)
            for r0 in range(0, y.shape[0], y.shape[0] // parts):
                tasks = slots.pop(0)
                if any(reads is f_v for _, reads in tasks):
                    f_v[_rows(zero + H0 + NT * TF, 8), :] = y[r0:r0 + 8]
                if any(reads is x_v for _, reads in tasks):
                    pace(y[r0:r0 + 16])
                for task, _ in tasks:
                    task()
            return y
        return product

    def project7(product, s, j):
        lhs_row = jnp.where(s == O, NA + (j & 3), j) * (7 * TA // 4)
        s_w, w_w = s_v.bitcast(I32), wgu2_v[1].bitcast(I32)
        w_row, y_row = s * (_wterm(1, 0, 0) // 2), _tile(s, 0) + j * TA
        for t in range(NT // 2):
            for q, y in _quadrants(lambda n: product(
                    [s_w[k, _rows(lhs_row + n * TA // 4, TA // 4), :] for k in range(NT // 2)],
                    w_w[_rows(w_row + _wterm(0, n, t) // 2, D // 4), :]), UP_ORDER):
                f_v[_rows(y_row + ((2 * t + q % 2) * KS + q // 2 * (TA // 2)), TA // 2), :] = y

    def step(i, _):
        last, late, n = i == NA - 1, i >= NA - 5, i - 1
        next_chunk(n >> 2, (n & 3) == 0)
        product = paced(84 * 8, 8, (attention(i), range(84 * 8), f_v), (flush(i - 1), range(4 * 8), None),
                        (weights2(0, n >> 2, n & 3, 4), range(82 * 8), x_v))
        project7(product, jnp.where(last, O, Q), jnp.where(last, NA - 4, i + 1))
        project7(product, jnp.where(last, O, V), jnp.where(last, NA - 3, i + 1))
        project7(product, jnp.where(late, O, K), jnp.where(late, jnp.where(last, NA - 2, i + 5 - NA), i + 5))
    lax.fori_loop(1, NA, step, None)
    run(flush(NA - 1))
    project7(paced(28 * 8, 8, (weights2(0, 1, 3, 4), range(130), x_v), (norm2(0) + norm2_terms(0), range(220), f_v)),
             O, NA - 1)

    def ffn(p, j, _):
        spans = []
        early, down = list(range(392)), list(range(392, 568))
        if p < 2:
            next_chunk(2 * p + 2 + (j >> 1), (j & 1) == 0)
            spans.append((weights2(p + 1, j >> 1, j & 1, 2), early + down[::2], x_v))
        if p == 2:
            next_chunk(2 * p + 2 + zero, j == 0)
            spans.append((weights2(p + 1, 0, j, NF), early + down[::2], x_v))
        if p == 0:
            nxt = jnp.minimum(j + 1, NF - 1)
            spans += [(norm2(nxt), early, f_v), (norm2_terms(nxt), range(420, 580), f_v)]
        product = paced(588, 2, *spans)

        def lhs(n):
            row, col = hn2(j, n)
            return [m_w[col + t, _rows(row, TF // 8), :] for t in range(2)]

        chunks = 2 if p < 3 else 1
        wgu_w, wd_w, a_w = (ref.bitcast(I32) for ref in (wgu2_v[p % 2], wd2_v[p % 2], a_v))
        queue = []

        def terms(c, k, r0):
            for n, term in _inner_terms(LHS, k, lambda r, t: act_v[c][4 * r + t, pl.ds(r0, 16), :]):
                a_v[n, c, pl.ds(r0, 16), :] = term.astype(BF16)

        def up_product(c, m, n):
            y = product(lhs(n), wgu_w[pl.ds(((c * 49 + n) * 2 + m) * 128, 128), :])
            if queue:
                act_v[queue[0][0]][zero + 16, 0:8, :] = y[:8]
            for task in queue[:3 - chunks]:
                terms(*task)
            del queue[:3 - chunks]
            return y

        def down_product(i, n):
            while any(k == n // 7 for _, k, _ in queue):
                terms(*queue.pop(0))
            y = product([a_w[n, c] for c in range(chunks)], wd_w[n, i, 0:chunks * 64, :])
            if queue:
                act_v[queue[0][0]][zero + 16, 0:8, :] = y[:8]
            for task in queue[:1 if chunks == 2 else 3]:
                terms(*task)
            del queue[:1 if chunks == 2 else 3]
            return y
        for c in range(chunks):
            for r, t, g in _sixteenths(P(up_product, c, 0), GATE_ORDER):
                g_v[zero + 4 * r + t] = _gelu(g)
            have, todo = [0] * 4, list(DOWN_ORDER)
            for r, t, u in _sixteenths(P(up_product, c, 1), UP_ORDER):
                act_v[c][zero + 4 * r + t] = g_v[4 * r + t] * u
                have[r // 2 * 2 + t // 2] += 1
                for k in [k for k in todo if have[LHS[k][0]] == have[LHS[k][2]] == 4]:
                    todo.remove(k)
                    queue += [(c, k, r0) for r0 in range(0, TF // 4, 16)]
        for i in range(2):
            rows = lambda r, c: _rows(_tile(Q, 4 * i + c) + j * TF + r * (TF // 4), TF // 4)
            for r, c, y in _sixteenths(P(down_product, i), DOWN_ORDER):
                if p < 3:
                    f_v[rows(r, c), :] = y + f_v[rows(r, c), :] if p else y
                else:
                    y = y + (f_v[rows(r, c), :] + hidden(j * TF + r * (TF // 4), TF // 4, [4 * i + c]))
                    block = (_rows(j * TF + r * (TF // 4), TF // 4), pl.ds((4 * i + c) * 128, 128))
                    x_v[block] = y.astype(BF16)
                    pltpu.make_async_copy(x_v.at[block], out_hbm.at[block], sems.at[0]).start()

    for p in range(4):
        lax.fori_loop(0, NF, P(ffn, p), None)
    pltpu.make_async_copy(x_v.at[pl.ds(0, S)], x_v.at[pl.ds(0, S)], sems.at[0]).wait()


@jax.jit
def pallas_sequential_preLN__sliding_local_dilated__glu_gated_geglu__prompt_kernel(
        A_x, A_wqkv, A_wo, B_x, B_w_gate, B_w_up, B_w_down):
    del B_x
    in_hbm = pl.BlockSpec(memory_space=pl.ANY)
    vmem = pltpu.VMEM
    out = pl.pallas_call(
        _kernel,
        in_specs=[in_hbm] * 6,
        out_specs=in_hbm,
        out_shape=jax.ShapeDtypeStruct((S, D), BF16),
        scratch_shapes=[
            vmem((S + 3 * D + 64, D), BF16),
            vmem((D, D), BF16), [vmem((2 * 49 * 2 * 256, 128), BF16), vmem((_wterm(4, 0, 0) + 512, 128), BF16)], [vmem((49, 2, FC // 2, 128), BF16)] * 2,
            vmem((NT, RING + 32, 128), I32), vmem((NT, RING, 128), I32), vmem((2 * H * (DH + 4), 128), F32),
            vmem((NT, NF * 13 * TF // 4, 128), BF16), vmem((NT // 2, (NA + 4) * 7 * TA // 2, 128), BF16),
            vmem((H0 + NT * TF + 256, 128), F32),
            vmem((W, TA, 128), F32), vmem((2, NT, TA, 128), F32),
            vmem((16, TF // 4, 128), F32), [vmem((18, TF // 4, 128), F32)] * 2, vmem((49, 2, TF // 4, 128), BF16),
            pltpu.SemaphoreType.DMA((3,)),
        ],
        compiler_params=pltpu.CompilerParams(vmem_limit_bytes=127 * 1024 * 1024, disable_bounds_checks=True),
    )(A_x.reshape(S, D), A_wqkv, A_wo, B_w_gate, B_w_up, B_w_down)
    return out.reshape(A_x.shape)
```

```python
import functools

import jax
import jax.experimental.pallas as pl
import jax.experimental.pallas.tpu as pltpu
import jax.numpy as jnp
import numpy as np
from jax import lax

S, D, DF = 2048, 1024, 3584
H, DH, W, DIL = 32, 32, 8, 2
NT = D // 128
TA = 256
NA = S // TA
TF, NF = 512, S // 512
FC = 512
HALO = 16
KS = HALO + S
K, Q, V, O = 0, 1, 2, 3
H0 = 4 * NT * KS
PR, RP = 32, 32
RING = 128
KC = 256
F32, BF16, I32 = jnp.float32, jnp.bfloat16, jnp.int32
P = functools.partial


def _layernorm(x):
    xc = x - jnp.mean(x, axis=-1, keepdims=True)
    return xc * lax.rsqrt(jnp.mean(xc * xc, axis=-1, keepdims=True) + 1e-5)


def _gelu(x):
    c = np.sqrt(2 / np.pi)
    half = 0.5 * x
    return half + half * jnp.tanh(x * (c + (c * 0.044715) * (x * x)))


def _operand(tiles):
    return pltpu.bitcast(jnp.concatenate(tiles, axis=1), BF16)


def _gather_tiles(tiles, sign):
    g = (lax.broadcasted_iota(I32, tiles[0].shape, 1) >> 2) & 7
    cur = [tiles[(sign * m) % NT] for m in range(NT)]
    for b in (1, 2, 4):
        cur = [jnp.where((g & b) != 0, cur[(m + sign * b) % NT], cur[m]) for m in range(NT)]
    return cur


def _shuffle_lanes(u, m):
    lane = lax.broadcasted_iota(I32, u.shape, 1)
    return jnp.take_along_axis(u, (lane & 3) * 32 + (((lane >> 2) - m) & 7) * 4 + (lane >> 5), axis=1)


LHS = ((0, 1, 3), (2, 1, 3), (0, 0, 0), (3, 0, 3), (0, 1, 1), (2, -1, 0), (1, -1, 3))
RHS = ((0, 1, 3), (0, 0, 0), (1, -1, 3), (2, -1, 0), (3, 0, 3), (0, 1, 1), (2, 1, 3))


def _term(rule, quadrant):
    a, sign, b = rule
    if sign == 0:
        return quadrant(a)
    x, y = quadrant(a).astype(F32), quadrant(b).astype(F32)
    return x + y if sign > 0 else x - y


def _terms(rules, *quadrants):
    return [_term(rule, quadrants.__getitem__) for rule in rules]


USES = (((0, 1), (3, 1)), ((2, 1), (3, -1)), ((1, 1), (3, 1)), ((0, 1), (2, 1)), ((1, 1), (0, -1)), ((3, 1),), ((0, 1),))
GATE_ORDER = (6, 3, 1, 0, 4, 2, 5)
UP_ORDER = (3, 1, 0, 5, 2, 4, 6)
DOWN_ORDER = (3, 1, 6, 0, 4, 2, 5)


def _combine(products, order):
    acc, left = {}, [4, 2, 2, 4]
    for n in order:
        for part, m in products(n):
            for q, sign in USES[n]:
                if (q, part) not in acc:
                    acc[q, part] = (sign, m)
                else:
                    s, c = acc[q, part]
                    acc[q, part] = (1, c + m if s == sign else c - m if s > 0 else m - c)
                if left[q] == 1:
                    yield q, part, acc[q, part][1]
        for q, _ in USES[n]:
            left[q] -= 1


def _quadrants(product, order):
    return ((q, y) for q, _, y in _combine(lambda n: [(0, product(n))], order))


def _inner_terms(rules, k, block):
    outer = [_term(rules[k], lambda q: block(q // 2 * 2 + i, q % 2 * 2 + j)) for i in (0, 1) for j in (0, 1)]
    return enumerate(_terms(rules, *outer), 7 * k)


def _sixteenths(product, order):
    for o, i, y in _combine(lambda k: _quadrants(lambda n: product(7 * k + n), UP_ORDER), order):
        yield o // 2 * 2 + i // 2, o % 2 * 2 + i % 2, y


def _merge(*lists):
    keyed = [((n + 0.5) / len(l), k, t) for k, l in enumerate(lists) for n, t in enumerate(l)]
    return [t for _, _, t in sorted(keyed, key=lambda e: e[:2])]


def _pad(tasks, n, front=0):
    return [lambda: None] * front + tasks + [lambda: None] * n


def _rows(r, n):
    return pl.ds(r if isinstance(r, int) else pl.multiple_of(r, min(n, 16)), n)


def _cols(t):
    return slice(t * 128, (t + 1) * 128)


def _tile(s, t):
    return (s * NT + t) * KS + HALO


def _wterm(s, n, t):
    return ((s * 7 + n) * (NT // 2) + t) * (D // 2)


def _kernel(x_hbm, wqkv_hbm, wo_hbm, wg_hbm, wu_hbm, wd_hbm, out_hbm,
            x_v,
            wk_v,
            wgu2_v, wd2_v,
            t1_v, t2_v, t3_v,
            m_v,
            s_v,
            f_v,
            p_v, o_v,
            g_v, act_v, a_v,
            sems):
    m_w = m_v.bitcast(I32)
    raw = {Q: S, V: S + D, O: S + 2 * D}

    blocks = lambda lo, hi: (x_hbm.at[pl.ds(lo * TA, (hi - lo) * TA)], x_v.at[pl.ds(lo * TA, (hi - lo) * TA)])
    wk = lambda c: (wqkv_hbm.at[:, pl.ds(D + c * KC, KC)], wk_v.at[:, pl.ds(c * KC, KC)])
    copies = {
        'x0': blocks(0, 1), 'wk0': wk(0), 'x1': blocks(1, 2), 'wk1': wk(1), 'wk2': wk(2), 'wk3': wk(3),
        'x2': blocks(2, 3), 'x3': blocks(3, 5),
        'wq': (wqkv_hbm.at[:, pl.ds(0, D)], x_v.at[pl.ds(raw[Q], D)]),
        'wv': (wqkv_hbm.at[:, pl.ds(2 * D, D)], x_v.at[pl.ds(raw[V], D)]),
        'x5': blocks(5, NA), 'wo': (wo_hbm, x_v.at[pl.ds(raw[O], D)])}
    copies = {name: pltpu.make_async_copy(*c, sems.at[n % 3]) for n, (name, c) in enumerate(copies.items())}

    def start(*names):
        for n in names:
            copies[n].start()

    def wait(*names):
        for n in names:
            copies[n].wait()

    start('x0', 'wk0')
    zero = lax.while_loop(lambda c: c > 0, lambda c: c - 16, 16)

    def pace(y):
        x_v[_rows(zero + S + 3 * D, 16), 0:128] = y[:16, :128].astype(BF16)

    def run(*lists):
        for task in _merge(*lists):
            task()

    def project(s, j, tiles=range(NT), as_given=False):
        held = {}
        lhs_row, w_row, y_row = j * TA // 2, (S + s * D) // 2, _tile(s, 0) + j * TA

        def task(t, r0):
            if r0 == 0:
                lhs = _operand([m_w[k, _rows(lhs_row, TA // 2), :] for k in range(NT)])
                if as_given:
                    w = wk_v[:, _cols(t)]
                else:
                    w = _operand([m_w[t, _rows(w_row, D // 2), :]])
                held['y'] = jnp.dot(lhs, w, preferred_element_type=F32)
            y = held['y'][r0:r0 + RP]
            r = y_row + (t * KS + r0)
            pace(y)
            if as_given:
                t1_v[0, _rows(zero + RING, 8), :] = pltpu.bitcast(y[:8], I32)
            if (s, j) in ((V, 0), (Q, 1), (V, 1), (K, 4)):
                wgu2_v[1][_rows(zero + _wterm(4, 0, 0), 16), :] = y[:16].astype(BF16)
            f_v[_rows(r + zero, RP), :] = y
        return [P(task, t, r0) for t in tiles for r0 in range(0, TA, RP)]

    def lhs_terms(b, get):
        held, row = [], b * (7 * TA // 2)

        def task(r0, t):
            for n, lo, tile, u in held:
                s_v[tile, _rows(row + (n * (TA // 2) + lo), 16), :] = u
            held.clear()
            if r0 < TA // 2:
                blocks = [get(r, c) for r in (r0, r0 + TA // 2) for c in (t, t + NT // 2)]
                held.extend((n, r0, t, u.astype(BF16)) for n, u in enumerate(_terms(LHS, *blocks)))
        return [P(task, r0, t) for r0 in range(0, TA // 2, 16) for t in range(NT // 2)] + [P(task, TA // 2, 0)]

    def norm1(lo, hi):
        def task(j, r0):
            y = _layernorm(x_v[pl.ds(j * TA + r0, 16), :].astype(F32))
            for t in range(NT):
                if j <= 4:
                    m_v[t, pl.ds(j * TA + r0, 16), :] = y[:, _cols(t)].astype(BF16)
                if j >= 2:
                    o_v[zero + j % 2, t, pl.ds(r0, 16), :] = y[:, _cols(t)]
        tasks = []
        for j in range(lo, hi):
            late = lhs_terms(j - 1, lambda r, t, j=j: o_v[(j - 1) % 2, t, pl.ds(r, 16), :]) if j > 2 else []
            tasks += _merge([P(task, j, r) for r in range(0, TA, 16)], late)
        if hi == NA:
            tasks += lhs_terms(NA - 1, lambda r, t: o_v[(NA - 1) % 2, t, pl.ds(r, 16), :])
        return _pad(tasks, 2)

    def weights1(s):
        def task(r0, t):
            blocks = [m_v[c, pl.ds(S + s * D + r, 16), :] for r in (r0, r0 + D // 2) for c in (2 * t, 2 * t + 1)]
            for n, u in enumerate(_terms(RHS, *blocks)):
                wgu2_v[1][pl.ds(_wterm(s, n, t) + r0, 16), :] = u.astype(BF16)
        return [P(task, r0, t) for t in range(NT // 2) for r0 in range(0, D // 2, 16)]

    def hidden(r0, n, cs=range(NT)):
        y = jnp.concatenate([f_v[_rows(_tile(O, t) + r0, n), :] for t in cs], axis=1)
        return x_v[_rows(r0, n), cs[0] * 128:(cs[-1] + 1) * 128].astype(F32) + y

    def norm2(j):
        stats = {}

        def center(r):
            h = hidden(j * TF + r, 16)
            for t in range(NT):
                f_v[pl.ds(H0 + t * TF + r, 16), :] = h[:, _cols(t)]
            stats[r] = jnp.mean(h, axis=-1, keepdims=True)

        def spread(r):
            hc = jnp.concatenate([f_v[pl.ds(H0 + t * TF + r, 16), :] for t in range(NT)], axis=1) - stats[r]
            stats[r] = (stats[r], lax.rsqrt(jnp.mean(hc * hc, axis=-1, keepdims=True) + 1e-5))

        def scale(r):
            for t in range(NT):
                f_v[pl.ds(H0 + t * TF + r, 16), :] = (f_v[pl.ds(H0 + t * TF + r, 16), :] - stats[r][0]) * stats[r][1]
        return [P(f, r) for f in (center, spread, scale) for r in range(0, TF, 16)]

    def hn2(j, n):
        return j * (13 * TF // 8) + n // 4 * (TF // 8), n % 4 * 2

    def norm2_terms(j):
        def task(r0, t, k):
            for n, u in _inner_terms(LHS, k, lambda r, c: f_v[pl.ds(H0 + (2 * c + t) * TF + r * (TF // 4) + r0, 16), :]):
                row, col = hn2(0, n)
                m_v[col + t, _rows(j * (13 * TF // 4) + (2 * row + r0), 16), :] = u.astype(BF16)
        return [P(task, r0, t, k) for r0 in range(0, TF // 4, 16) for t in range(2) for k in range(7)]

    def staged(c):
        return S + (c & 1) * (D + FC)

    def ffn_copies(c):
        r, f = staged(c), pl.ds(c * FC if isinstance(c, int) else pl.multiple_of(c * FC, FC), FC)
        return [pltpu.make_async_copy(wg_hbm.at[:, f], x_v.at[_rows(r, D), pl.ds(0, FC)], sems.at[0]),
                pltpu.make_async_copy(wu_hbm.at[:, f], x_v.at[_rows(r, D), pl.ds(FC, FC)], sems.at[1]),
                pltpu.make_async_copy(wd_hbm.at[f], x_v.at[_rows(r + D, FC)], sems.at[2])]

    def weights2(p, c, part, parts):
        n = D // 4 // parts
        up_src, down_src = staged(c) + part * n, staged(c) + D + part * (n // 2)
        up_row, down_row = c * (98 * 256) + part * n, c * 128 + part * (n // 2)

        def quad(r0, pitch, col, k):
            return _inner_terms(RHS, k, lambda r, c: x_v[
                _rows(r0 + r * pitch, 16), pl.ds(col + c // 2 * 256, 256)][:, _cols(c % 2)])

        def gate_up(r0, m, k):
            for n, u in quad(up_src + r0, D // 4, m * FC, k):
                wgu2_v[p % 2][_rows(up_row + ((2 * n + m) * 256 + r0), 16), :] = u.astype(BF16)

        def down(r0, t, k):
            for n, u in quad(down_src + r0, FC // 4, t * 512, k):
                wd2_v[p % 2][n, t, _rows(down_row + r0, 16), :] = u.astype(BF16)
        return ([P(gate_up, r, m, k) for r in range(0, n, 16) for m in (0, 1) for k in range(7)]
                + [P(down, r, t, k) for r in range(0, n // 2, 16) for t in (0, 1) for k in range(7)])

    def reorder_cols(s):
        def stage1(r0):
            src = (lambda t: wk_v[pl.ds(2 * r0, 16), _cols(t)]) if s == K else (
                lambda t: x_v[pl.ds(raw[s] + 2 * r0, 16), _cols(t)])
            for m, u in enumerate(_gather_tiles([pltpu.bitcast(src(t), I32) for t in range(NT)], 1)):
                t1_v[m, _rows(zero + r0 % RING, 8), :] = u

        def stage2(r0, m):
            t2_v[m, _rows(zero + r0 % RING, PR), :] = _shuffle_lanes(t1_v[m, pl.ds(r0 % RING, PR), :], m)

        def stage3(r0):
            for t, u in enumerate(_gather_tiles([t2_v[m, pl.ds(r0 % RING, 8), :] for m in range(NT)], -1)):
                m_w[t, pl.ds((S + s * D) // 2 + r0, 8), :] = u
        tasks = []
        for r0 in range(0, D // 2 + 2 * PR, PR):
            tasks += _merge([P(stage1, r) for r in range(r0, r0 + PR, 8) if r < D // 2],
                            [P(stage2, r0 - PR, m) for m in range(NT) if 0 <= r0 - PR < D // 2],
                            [P(stage3, r - 2 * PR) for r in range(r0, r0 + PR, 8) if r >= 2 * PR])
        return _pad(tasks, 16)

    def reorder_keys(j):
        held = []

        def task(r0):
            if held:
                lo, tiles = held.pop()
                for t, u in enumerate(tiles):
                    f_v[pl.ds(_tile(K, t) + lo, 8), :] = u
            if r0 < (j + 1) * TA:
                tiles = _gather_tiles([f_v[pl.ds(_tile(K, t) + r0, 8), :] for t in range(NT)], 1)
                held.append((r0, _gather_tiles([_shuffle_lanes(u, m) for m, u in enumerate(tiles)], -1)))
        return [P(task, r) for r in range(j * TA, (j + 1) * TA + 8, 8)]

    def reorder_rows():
        def stage1(t, h0):
            for h in range(h0, h0 + 4):
                t3_v[pl.ds(zero + (t % 2 * H * (DH + 4) + h * (DH + 1)), DH), :] = x_v[pl.ds(raw[O] + h * DH, DH), _cols(t)].astype(F32)

        def stage2(t, d0):
            for d in range(d0, d0 + 4):
                m_v[t, pl.ds(S + O * D + d * H, H), :] = t3_v[pl.ds(t % 2 * H * (DH + 4) + d, H, stride=DH + 1), :].astype(BF16)
        tasks = []
        for t in range(NT + 1):
            tasks += _merge([P(stage1, t, h) for h in range(0, H, 4) if t < NT],
                            [P(stage2, t - 1, d) for d in range(0, DH, 4) if t > 0])
        return _pad(tasks, 4)

    def fill_halo(s, t):
        f_v[pl.ds(_tile(s, t) - HALO, HALO), :] = jnp.broadcast_to(f_v[pl.ds(_tile(s, t), 1), :], (HALO, 128))

    def flush(j):
        return lhs_terms(NA + (j & 3), lambda r, t: o_v[j & 1, t, pl.ds(r, 16), :])

    def attention(i):
        lag = 32
        first = isinstance(i, int) and i == 0
        scale = DH ** -0.5

        def scores(parts, r0, ws):
            for t in range(NT):
                q = f_v[_rows(_tile(Q, t) + i * TA + r0, 16), :]
                for w in ws:
                    qk = q * f_v[pl.ds(_tile(K, t) + i * TA + r0 - DIL * w, 16), :]
                    parts[w] = qk if t == 0 else parts[w] + qk
            if len(parts) < W:
                return
            logits = []
            for w in range(W):
                l = parts[w] + pltpu.roll(parts[w], 64, 1)
                l = l + pltpu.roll(l, 32, 1)
                if first and r0 < DIL * w:
                    l = jnp.where(lax.broadcasted_iota(I32, l.shape, 0) + r0 >= DIL * w, l, -1e9 / scale)
                logits.append(l)
            top = functools.reduce(jnp.maximum, logits)
            e = [jnp.exp2((l - top) * (scale * np.log2(np.e))) for l in logits]
            inv = 1.0 / functools.reduce(jnp.add, e)
            for w in range(W):
                p_v[w, pl.ds(r0, 16), :] = e[w] * inv

        def mix(r0, ts):
            p = [p_v[w, pl.ds(r0, 16), :] for w in range(W)]
            for t in ts:
                o_v[i & 1, t, pl.ds(r0, 16), :] = functools.reduce(jnp.add, [
                    p[w] * f_v[pl.ds(_tile(V, t) + i * TA + r0 - DIL * w, 16), :] for w in range(W)])
        tasks = []
        for r0 in range(0, TA + lag, 16):
            a, b = [], []
            if r0 < TA:
                parts = {}
                a = [P(scores, parts, r0, [w]) for w in range(W)]
            if r0 >= lag:
                b = [P(mix, r0 - lag, [t]) for t in range(NT)]
            tasks += _merge(a, b)
        return _pad(tasks, 4)

    def keys01(lo, hi):
        return sum((project(K, j, [t], True) for t in range(lo, hi) for j in (0, 1)), [])

    wait('x0')
    start('x1')
    run(norm1(0, 1))
    wait('wk0')
    start('wk1')
    run(project(K, 0, range(2), True))
    wait('x1')
    start('wk2')
    run(norm1(1, 2) + project(K, 1, range(2), True))
    wait('wk1')
    start('wk3', 'x2')
    run(keys01(2, 4))
    wait('wk2', 'wk3')
    start('x3')
    run(keys01(4, NT), reorder_cols(K), _pad([P(start, 'wq')], 1, 1))
    wait('x2', 'x3')
    run(norm1(2, 3) + project(K, 2), _pad(reorder_keys(0), 2, 12), _pad(norm1(3, 5), 0, 12), [P(start, 'wv')])
    wait('wq')
    run(project(K, 3), reorder_cols(Q), [P(fill_halo, K, t) for t in range(NT)], [P(start, 'x5')])
    wait('wv')
    start('wo')
    run(project(Q, 0), reorder_cols(V))
    wait('x5')
    run(project(V, 0) + project(Q, 1), reorder_keys(1), norm1(5, NA), weights1(K) + weights1(Q),
        _pad([P(fill_halo, V, t) for t in range(NT)], 0, NT))
    wait('wo')
    for copy in ffn_copies(0):
        copy.start()
    run(project(V, 1) + project(K, 4), attention(0),
        _merge(reorder_rows(), weights1(V)) + weights1(O))

    def next_chunk(c, when):
        @pl.when(when)
        def _():
            for copy in ffn_copies(c):
                copy.wait()

            @pl.when(c < DF // FC - 1)
            def _():
                for copy in ffn_copies(c + 1):
                    copy.start()

    def paced(n_slots, parts, *spans):
        slots = [[] for _ in range(n_slots)]
        for tasks, where, reads in spans:
            for n, task in enumerate(tasks):
                slots[where[n * len(where) // len(tasks)]].append((task, reads))

        def product(lhs, rhs):
            y = jnp.dot(_operand(lhs), _operand([rhs]), preferred_element_type=F32)
            for r0 in range(0, y.shape[0], y.shape[0] // parts):
                tasks = slots.pop(0)
                if any(reads is f_v for _, reads in tasks):
                    f_v[_rows(zero + H0 + NT * TF, 8), :] = y[r0:r0 + 8]
                if any(reads is x_v for _, reads in tasks):
                    pace(y[r0:r0 + 16])
                for task, _ in tasks:
                    task()
            return y
        return product

    def project7(product, s, j):
        lhs_row = jnp.where(s == O, NA + (j & 3), j) * (7 * TA // 4)
        s_w, w_w = s_v.bitcast(I32), wgu2_v[1].bitcast(I32)
        w_row, y_row = s * (_wterm(1, 0, 0) // 2), _tile(s, 0) + j * TA
        for t in range(NT // 2):
            for q, y in _quadrants(lambda n: product(
                    [s_w[k, _rows(lhs_row + n * TA // 4, TA // 4), :] for k in range(NT // 2)],
                    w_w[_rows(w_row + _wterm(0, n, t) // 2, D // 4), :]), UP_ORDER):
                f_v[_rows(y_row + ((2 * t + q % 2) * KS + q // 2 * (TA // 2)), TA // 2), :] = y

    def step(i, _):
        last, late, n = i == NA - 1, i >= NA - 4, i - 1
        next_chunk(n >> 2, (n & 3) == 0)
        product = paced(84 * 8, 8, (attention(i), range(84 * 8), f_v), (flush(i - 1), range(5 * 8), None),
                        (weights2(0, n >> 2, n & 3, 4), list(range(40, 84 * 8)) + list(range(76 * 8, 84 * 8)), x_v))
        project7(product, jnp.where(last, O, Q), jnp.where(last, NA - 5, i + 1))
        project7(product, jnp.where(last, O, V), jnp.where(last, NA - 4, i + 1))
        project7(product, jnp.where(late, O, K), jnp.where(late, jnp.where(last, NA - 3, i + 4 - NA), i + 4))
    lax.fori_loop(1, NA, step, None)
    product = paced(56 * 8, 8, (flush(NA - 1), range(100), None), (weights2(0, 1, 3, 4), range(440), x_v),
                    (norm2(0) + norm2_terms(0), range(440), f_v))
    project7(product, O, NA - 2)
    project7(product, O, NA - 1)

    def ffn(p, j, _):
        spans = []
        early, down = list(range(392)), list(range(392, 568))
        if p < 2:
            next_chunk(2 * p + 2 + (j >> 1), (j & 1) == 0)
            spans.append((weights2(p + 1, j >> 1, j & 1, 2), early + down[::2], x_v))
        if p == 2:
            next_chunk(2 * p + 2 + zero, j == 0)
            spans.append((weights2(p + 1, 0, j, NF), early + down[::2], x_v))
        if p == 0:
            nxt = jnp.minimum(j + 1, NF - 1)
            spans += [(norm2(nxt), early, f_v), (norm2_terms(nxt), range(420, 580), f_v)]
        product = paced(588, 2, *spans)

        def lhs(n):
            row, col = hn2(j, n)
            return [m_w[col + t, _rows(row, TF // 8), :] for t in range(2)]

        chunks = 2 if p < 3 else 1
        wgu_w, wd_w, a_w = (ref.bitcast(I32) for ref in (wgu2_v[p % 2], wd2_v[p % 2], a_v))
        queue = []

        def terms(c, k, r0):
            for n, term in _inner_terms(LHS, k, lambda r, t: act_v[c][4 * r + t, pl.ds(r0, 16), :]):
                a_v[n, c, pl.ds(r0, 16), :] = term.astype(BF16)

        def up_product(c, m, n):
            y = product(lhs(n), wgu_w[pl.ds(((c * 49 + n) * 2 + m) * 128, 128), :])
            if queue:
                act_v[queue[0][0]][zero + 16, 0:8, :] = y[:8]
            for task in queue[:3 - chunks]:
                terms(*task)
            del queue[:3 - chunks]
            return y

        def down_product(i, n):
            while any(k == n // 7 for _, k, _ in queue):
                terms(*queue.pop(0))
            y = product([a_w[n, c] for c in range(chunks)], wd_w[n, i, 0:chunks * 64, :])
            if queue:
                act_v[queue[0][0]][zero + 16, 0:8, :] = y[:8]
            for task in queue[:1 if chunks == 2 else 3]:
                terms(*task)
            del queue[:1 if chunks == 2 else 3]
            return y
        for c in range(chunks):
            for r, t, g in _sixteenths(P(up_product, c, 0), GATE_ORDER):
                g_v[zero + 4 * r + t] = _gelu(g)
            have, todo = [0] * 4, list(DOWN_ORDER)
            for r, t, u in _sixteenths(P(up_product, c, 1), UP_ORDER):
                act_v[c][zero + 4 * r + t] = g_v[4 * r + t] * u
                have[r // 2 * 2 + t // 2] += 1
                for k in [k for k in todo if have[LHS[k][0]] == have[LHS[k][2]] == 4]:
                    todo.remove(k)
                    queue += [(c, k, r0) for r0 in range(0, TF // 4, 16)]
        for i in range(2):
            rows = lambda r, c: _rows(_tile(Q, 4 * i + c) + j * TF + r * (TF // 4), TF // 4)
            for r, c, y in _sixteenths(P(down_product, i), DOWN_ORDER):
                if p < 3:
                    f_v[rows(r, c), :] = y + f_v[rows(r, c), :] if p else y
                else:
                    y = y + (f_v[rows(r, c), :] + hidden(j * TF + r * (TF // 4), TF // 4, [4 * i + c]))
                    block = (_rows(j * TF + r * (TF // 4), TF // 4), pl.ds((4 * i + c) * 128, 128))
                    x_v[block] = y.astype(BF16)
                    pltpu.make_async_copy(x_v.at[block], out_hbm.at[block], sems.at[0]).start()

    for p in range(4):
        lax.fori_loop(0, NF, P(ffn, p), None)
    pltpu.make_async_copy(x_v.at[pl.ds(0, S)], x_v.at[pl.ds(0, S)], sems.at[0]).wait()


@jax.jit
def pallas_sequential_preLN__sliding_local_dilated__glu_gated_geglu__prompt_kernel(
        A_x, A_wqkv, A_wo, B_x, B_w_gate, B_w_up, B_w_down):
    del B_x
    in_hbm = pl.BlockSpec(memory_space=pl.ANY)
    vmem = pltpu.VMEM
    out = pl.pallas_call(
        _kernel,
        in_specs=[in_hbm] * 6,
        out_specs=in_hbm,
        out_shape=jax.ShapeDtypeStruct((S, D), BF16),
        scratch_shapes=[
            vmem((S + 3 * D + 64, D), BF16),
            vmem((D, D), BF16), [vmem((2 * 49 * 2 * 256, 128), BF16), vmem((_wterm(4, 0, 0) + 512, 128), BF16)], [vmem((49, 2, FC // 2, 128), BF16)] * 2,
            vmem((NT, RING + 32, 128), I32), vmem((NT, RING, 128), I32), vmem((2 * H * (DH + 4), 128), F32),
            vmem((NT, NF * 13 * TF // 4, 128), BF16), vmem((NT // 2, (NA + 4) * 7 * TA // 2, 128), BF16),
            vmem((H0 + NT * TF + 256, 128), F32),
            vmem((W, TA, 128), F32), vmem((2, NT, TA, 128), F32),
            vmem((16, TF // 4, 128), F32), [vmem((18, TF // 4, 128), F32)] * 2, vmem((49, 2, TF // 4, 128), BF16),
            pltpu.SemaphoreType.DMA((3,)),
        ],
        compiler_params=pltpu.CompilerParams(vmem_limit_bytes=127 * 1024 * 1024, disable_bounds_checks=True),
    )(A_x.reshape(S, D), A_wqkv, A_wo, B_w_gate, B_w_up, B_w_down)
    return out.reshape(A_x.shape)
```
